```python
import jax
import jax.numpy as jnp

def _softmax(x, axis=-1):
    return jax.nn.softmax(x, axis=axis)
def _gelu(x):
    return jax.nn.gelu(x, approximate=True)
def _silu(x):
    return jax.nn.silu(x)
def _sigmoid(x):
    return jax.nn.sigmoid(x)
def _layernorm(x, axis=-1, eps=1e-5):
    m = jnp.mean(x, axis=axis, keepdims=True)
    v = jnp.var(x, axis=axis, keepdims=True)
    return (x - m) / jnp.sqrt(v + eps)
def _scatter_add(tgt, idx, src, axis=0):
    return tgt.at[idx].add(src)
def _segment_sum(src, seg, n):
    return jax.ops.segment_sum(src, seg, n)
class _Rng:
    def __init__(self, key):
        self._k = key
    def _next(self):
        self._k, sub = jax.random.split(self._k)
        return sub
    def normal(self, shape):
        return jax.random.normal(self._next(), shape, dtype=jnp.bfloat16)
    def randint(self, lo, hi, shape):
        return jax.random.randint(self._next(), shape, lo, hi, dtype=jnp.int32)
    def uniform(self, shape, lo=0.0, hi=1.0):
        return jax.random.uniform(self._next(), shape, jnp.bfloat16, lo, hi)
    def permutation(self, n):
        return jax.random.permutation(self._next(), n)


kernel_name = 'standalone__modern_conv_block_convnext_v2__vision'

def setup_inputs():
    _rng = _Rng(jax.random.key(int.from_bytes(__import__("os").urandom(4), "little")))
    _w = (lambda a: (lambda t: t.astype(jnp.bfloat16) if jnp.issubdtype(t.dtype, jnp.floating) else t)(jnp.asarray(a)))
    H = W = 512
    C = 96
    K = 3
    return {
        "x": _w((lambda *s: _rng.normal(s) * 0.05)(1, H, W, C)),
        "dw": _w((lambda *s: _rng.normal(s) * 0.05)(K, K, C)),
        "w1": _w((lambda *s: _rng.normal(s) * 0.05)(C, 4 * C)),
        "w2": _w((lambda *s: _rng.normal(s) * 0.05)(4 * C, C)),
        "grn_gamma": _w((lambda *s: _rng.normal(s) * 0.05)(4 * C)),
        "grn_beta": _w((lambda *s: _rng.normal(s) * 0.05)(4 * C)),
    }

def reference(x, dw, w1, w2, grn_gamma, grn_beta):
    B, H, W, C = x.shape
    K = dw.shape[0]
    pad = K // 2
    xp = jnp.pad(x, ((0,0),(pad,pad),(pad,pad),(0,0)))
    out = jnp.zeros_like(x)
    for i in range(K):
        for j in range(K):
            out = out + xp[:, i:i+H, j:j+W, :] * dw[i, j][None, None, None, :]
    h = _layernorm(out, axis=-1)
    h = jnp.einsum('bhwc,ce->bhwe', h, w1)
    h = _gelu(h)
    gx = jnp.sqrt((h * h).sum(axis=(1, 2), keepdims=True) + 1e-6)
    nx = gx / (gx.mean(axis=-1, keepdims=True) + 1e-6)
    h = grn_gamma * (h * nx) + grn_beta + h
    h = jnp.einsum('bhwe,ec->bhwc', h, w2)
    return x + h
```

```python
import functools
import math

import jax
import jax.numpy as jnp
import jax.experimental.pallas as pl
import jax.experimental.pallas.tpu as pltpu

F32 = jnp.float32
BF16 = jnp.bfloat16
U32 = jnp.uint32

_C0 = math.sqrt(2.0 / math.pi)
_KAPPA = (_C0 * 0.044715) ** (1.0 / 3.0)
_A = _C0 / _KAPPA
_GS = 2.0 * _KAPPA


def _u(x):
    return pltpu.bitcast(x, U32)


def _b(x):
    return pltpu.bitcast(x, BF16)


def _pk(v):
    k = v.shape[0] // 16
    ps = [pltpu.bitcast(pltpu.pack_elementwise(
        [v[16 * i:16 * i + 8], v[16 * i + 8:16 * i + 16]], packed_dtype=BF16), U32) for i in range(k)]
    return ps[0] if k == 1 else jnp.concatenate(ps, axis=0)


def _upk(p):
    return jnp.concatenate(
        [pltpu.unpack_elementwise(p, index=i, packed_dtype=BF16, unpacked_dtype=F32) for i in range(2)], axis=0)


def _perm(r):
    return (r // 16) * 16 + (r % 8) * 2 + (r % 16) // 8


def build(NBQ=2, XS=3, OS=3, U=4, P3=128, QA=(0, 2, 3), QB=None, vmem_mb=128, do1=True, do2=True):
    H, W, C, E = 512, 512, 96, 384
    NT = W // 128
    NQ = C // 16
    CH = 8
    NCH = H // CH
    NP = H // 2

    def kernel(x_hbm, dw_ref, w1_ref, w2t_ref, gam_ref, bet_ref,
               o_hbm,
               hst, xst, xr, w1t, w2s, b2b, acc, xsem, osem):

        def xcopy(c):
            return pltpu.make_async_copy(
                x_hbm.at[pl.ds((c % NCH) * CH, CH)], xr.at[pl.ds((c % XS) * CH, CH)], xsem.at[c % XS])

        for c in range(XS - 2):
            xcopy(c).start()

        def tiles(v):
            return [v[:, t * 128:(t + 1) * 128] for t in range(NT)]

        def mm1(xn_u, e0=0, e1=E):
            xp = jnp.concatenate([xn_u, jnp.zeros((64 - C // 2, W), U32)], axis=0)
            return jnp.dot(_b(w1t[e0 // 2:e1 // 2, :]), _b(xp), preferred_element_type=F32)

        def gelu(v):
            z = v * (v * v + _A)
            return v * (jnp.tanh(z) + 1.0)

        def pass1(dwb, la, lb, clr, ccu, ccf, cbuf, xnt, stat, nrm):
            rr = jax.lax.broadcasted_iota(jnp.int32, (C, C), 0)
            cc = jax.lax.broadcasted_iota(jnp.int32, (C, C), 1)
            dv = []
            for a in range(3):
                for b in range(3):
                    row = dw_ref[a, b:b + 1, :].astype(F32)
                    d = jnp.where(_perm(rr) == cc, jnp.broadcast_to(row, (C, C)), 0.0)
                    col = jnp.sum(d, axis=1, keepdims=True)
                    dv.append(jnp.broadcast_to(col, (C, 128)))
                dwb[a] = dv[a * 3 + 1]
            r16 = _perm(jax.lax.broadcasted_iota(jnp.int32, (16, 128), 0))
            c16 = jax.lax.broadcasted_iota(jnp.int32, (16, 128), 1)
            for q in range(NQ):
                ta, tb = [], []
                sf = slice(q * 16, q * 16 + 16)
                for o in range(2):
                    ma = jnp.zeros((16, 128), F32)
                    mb = jnp.zeros((16, 128), F32)
                    for a in range(3):
                        ma = jnp.where(c16 == (a + o) * 16 + r16, dv[a * 3 + 0][sf, :], ma)
                        ma = jnp.where(c16 == (4 + a + o) * 16 + r16, dv[a * 3 + 2][sf, :], ma)
                        mb = jnp.where(c16 == (a + o) * 16 + r16, dv[a * 3 + 1][sf, :], mb)
                    ta.append(ma)
                    tb.append(mb)
                la[q] = _u(jnp.concatenate(ta, axis=0).astype(BF16))
                lb[q] = _u(jnp.concatenate(tb, axis=0).astype(BF16))
            re = jax.lax.broadcasted_iota(jnp.int32, (E, E), 0)
            ce = jax.lax.broadcasted_iota(jnp.int32, (E, E), 1)
            eye = jnp.where(_perm(re) == ce, 1.0, 0.0).astype(BF16)
            w1p = jnp.concatenate([w1_ref[...], jnp.zeros((128 - C, E), BF16)], axis=0)
            t = jax.lax.dot_general(eye, w1p, (((1,), (1,)), ((), ())),
                                    preferred_element_type=F32)
            w1t[...] = _u(t.astype(BF16))
            acc[...] = jnp.zeros_like(acc)
            clr[...] = jnp.zeros_like(clr)
            ccu[...] = jnp.zeros_like(ccu)
            ccf[...] = jnp.zeros_like(ccf)
            xnt[...] = jnp.zeros_like(xnt)
            cbuf[...] = jnp.zeros_like(cbuf)
            stat[...] = jnp.zeros_like(stat)
            nrm[...] = jnp.zeros_like(nrm)
            xr[XS * CH:XS * CH + 2] = jnp.zeros((2, C, W), BF16)

            lane = jax.lax.broadcasted_iota(jnp.int32, (8, 128), 1)
            m0 = lane == 0
            m127 = lane == 127
            sub = jax.lax.broadcasted_iota(jnp.int32, (8, 128), 0)

            def butterfly(vs):
                for d in (1, 2, 4):
                    mk = (sub % (2 * d)) < d
                    vs = [jnp.where(mk, vs[i], vs[i + 1]) + pltpu.roll(jnp.where(mk, vs[i + 1], vs[i]), d, 0)
                          for i in range(0, len(vs), 2)]
                return vs[0]

            def s3(j, hidx, e0, e1):
                v_all = mm1(xnt[j], e0, e1)
                for e in range(e0 // 16, e1 // 16):
                    g = gelu(v_all[e * 16 - e0:(e + 1) * 16 - e0, :])
                    g2 = tiles(g * g)
                    acc[e * 16:(e + 1) * 16, :] += (g2[0] + g2[1]) + (g2[2] + g2[3])
                    if j == 0:
                        hst[hidx, e * 8:(e + 1) * 8, :] = _pk(g)

            def s2a(par, row, qs, fin):
                zero = jnp.zeros((8, 128), U32)
                if fin is None:
                    s1 = [None, None]
                    s2 = [None, None]
                else:
                    s1 = [stat[o, 0] for o in range(2)]
                    s2 = [stat[o, 1] for o in range(2)]

                def put(o, sf, c):
                    cbuf[par, o, sf, :] = c
                    a = c[0:8] + c[8:16]
                    b = c[0:8] * c[0:8] + c[8:16] * c[8:16]
                    s1[o] = a if s1[o] is None else s1[o] + a
                    s2[o] = b if s2[o] is None else s2[o] + b

                for q in qs:
                    su = slice(q * 8, q * 8 + 8)
                    sf = slice(q * 16, q * 16 + 16)
                    for n in range(2):
                        p = _u(xr[row + n, sf, :])
                        pt = tiles(p)
                        rl = [pltpu.roll(pt[t], 1, 1) for t in range(NT)]
                        rg = [pltpu.roll(pt[t], 127, 1) for t in range(NT)]
                        clr[par, n, 0, su, :] = jnp.concatenate(
                            [jnp.where(m0, rl[t - 1] if t > 0 else zero, rl[t]) for t in range(NT)], axis=1)
                        clr[par, n, 1, su, :] = jnp.concatenate(
                            [jnp.where(m127, rg[t + 1] if t < NT - 1 else zero, rg[t]) for t in range(NT)], axis=1)
                        if q < NBQ:
                            ccu[par, n, su, :] = p
                        else:
                            ccf[par, n, sf, :] = _upk(p)
                    rows = [(1 - par, 0), (1 - par, 1), (par, 0), (par, 1)]
                    rhs = _b(jnp.concatenate(
                        [clr[a, n, 0, su, :] for a, n in rows] + [clr[a, n, 1, su, :] for a, n in rows], axis=0))
                    ca = jnp.dot(_b(la[q]), rhs, preferred_element_type=F32)
                    if q < NBQ:
                        cs = [ccu[a, n, su, :] for a, n in rows] + [jnp.zeros((32, W), U32)]
                        rb = _b(jnp.concatenate(cs, axis=0))
                        ca = ca + jnp.dot(_b(lb[q]), rb, preferred_element_type=F32)
                        for o in range(2):
                            put(o, sf, ca[o * 16:(o + 1) * 16, :])
                    else:
                        cf = [ccf[a, n, sf, :] for a, n in rows]
                        ws = [jnp.concatenate([dwb[a, sf, :]] * NT, axis=1) for a in range(3)]
                        for o in range(2):
                            put(o, sf, (ca[o * 16:(o + 1) * 16, :] + ws[0] * cf[o]) + (
                                ws[1] * cf[o + 1] + ws[2] * cf[o + 2]))
                if fin is None:
                    for o in range(2):
                        stat[o, 0] = s1[o]
                        stat[o, 1] = s2[o]
                else:
                    m = butterfly(tiles(s1[0]) + tiles(s1[1])) * (1.0 / C)
                    q2 = butterfly(tiles(s2[0]) + tiles(s2[1])) * (1.0 / C)
                    var = jnp.maximum(q2 - m * m, 0.0)
                    rs = jax.lax.rsqrt(var + 1e-5) * jnp.where(sub < 4, fin[0], fin[1])
                    nrm[par, 0] = rs
                    nrm[par, 1] = m * rs

            def s2b(par, j, xidx):
                for t in range(NT):
                    rs = nrm[par, 0, j * 4 + t:j * 4 + t + 1, :]
                    mrs = nrm[par, 1, j * 4 + t:j * 4 + t + 1, :]
                    for q in range(NQ):
                        c = cbuf[par, j, q * 16:(q + 1) * 16, t * 128:(t + 1) * 128]
                        xn = _pk(c * rs - mrs)
                        xnt[j, q * 8:(q + 1) * 8, t * 128:(t + 1) * 128] = xn
                        if j == 1:
                            xst[xidx, q * 8:(q + 1) * 8, t * 128:(t + 1) * 128] = xn

            NSUB = CH // 2 // U
            QBB = QB if QB is not None else tuple(q for q in range(NQ) if q not in QA)
            P1 = E - P3

            def body1(kk, carry):
                c = kk // NSUB

                @pl.when(jnp.logical_and(kk % NSUB == 0, c < NCH))
                def _():
                    xcopy(c).wait()
                    xcopy(c + XS - 2).start()

                def xrow(k):
                    return jnp.where(jnp.logical_and(k >= 0, k < NP), (2 * k) % (XS * CH), XS * CH)

                for u in range(U):
                    k = kk * U + u - 1
                    par = (u + 1) % 2
                    j = k - 1
                    sc0 = jnp.where(jnp.logical_and(k >= 1, k <= NP), _KAPPA, 0.0)
                    sc1 = jnp.where(jnp.logical_and(k >= 0, k < NP), _KAPPA, 0.0)
                    xidx = jnp.where(j >= 0, jnp.minimum(j, NP), NP)
                    hidx = jnp.clip(k - 2, 0, NP)
                    s3(1, None, P1, E)
                    s2b(1 - par, 0, None)
                    s3(0, hidx, 0, P1)
                    s2a(par, xrow(k), QBB, (sc0, sc1))
                    s3(0, hidx, P1, E)
                    s2b(1 - par, 1, xidx)
                    s3(1, None, 0, P1)
                    s2a(1 - par, xrow(k + 1), QA, None)
                return carry
            if do1:
                jax.lax.fori_loop(0, -(-(NP + 3) // U), body1, 0)
                xcopy(NCH + XS - 2).start()
            else:
                for c in range(XS - 2):
                    xcopy(c).wait()
                for c in range(XS - 1):
                    xcopy(c + NCH).start()

        pl.run_scoped(
            pass1,
            pltpu.VMEM((3, C, 128), F32),
            pltpu.VMEM((NQ, 16, 128), U32),
            pltpu.VMEM((NQ, 16, 128), U32),
            pltpu.VMEM((2, 2, 2, C // 2, W), U32),
            pltpu.VMEM((2, 2, C // 2, W), U32),
            pltpu.VMEM((2, 2, C, W), F32),
            pltpu.VMEM((2, 2, C, W), F32),
            pltpu.VMEM((2, C // 2, W), U32),
            pltpu.VMEM((2, 2, 8, W), F32),
            pltpu.VMEM((2, 2, 8, 128), F32),
        )

        col = jnp.sum(acc[...], axis=1, keepdims=True)
        re = jax.lax.broadcasted_iota(jnp.int32, (E, E), 0)
        ce = jax.lax.broadcasted_iota(jnp.int32, (E, E), 1)
        a = jnp.where(_perm(re) == ce, jnp.broadcast_to(col, (E, E)), 0.0)
        ssq = jnp.sum(a, axis=0, keepdims=True) * (1.0 / (_GS * _GS))
        gx = jnp.sqrt(ssq + 1e-6)
        nx = gx / (jnp.mean(gx, axis=1, keepdims=True) + 1e-6)
        s = (gam_ref[...].astype(F32) * nx + 1.0) * (1.0 / _GS)
        w2f = w2t_ref[...].astype(F32)
        w2s[...] = _u((w2f * s).astype(BF16))
        b = jnp.sum(w2f * bet_ref[...].astype(F32), axis=1, keepdims=True)
        b2b[...] = jnp.broadcast_to(b, (C, 128))

        def pass2(orr, gt):
            def ocopy(c):
                return pltpu.make_async_copy(
                    orr.at[c % OS], o_hbm.at[pl.ds(c * CH, CH)], osem.at[c % OS])

            def t1(m, gslot):
                v_all = mm1(xst[m])
                for e in range(E // 16):
                    g = gelu(v_all[e * 16:(e + 1) * 16, :])
                    gt[gslot, e * 8:(e + 1) * 8, :] = _pk(g)

            def t2(g_u, xslot, oslot, row):
                y = jnp.dot(_b(w2s[...]), _b(g_u), preferred_element_type=F32)
                bb = jnp.concatenate([b2b[...]] * NT, axis=1)
                orr[oslot, row] = (y + (bb + xr[xslot * CH + row].astype(F32))).astype(BF16)

            def body2(c, carry):
                xcopy(NCH + c).wait()

                @pl.when(c + XS - 1 < NCH)
                def _():
                    xcopy(NCH + c + XS - 1).start()

                @pl.when(c >= OS)
                def _():
                    ocopy(c - OS).wait()

                xslot = (NCH + c) % XS
                oslot = c % OS
                for u in range(4):
                    m = c * 4 + u
                    t2(gt[u % 2], xslot, oslot, 2 * u)
                    t1(m + 1, (u + 1) % 2)
                    t2(hst[m], xslot, oslot, 2 * u + 1)
                ocopy(c).start()
                return carry

            if do2:
                t1(0, 0)
                jax.lax.fori_loop(0, NCH, body2, 0)
                for c in range(NCH - OS, NCH):
                    ocopy(c).wait()
            else:
                for c in range(XS - 1):
                    xcopy(c + NCH).wait()

        pl.run_scoped(pass2, pltpu.VMEM((OS, CH, C, W), BF16), pltpu.VMEM((2, E // 2, W), U32))

    @jax.jit
    def f(x, dw, w1, w2, grn_gamma, grn_beta):
        xt = jnp.transpose(x, (0, 1, 3, 2)).reshape(H, C, W)
        w2t = jnp.transpose(w2)
        gam = grn_gamma.reshape(1, E)
        bet = grn_beta.reshape(1, E)
        vm = pl.BlockSpec(memory_space=pltpu.VMEM)
        out = pl.pallas_call(
            kernel,
            in_specs=[pl.BlockSpec(memory_space=pl.ANY), vm, vm, vm, vm, vm],
            out_specs=pl.BlockSpec(memory_space=pl.ANY),
            out_shape=jax.ShapeDtypeStruct((H, C, W), BF16),
            scratch_shapes=[
                pltpu.VMEM((NP + 1, E // 2, W), U32),
                pltpu.VMEM((NP + 1, C // 2, W), U32),
                pltpu.VMEM((XS * CH + 2, C, W), BF16),
                pltpu.VMEM((E // 2, 128), U32),
                pltpu.VMEM((C // 2, E), U32),
                pltpu.VMEM((C, 128), F32),
                pltpu.VMEM((E, 128), F32),
                pltpu.SemaphoreType.DMA((XS,)),
                pltpu.SemaphoreType.DMA((OS,)),
            ],
            compiler_params=pltpu.CompilerParams(vmem_limit_bytes=vmem_mb << 20),
        )(xt, dw, w1, w2t, gam, bet)
        return jnp.transpose(out.reshape(1, H, C, W), (0, 1, 3, 2))
    return f


pallas_standalone__modern_conv_block_convnext_v2__vision_kernel = build(**{'NBQ':1,'U':4,'QA':(2,3,1),'QB':(4,5,0)})
```

```python
import functools
import math

import jax
import jax.numpy as jnp
import jax.experimental.pallas as pl
import jax.experimental.pallas.tpu as pltpu

F32 = jnp.float32
BF16 = jnp.bfloat16
U32 = jnp.uint32

_C0 = math.sqrt(2.0 / math.pi)
_KAPPA = (_C0 * 0.044715) ** (1.0 / 3.0)
_A = _C0 / _KAPPA
_GS = 2.0 * _KAPPA


def _u(x):
    return pltpu.bitcast(x, U32)


def _b(x):
    return pltpu.bitcast(x, BF16)


def build(NBQ=1, R2=16, LEAD=1, QA=(2, 3, 1), QB=(4, 5, 0), vmem_mb=128, do1=True, do2=True):
    H, W, C, E = 512, 512, 96, 384
    NT = W // 128
    NQ = C // 16
    CH = 16
    NCH = H // CH
    U = CH // 2
    XS = 3
    ZROW = XS * CH
    NP = H // 2
    S2 = XS * CH // R2
    NC2 = H // R2

    def kernel(x_hbm, dw_ref, w1_ref, w2t_ref, gam_ref, bet_ref,
               o_hbm,
               hst, xst, xr, w1t, w2s, b2b, acc, xsem, osem):

        def xcopy(c, slot):
            return pltpu.make_async_copy(
                x_hbm.at[pl.ds(c * CH, CH)], xr.at[pl.ds(slot * CH, CH)], xsem.at[slot])

        def x2copy(c, slot):
            row = ((NCH - 2) % XS) * CH + slot * R2
            row = jnp.where(row >= ZROW, row - ZROW, row)
            return pltpu.make_async_copy(
                x_hbm.at[pl.ds(c * R2, R2)], xr.at[pl.ds(row, R2)], xsem.at[XS + slot])

        def nxt(s, n):
            return jnp.where(s == n - 1, 0, s + 1)

        for c in range(XS):
            xcopy(c, c).start()

        def tiles(v):
            return [v[:, t * 128:(t + 1) * 128] for t in range(NT)]

        def mm1(xp):
            return jnp.dot(_b(w1t[...]), xp, preferred_element_type=F32)

        def padk(xn):
            return jnp.concatenate([xn, jnp.zeros((128 - C, W), xn.dtype)], axis=0)

        def gelu(v):
            z = v * (v * v + _A)
            return v * (jnp.tanh(z) + 1.0)

        lane = jax.lax.broadcasted_iota(jnp.int32, (8, 128), 1)
        m0 = lane == 0
        m127 = lane == 127

        def pass1(dwb, la, lb, clr, ccu, ccf, cbuf, stat, nrm):
            rr = jax.lax.broadcasted_iota(jnp.int32, (C, C), 0)
            cc = jax.lax.broadcasted_iota(jnp.int32, (C, C), 1)
            dv = []
            for a in range(3):
                for b in range(3):
                    row = dw_ref[a, b:b + 1, :].astype(F32)
                    d = jnp.where(rr == cc, jnp.broadcast_to(row, (C, C)), 0.0)
                    col = jnp.sum(d, axis=1, keepdims=True)
                    dv.append(jnp.broadcast_to(col, (C, 128)))
                dwb[a] = dv[a * 3 + 1]
            r16 = jax.lax.broadcasted_iota(jnp.int32, (16, 128), 0)
            c16 = jax.lax.broadcasted_iota(jnp.int32, (16, 128), 1)
            for q in range(NQ):
                ta, tb = [], []
                sf = slice(q * 16, q * 16 + 16)
                for o in range(2):
                    ma = jnp.zeros((16, 128), F32)
                    mb = jnp.zeros((16, 128), F32)
                    for a in range(3):
                        ma = jnp.where(c16 == (a + o) * 16 + r16, dv[a * 3 + 0][sf, :], ma)
                        ma = jnp.where(c16 == (4 + a + o) * 16 + r16, dv[a * 3 + 2][sf, :], ma)
                        mb = jnp.where(c16 == (a + o) * 16 + r16, dv[a * 3 + 1][sf, :], mb)
                    ta.append(ma)
                    tb.append(mb)
                la[q] = _u(jnp.concatenate(ta, axis=0).astype(BF16))
                lb[q] = _u(jnp.concatenate(tb, axis=0).astype(BF16))
            re = jax.lax.broadcasted_iota(jnp.int32, (E, E), 0)
            ce = jax.lax.broadcasted_iota(jnp.int32, (E, E), 1)
            eye = jnp.where(re == ce, 1.0, 0.0).astype(BF16)
            w1f = w1_ref[...].astype(F32)
            w1c = (w1f - jnp.mean(w1f, axis=0, keepdims=True)).astype(BF16)
            w1p = jnp.concatenate([w1c, jnp.zeros((128 - C, E), BF16)], axis=0)
            t = jax.lax.dot_general(eye, w1p, (((1,), (1,)), ((), ())),
                                    preferred_element_type=F32)
            w1t[...] = _u(t.astype(BF16))
            acc[...] = jnp.zeros_like(acc)
            cbuf[1] = jnp.zeros((2, C, W), F32)
            nrm[...] = jnp.zeros_like(nrm)
            xr[ZROW] = jnp.zeros((C, W), BF16)

            sub = jax.lax.broadcasted_iota(jnp.int32, (8, 128), 0)

            def butterfly(vs):
                for d in (1, 2, 4):
                    mk = (sub % (2 * d)) < d
                    vs = [jnp.where(mk, vs[i], vs[i + 1]) + pltpu.roll(jnp.where(mk, vs[i + 1], vs[i]), d, 0)
                          for i in range(0, len(vs), 2)]
                return vs[0]

            def s3(xp, hidx):
                v_all = mm1(xp)
                for e in range(E // 16):
                    g = gelu(v_all[e * 16:(e + 1) * 16, :])
                    g2 = tiles(g * g)
                    acc[e * 16:(e + 1) * 16, :] += (g2[0] + g2[1]) + (g2[2] + g2[3])
                    if hidx is not None:
                        hst[hidx, e * 16:(e + 1) * 16, :] = g.astype(BF16)

            def prep(par, rows, q):
                zero = jnp.zeros((8, 128), U32)
                su = slice(q * 8, q * 8 + 8)
                sf = slice(q * 16, q * 16 + 16)
                for n in range(2):
                    p = _u(xr[rows[n], sf, :])
                    pt = tiles(p)
                    rl = [pltpu.roll(pt[t], 1, 1) for t in range(NT)]
                    rg = [pltpu.roll(pt[t], 127, 1) for t in range(NT)]
                    clr[par, n, 0, su, :] = jnp.concatenate(
                        [jnp.where(m0, rl[t - 1] if t > 0 else zero, rl[t]) for t in range(NT)], axis=1)
                    clr[par, n, 1, su, :] = jnp.concatenate(
                        [jnp.where(m127, rg[t + 1] if t < NT - 1 else zero, rg[t]) for t in range(NT)], axis=1)
                    if q < NBQ:
                        ccu[par, n, su, :] = p
                    else:
                        ccf[par, n, q - NBQ] = _b(p).astype(F32)

            def s2a(par, xrows, qs, fin):
                if fin:
                    s1 = [stat[o, 0] for o in range(2)]
                    s2 = [stat[o, 1] for o in range(2)]
                else:
                    s1 = [None, None]
                    s2 = [None, None]

                def put(o, sf, c):
                    cbuf[par, o, sf, :] = c
                    a = c[0:8] + c[8:16]
                    b = c[0:8] * c[0:8] + c[8:16] * c[8:16]
                    s1[o] = a if s1[o] is None else s1[o] + a
                    s2[o] = b if s2[o] is None else s2[o] + b

                for q in qs:
                    su = slice(q * 8, q * 8 + 8)
                    sf = slice(q * 16, q * 16 + 16)
                    prep(par, xrows, q)
                    rows = [(1 - par, 0), (1 - par, 1), (par, 0), (par, 1)]
                    rhs = _b(jnp.concatenate(
                        [clr[a, n, 0, su, :] for a, n in rows] + [clr[a, n, 1, su, :] for a, n in rows], axis=0))
                    ca = jnp.dot(_b(la[q]), rhs, preferred_element_type=F32)
                    if q < NBQ:
                        cs = [ccu[a, n, su, :] for a, n in rows] + [jnp.zeros((32, W), U32)]
                        rb = _b(jnp.concatenate(cs, axis=0))
                        ca = ca + jnp.dot(_b(lb[q]), rb, preferred_element_type=F32)
                        for o in range(2):
                            put(o, sf, ca[o * 16:(o + 1) * 16, :])
                    else:
                        cf = [ccf[a, n, q - NBQ] for a, n in rows]
                        ws = [jnp.concatenate([dwb[a, sf, :]] * NT, axis=1) for a in range(3)]
                        for o in range(2):
                            put(o, sf, (ca[o * 16:(o + 1) * 16, :] + ws[0] * cf[o]) + (
                                ws[1] * cf[o + 1] + ws[2] * cf[o + 2]))
                if fin:
                    m = butterfly(tiles(s1[0]) + tiles(s1[1])) * (1.0 / C)
                    q2 = butterfly(tiles(s2[0]) + tiles(s2[1])) * (1.0 / C)
                    var = jnp.maximum(q2 - m * m, 0.0)
                    nrm[par] = jax.lax.rsqrt(var + 1e-5) * _KAPPA
                else:
                    for o in range(2):
                        stat[o, 0] = s1[o]
                        stat[o, 1] = s2[o]

            def s2b(par, j, xidx):
                xs = [cbuf[par, j, :, t * 128:(t + 1) * 128] * nrm[par, j * 4 + t:j * 4 + t + 1, :]
                      for t in range(NT)]
                xn = jnp.concatenate(xs, axis=1)
                if xidx is not None:
                    xst[xidx] = xn.astype(BF16)
                return padk(xn).astype(BF16)

            def body1(kk, slot):
                ns = nxt(slot, XS)
                cur = slot * CH
                last = kk == NCH - 1

                def xrow(r):
                    return cur + r if r < CH else jnp.where(last, ZROW, ns * CH + (r - CH))

                for u in range(U):
                    par = u % 2
                    idx = kk * U + u - 1 if u > 0 else jnp.maximum(kk * U - 1, 0)
                    s3(s2b(1 - par, 0, idx), None)
                    s2a(par, (xrow(2 * u + 1), xrow(2 * u + 2)), QB, True)
                    s3(s2b(1 - par, 1, None), idx)
                    s2a(1 - par, (xrow(2 * u + 3), xrow(2 * u + 4)), QA, False)

                @pl.when(kk + 2 < NCH)
                def _():
                    xcopy(kk + 2, nxt(ns, XS)).wait()

                @pl.when(kk + XS < NCH)
                def _():
                    xcopy(kk + XS, slot).start()

                @pl.when(kk == NCH - 2)
                def _():
                    for c in range(CH // R2):
                        x2copy(c, c).start()
                return ns

            xcopy(0, 0).wait()
            xcopy(1, 1).wait()
            for q in range(NQ):
                prep(1, (ZROW, 0), q)
            s2a(0, (1, 2), QA, False)
            if do1:
                jax.lax.fori_loop(0, NCH, body1, 0)
                for c in range(CH // R2, S2 - LEAD):
                    x2copy(c, c).start()
                s3(s2b(1, 0, NP - 1), None)
                s3(s2b(1, 1, None), NP - 1)
            else:
                for c in range(2, XS):
                    xcopy(c, c).wait()
                for c in range(S2 - LEAD):
                    x2copy(c, c).start()

        pl.run_scoped(
            pass1,
            pltpu.VMEM((3, C, 128), F32),
            pltpu.VMEM((NQ, 16, 128), U32),
            pltpu.VMEM((NQ, 16, 128), U32),
            pltpu.VMEM((2, 2, 2, C // 2, W), U32),
            pltpu.VMEM((2, 2, max(NBQ, 1) * 8, W), U32),
            pltpu.VMEM((2, 2, max(NQ - NBQ, 1), 16, W), F32),
            pltpu.VMEM((2, 2, C, W), F32),
            pltpu.VMEM((2, 2, 8, W), F32),
            pltpu.VMEM((2, 8, 128), F32),
        )

        a = jnp.transpose(acc[...])
        ssq = jnp.sum(a, axis=0, keepdims=True) * (1.0 / (_GS * _GS))
        gx = jnp.sqrt(ssq + 1e-6)
        nx = gx / (jnp.mean(gx, axis=1, keepdims=True) + 1e-6)
        s = (gam_ref[...].astype(F32) * nx + 1.0) * (1.0 / _GS)
        w2f = w2t_ref[...].astype(F32)
        w2s[...] = _u((w2f * s).astype(BF16))
        b = jnp.sum(w2f * bet_ref[...].astype(F32), axis=1, keepdims=True)
        b2b[...] = jnp.broadcast_to(b, (C, 128))

        def pass2(gt):
            def ring_row(slot):
                row = ((NCH - 2) % XS) * CH + slot * R2
                return jnp.where(row >= ZROW, row - ZROW, row)

            def ocopy(c, slot):
                return pltpu.make_async_copy(
                    xr.at[pl.ds(ring_row(slot), R2)], o_hbm.at[pl.ds(c * R2, R2)], osem.at[slot])

            def t1(m, gslot):
                v_all = mm1(padk(xst[m]))
                for e in range(E // 16):
                    g = gelu(v_all[e * 16:(e + 1) * 16, :])
                    gt[gslot, e * 16:(e + 1) * 16, :] = g.astype(BF16)

            def t2(g, row):
                y = jnp.dot(_b(w2s[...]), g, preferred_element_type=F32)
                bb = jnp.concatenate([b2b[...]] * NT, axis=1)
                xr[row] = (y + (bb + xr[row].astype(F32))).astype(BF16)

            def body2(c, carry):
                slot, fslot = carry
                xb = ring_row(slot)
                for u in range(R2 // 2):
                    m = c * (R2 // 2) + u
                    t2(gt[u % 2], xb + 2 * u)
                    t1(jnp.minimum(m + 1, NP - 1), (u + 1) % 2)
                    t2(hst[m], xb + 2 * u + 1)
                ocopy(c, slot).start()

                @pl.when(c >= LEAD)
                def _():
                    ocopy(c - LEAD, fslot).wait()

                @pl.when(c + S2 - LEAD < NC2)
                def _():
                    x2copy(c + S2 - LEAD, fslot).start()

                ns = nxt(slot, S2)

                @pl.when(c + 1 < NC2)
                def _():
                    x2copy(c + 1, ns).wait()
                return ns, nxt(fslot, S2)

            x2copy(0, 0).wait()
            if do2:
                t1(0, 0)
                jax.lax.fori_loop(0, NC2, body2, (0, S2 - LEAD))
                for c in range(NC2 - LEAD, NC2):
                    ocopy(c, c % S2).wait()
            else:
                for c in range(1, S2 - LEAD):
                    x2copy(c, c).wait()

        pl.run_scoped(pass2, pltpu.VMEM((2, E, W), BF16))

    @jax.jit
    def f(x, dw, w1, w2, grn_gamma, grn_beta):
        xt = jnp.transpose(x, (0, 1, 3, 2)).reshape(H, C, W)
        w2t = jnp.transpose(w2)
        gam = grn_gamma.reshape(1, E)
        bet = grn_beta.reshape(1, E)
        vm = pl.BlockSpec(memory_space=pltpu.VMEM)
        out = pl.pallas_call(
            kernel,
            in_specs=[pl.BlockSpec(memory_space=pl.ANY), vm, vm, vm, vm, vm],
            out_specs=pl.BlockSpec(memory_space=pl.ANY),
            out_shape=jax.ShapeDtypeStruct((H, C, W), BF16),
            scratch_shapes=[
                pltpu.VMEM((NP, E, W), BF16),
                pltpu.VMEM((NP, C, W), BF16),
                pltpu.VMEM((XS * CH + 1, C, W), BF16),
                pltpu.VMEM((E // 2, 128), U32),
                pltpu.VMEM((C // 2, E), U32),
                pltpu.VMEM((C, 128), F32),
                pltpu.VMEM((E, 128), F32),
                pltpu.SemaphoreType.DMA((XS + S2,)),
                pltpu.SemaphoreType.DMA((S2,)),
            ],
            compiler_params=pltpu.CompilerParams(vmem_limit_bytes=vmem_mb << 20),
        )(xt, dw, w1, w2t, gam, bet)
        return jnp.transpose(out.reshape(1, H, C, W), (0, 1, 3, 2))
    return f


pallas_standalone__modern_conv_block_convnext_v2__vision_kernel = build(**{})
```

```python
import functools
import math

import jax
import jax.numpy as jnp
import jax.experimental.pallas as pl
import jax.experimental.pallas.tpu as pltpu

F32 = jnp.float32
BF16 = jnp.bfloat16
U32 = jnp.uint32

_C0 = math.sqrt(2.0 / math.pi)
_KAPPA = (_C0 * 0.044715) ** (1.0 / 3.0)
_A = _C0 / _KAPPA
_GS = 2.0 * _KAPPA


def _u(x):
    return pltpu.bitcast(x, U32)


def _b(x):
    return pltpu.bitcast(x, BF16)


def build(NBQ=1, XS=5, OS=3, NR=7, NF=0, SPL=6, ANCH=True, PA=320, REL=1, QA=(2, 3, 1), QB=(4, 5, 0),
          vmem_mb=128, do1=True, do2=True):
    H, W, C, E = 512, 512, 96, 384
    NT = W // 128
    NQ = C // 16
    CH = 16
    NCH = H // CH
    U = CH // 2
    NP = H // 2
    REC = list(range(1, NR + 1))
    STO = [r for r in range(CH) if r not in REC]
    NS = len(STO)
    ZROW = XS * CH
    CROWS = NBQ * 8 + (NQ - NBQ) * 16

    def kernel(x_hbm, dw_ref, w1_ref, w2t_ref, gam_ref, bet_ref,
               o_hbm,
               hst, rst, xr, dwb, w1t, w2s, b2b, acc, zs, xsem, osem):

        def xcopy(c, slot):
            return pltpu.make_async_copy(
                x_hbm.at[pl.ds(c * CH, CH)], xr.at[pl.ds(slot * CH, CH)], xsem.at[slot])

        def nxt(s, n):
            return jnp.where(s == n - 1, 0, s + 1)

        def xpart(lo, hi, sem):
            return pltpu.make_async_copy(x_hbm.at[pl.ds(lo, hi - lo)], xr.at[pl.ds(lo, hi - lo)], xsem.at[sem])

        xpart(0, CH + 3, 0).start()
        zs[0] = 0

        def tiles(v):
            return [v[:, t * 128:(t + 1) * 128] for t in range(NT)]

        def mm1(xp, e0=0, e1=E):
            return jnp.dot(_b(w1t[e0 // 2:e1 // 2, :]), xp, preferred_element_type=F32)

        def padk(xn):
            return jnp.concatenate([xn, jnp.zeros((128 - C, W), xn.dtype)], axis=0)

        def gelu(v):
            z = v * (v * v + _A)
            return v * (jnp.tanh(z) + 1.0)

        lane = jax.lax.broadcasted_iota(jnp.int32, (8, 128), 1)
        m0 = lane == 0
        m127 = lane == 127

        def pass1(la, lb, cw, cbuf, stat, nrm):
            rr = jax.lax.broadcasted_iota(jnp.int32, (C, C), 0)
            cc = jax.lax.broadcasted_iota(jnp.int32, (C, C), 1)
            for a in range(3):
                for b in range(3):
                    row = dw_ref[a, b:b + 1, :].astype(F32)
                    d = jnp.where(rr == cc, jnp.broadcast_to(row, (C, C)), 0.0)
                    col = jnp.sum(d, axis=1, keepdims=True)
                    dwb[a * 3 + b] = jnp.broadcast_to(col, (C, 128))
            r16 = jax.lax.broadcasted_iota(jnp.int32, (16, 128), 0)
            c16 = jax.lax.broadcasted_iota(jnp.int32, (16, 128), 1)
            for q in range(NQ):
                ta, tb = [], []
                sf = slice(q * 16, q * 16 + 16)
                for o in range(2):
                    ma = jnp.zeros((16, 128), F32)
                    mb = jnp.zeros((16, 128), F32)
                    for a in range(3):
                        ma = jnp.where(c16 == (a + o) * 16 + r16, dwb[a * 3 + 0, sf, :], ma)
                        ma = jnp.where(c16 == (4 + a + o) * 16 + r16, dwb[a * 3 + 2, sf, :], ma)
                        mb = jnp.where(c16 == (a + o) * 16 + r16, dwb[a * 3 + 1, sf, :], mb)
                    ta.append(ma)
                    tb.append(mb)
                la[q] = _u(jnp.concatenate(ta, axis=0).astype(BF16))
                lb[q] = _u(jnp.concatenate(tb, axis=0).astype(BF16))
            re = jax.lax.broadcasted_iota(jnp.int32, (E, E), 0)
            ce = jax.lax.broadcasted_iota(jnp.int32, (E, E), 1)
            eye = jnp.where(re == ce, 1.0, 0.0).astype(BF16)
            w1f = w1_ref[...].astype(F32)
            w1c = (w1f - jnp.mean(w1f, axis=0, keepdims=True)).astype(BF16)
            w1p = jnp.concatenate([w1c, jnp.zeros((128 - C, E), BF16)], axis=0)
            t = jax.lax.dot_general(eye, w1p, (((1,), (1,)), ((), ())),
                                    preferred_element_type=F32)
            w1t[...] = _u(t.astype(BF16))
            acc[...] = jnp.zeros_like(acc)
            cbuf[1] = jnp.zeros((2, C, W), F32)
            cw[0:16, :] = jnp.zeros((16, W), U32)
            nrm[...] = jnp.zeros_like(nrm)
            xr[ZROW] = jnp.zeros((C, W), BF16)

            sub = jax.lax.broadcasted_iota(jnp.int32, (8, 128), 0)

            def butterfly(vs):
                for d in (1, 2, 4):
                    mk = (sub % (2 * d)) < d
                    vs = [jnp.where(mk, vs[i], vs[i + 1]) + pltpu.roll(jnp.where(mk, vs[i + 1], vs[i]), d, 0)
                          for i in range(0, len(vs), 2)]
                return vs[0]

            def rlr(par, n, lr, q):
                o = ((par * 2 + n) * 2 + lr) * (C // 2) + q * 8
                return slice(o, o + 8)

            def rc(par, n, q):
                o = 4 * C + (par * 2 + n) * CROWS
                if q < NBQ:
                    return slice(o + q * 8, o + q * 8 + 8)
                o += NBQ * 8 + (q - NBQ) * 16
                return slice(o, o + 16)

            def s3p(xp, hidx, e0, e1):
                v_all = mm1(xp, e0, e1)
                for e in range(e0 // 16, e1 // 16):
                    g = gelu(v_all[e * 16 - e0:(e + 1) * 16 - e0, :])
                    g2 = tiles(g * g)
                    acc[e * 16:(e + 1) * 16, :] += (g2[0] + g2[1]) + (g2[2] + g2[3])
                    if hidx is not None:
                        hst[hidx, e * 16:(e + 1) * 16, :] = g.astype(BF16)

            def s3(xn, hidx, z=None):
                if z is None or not PA:
                    s3p(padk(xn).astype(BF16), hidx, 0, E)
                    return
                s3p(padk(xn).astype(BF16), hidx, 0, PA)
                pad = _b(cw[pl.ds(pl.multiple_of(z, 8), 16), :]).astype(F32)
                s3p(jnp.concatenate([xn, pad], axis=0).astype(BF16), hidx, PA, E)

            def prep(par, rows, q):
                zero = jnp.zeros((8, 128), U32)
                sf = slice(q * 16, q * 16 + 16)
                for n in range(2):
                    p = _u(xr[rows[n], sf, :])
                    pt = tiles(p)
                    rl = [pltpu.roll(pt[t], 1, 1) for t in range(NT)]
                    rg = [pltpu.roll(pt[t], 127, 1) for t in range(NT)]
                    cw[rlr(par, n, 0, q), :] = jnp.concatenate(
                        [jnp.where(m0, rl[t - 1] if t > 0 else zero, rl[t]) for t in range(NT)], axis=1)
                    cw[rlr(par, n, 1, q), :] = jnp.concatenate(
                        [jnp.where(m127, rg[t + 1] if t < NT - 1 else zero, rg[t]) for t in range(NT)], axis=1)
                    if q < NBQ:
                        cw[rc(par, n, q), :] = p
                    else:
                        cw[rc(par, n, q), :] = _u(_b(p).astype(F32))

            def s2a(par, qs, kidx, arow=None):
                fin = kidx is not None
                if fin:
                    s1 = [stat[o, 0] for o in range(2)]
                    s2 = [stat[o, 1] for o in range(2)]
                else:
                    s1 = [None, None]
                    s2 = [None, None]

                def put(o, sf, c):
                    cbuf[par, o, sf, :] = c
                    a = c[0:8] + c[8:16]
                    b = c[0:8] * c[0:8] + c[8:16] * c[8:16]
                    s1[o] = a if s1[o] is None else s1[o] + a
                    s2[o] = b if s2[o] is None else s2[o] + b

                for q in qs:
                    sf = slice(q * 16, q * 16 + 16)
                    rows = [(1 - par, 0), (1 - par, 1), (par, 0), (par, 1)]
                    rhs = [cw[rlr(a, n, 0, q), :] for a, n in rows] + [cw[rlr(a, n, 1, q), :] for a, n in rows]
                    lhs = _b(la[q])
                    if q < NBQ:
                        rhs += [cw[rc(a, n, q), :] for a, n in rows] + [jnp.zeros((32, W), U32)]
                        lhs = jnp.concatenate([lhs, _b(lb[q])], axis=1)
                    ca = jnp.dot(lhs, _b(jnp.concatenate(rhs, axis=0)), preferred_element_type=F32)
                    if arow is not None and q == qs[0]:
                        xr[arow, 0:8, 0:128] = ca[0:8, 0:128].astype(BF16)
                    if q < NBQ:
                        for o in range(2):
                            put(o, sf, ca[o * 16:(o + 1) * 16, :])
                    else:
                        cf = [pltpu.bitcast(cw[rc(a, n, q), :], F32) for a, n in rows]
                        ws = [jnp.concatenate([dwb[a * 3 + 1, sf, :]] * NT, axis=1) for a in range(3)]
                        for o in range(2):
                            put(o, sf, (ca[o * 16:(o + 1) * 16, :] + ws[0] * cf[o]) + (
                                ws[1] * cf[o + 1] + ws[2] * cf[o + 2]))
                if fin:
                    m = butterfly(tiles(s1[0]) + tiles(s1[1])) * (1.0 / C)
                    q2 = butterfly(tiles(s2[0]) + tiles(s2[1])) * (1.0 / C)
                    var = jnp.maximum(q2 - m * m, 0.0)
                    rs = jax.lax.rsqrt(var + 1e-5) * _KAPPA
                    nrm[par] = rs
                    rst[kidx] = rs
                else:
                    for o in range(2):
                        stat[o, 0] = s1[o]
                        stat[o, 1] = s2[o]

            def s2b(par, j):
                xs = [cbuf[par, j, :, t * 128:(t + 1) * 128] * nrm[par, j * 4 + t:j * 4 + t + 1, :]
                      for t in range(NT)]
                return jnp.concatenate(xs, axis=1)

            def hslot(chunk, r):
                return None if r in REC else chunk * NS + STO.index(r)

            def body1(kk, slot):
                ns = nxt(slot, XS)
                cur = slot * CH
                last = kk == NCH - 1
                z = zs[0]
                arow = cur + z if REL else None

                def xrow(r):
                    return cur + r if r < CH else jnp.where(last, ZROW, ns * CH + (r - CH))

                def hs(r):
                    return hslot(kk, r) if r >= 0 else hslot(jnp.maximum(kk - 1, 0), r + CH)

                for u in range(U):
                    par = u % 2
                    for q in QB:
                        prep(par, (xrow(2 * u + 1), xrow(2 * u + 2)), q)
                    s3(s2b(1 - par, 0), hs(2 * u - 2), z)
                    s2a(par, QB, kk * U + u, arow)
                    for q in QA:
                        prep(1 - par, (xrow(2 * u + 3), xrow(2 * u + 4)), q)
                    s3(s2b(1 - par, 1), hs(2 * u - 1), z)
                    s2a(1 - par, QA, None, arow)

                @pl.when(kk == 0)
                def _():
                    xpart(CH + 3, 2 * CH, 1).wait()

                @pl.when(kk + 2 < NCH)
                def _():
                    xcopy(kk + 2, nxt(ns, XS)).wait()

                cn = kk + XS
                xcopy(jnp.where(cn < NCH, cn, cn - NCH), slot).start()
                return ns

            xpart(0, CH + 3, 0).wait()
            xpart(CH + 3, 2 * CH, 1).start()
            for c in range(2, XS):
                xcopy(c, c).start()
            for q in range(NQ):
                prep(1, (ZROW, 0), q)
            for q in QA:
                prep(0, (1, 2), q)
            s2a(0, QA, None)
            if do1:
                jax.lax.fori_loop(0, NCH, body1, 0)
                for j in range(2):
                    s3(s2b(1, j), hslot(NCH - 1, CH - 2 + j))
            else:
                xpart(CH + 3, 2 * CH, 1).wait()
                for c in range(2, XS):
                    xcopy(c, c).wait()
                for c in range(XS):
                    xcopy(c, (NCH + c) % XS).start()

        pl.run_scoped(
            pass1,
            pltpu.VMEM((NQ, 16, 128), U32),
            pltpu.VMEM((NQ, 16, 128), U32),
            pltpu.VMEM((4 * C + 4 * CROWS, W), U32),
            pltpu.VMEM((2, 2, C, W), F32),
            pltpu.VMEM((2, 2, 8, W), F32),
            pltpu.VMEM((2, 8, 128), F32),
        )

        a = jnp.transpose(acc[...])
        ssq = jnp.sum(a, axis=0, keepdims=True) * (1.0 / (_GS * _GS))
        gx = jnp.sqrt(ssq + 1e-6)
        nx = gx / (jnp.mean(gx, axis=1, keepdims=True) + 1e-6)
        s = (gam_ref[...].astype(F32).reshape(1, E) * nx + 1.0) * (1.0 / _GS)
        w2f = w2t_ref[...].astype(F32)
        w2s[...] = _u((w2f * s).astype(BF16))
        b = jnp.sum(w2f * bet_ref[...].astype(F32).reshape(1, E), axis=1, keepdims=True)
        b2b[...] = jnp.broadcast_to(b, (C, 128))

        def pass2(orr, gt, xn2):
            def ocopy(c, slot):
                return pltpu.make_async_copy(
                    orr.at[slot], o_hbm.at[pl.ds(c * CH, CH)], osem.at[slot])

            def t0(c, xb, i, cg0, cg1):
                r = REC[i]
                rs = [rst[c * U + r // 2, (r % 2) * 4 + t:(r % 2) * 4 + t + 1, :] for t in range(NT)]
                for cg in range(cg0, cg1):
                    sl = slice(cg * 8, cg * 8 + 8)
                    xs = [tiles(xr[xb + r - 1 + a, sl, :].astype(F32)) for a in range(3)]
                    cs = []
                    for b in range(3):
                        ws = [dwb[a * 3 + b, sl, :] for a in range(3)]
                        cs.append([ws[0] * xs[0][t] + ws[1] * xs[1][t] + ws[2] * xs[2][t] for t in range(NT)])
                    rl = [pltpu.roll(cs[0][t], 1, 1) for t in range(NT)]
                    rg = [pltpu.roll(cs[2][t], 127, 1) for t in range(NT)]
                    row = []
                    for t in range(NT):
                        left = jnp.where(m0, rl[t - 1] if t > 0 else 0.0, rl[t])
                        right = jnp.where(m127, rg[t + 1] if t < NT - 1 else 0.0, rg[t])
                        row.append((cs[1][t] + (left + right)) * rs[t])
                    xn2[i, sl, :] = jnp.concatenate(row, axis=1).astype(BF16)

            def anchor(v, z):
                dwb[9 + z, 0:8, :] = v
                xr[ZROW + z, 0:8, 0:128] = v.astype(BF16)

            def t1(i, z):
                v_all = mm1(padk(xn2[i]))
                an = None
                for e in range(E // 16):
                    g = gelu(v_all[e * 16:(e + 1) * 16, :])
                    gt[i % 2, e * 16:(e + 1) * 16, :] = g.astype(BF16)
                    an = g[8:16, W - 128:W] if an is None else an + g[8:16, W - 128:W]
                if ANCH:
                    anchor(an, z)

            def t2(g, xb, oslot, row, z=None):
                y = jnp.dot(_b(w2s[...]), g, preferred_element_type=F32)
                bb = jnp.concatenate([b2b[...]] * NT, axis=1)
                orr[oslot, row] = (y + (bb + xr[xb + row].astype(F32))).astype(BF16)
                if z is not None:
                    an = y[0:8, W - 128:W]
                    for cg in range(1, C // 8):
                        an = an + y[cg * 8:(cg + 1) * 8, W - 128:W]
                    anchor(an, z)

            NCG = C // 8

            def body2(c, carry):
                xslot, oslot = carry
                xb = xslot * CH
                z = zs[0]
                c2 = jnp.minimum(c + 1, NCH - 1)
                xb2 = jnp.where(c + 1 < NCH, nxt(xslot, XS), xslot) * CH

                def t2s(i, zz=None):
                    t2(hst[c * NS + i], xb, oslot, STO[i], zz)

                def t0n(i, cg0, cg1):
                    if i < NR:
                        t0(c, xb, i, cg0, cg1)
                    else:
                        t0(c2, xb2, i - NR, cg0, cg1)

                si = 0
                for i in range(NF):
                    t2s(si)
                    si += 1
                for i in range(NR):
                    t1(i, z)
                    t0n(i + 2, 0, SPL)
                    zz = z if SPL < NCG else None
                    if i > 0:
                        t2(gt[(i - 1) % 2], xb, oslot, REC[i - 1], zz)
                    else:
                        t2s(si, zz)
                        si += 1
                    t0n(i + 2, SPL, NCG)
                    t2s(si)
                    si += 1
                t2(gt[(NR - 1) % 2], xb, oslot, REC[NR - 1])
                while si < NS:
                    t2s(si)
                    si += 1
                ocopy(c, oslot).start()
                nx_ = nxt(xslot, XS)
                no_ = nxt(oslot, OS)

                @pl.when(c + XS < NCH)
                def _():
                    xcopy(c + XS, xslot).start()

                @pl.when(c + 2 < NCH)
                def _():
                    xcopy(c + 2, nxt(nx_, XS)).wait()

                @pl.when(c + 1 >= OS)
                def _():
                    ocopy(c + 1 - OS, no_).wait()
                return nx_, no_

            s0 = NCH % XS
            xcopy(0, s0).wait()
            if do2:
                xcopy(1, (s0 + 1) % XS).wait()
                for i in range(2):
                    t0(0, s0 * CH, i, 0, NCG)
                jax.lax.fori_loop(0, NCH, body2, (s0, 0))
                for c in range(NCH + 1 - OS, NCH):
                    ocopy(c, c % OS).wait()
            else:
                for c in range(1, XS):
                    xcopy(c, (s0 + c) % XS).wait()

        pl.run_scoped(pass2, pltpu.VMEM((OS, CH, C, W), BF16), pltpu.VMEM((2, E, W), BF16),
                      pltpu.VMEM((NR, C, W), BF16))

    @jax.jit
    def f(x, dw, w1, w2, grn_gamma, grn_beta):
        xt = jnp.transpose(x, (0, 1, 3, 2)).reshape(H, C, W)
        w2t = jnp.transpose(w2)
        vm = pl.BlockSpec(memory_space=pltpu.VMEM)
        out = pl.pallas_call(
            kernel,
            in_specs=[pl.BlockSpec(memory_space=pl.ANY), vm, vm, vm, vm, vm],
            out_specs=pl.BlockSpec(memory_space=pl.ANY),
            out_shape=jax.ShapeDtypeStruct((H, C, W), BF16),
            scratch_shapes=[
                pltpu.VMEM((NCH * NS, E, W), BF16),
                pltpu.VMEM((NP, 8, 128), F32),
                pltpu.VMEM((XS * CH + 1, C, W), BF16),
                pltpu.VMEM((10, C, 128), F32),
                pltpu.VMEM((E // 2, 128), U32),
                pltpu.VMEM((C // 2, E), U32),
                pltpu.VMEM((C, 128), F32),
                pltpu.VMEM((E, 128), F32),
                pltpu.SMEM((1,), jnp.int32),
                pltpu.SemaphoreType.DMA((XS,)),
                pltpu.SemaphoreType.DMA((OS,)),
            ],
            compiler_params=pltpu.CompilerParams(vmem_limit_bytes=vmem_mb << 20),
        )(xt, dw, w1, w2t, grn_gamma, grn_beta)
        return jnp.transpose(out.reshape(1, H, C, W), (0, 1, 3, 2))
    return f


pallas_standalone__modern_conv_block_convnext_v2__vision_kernel = build(**{})
```

```python
import functools
import math

import jax
import jax.numpy as jnp
import jax.experimental.pallas as pl
import jax.experimental.pallas.tpu as pltpu

F32 = jnp.float32
BF16 = jnp.bfloat16
U32 = jnp.uint32

_C0 = math.sqrt(2.0 / math.pi)
_KAPPA = (_C0 * 0.044715) ** (1.0 / 3.0)
_A = _C0 / _KAPPA
_GS = 2.0 * _KAPPA


def _u(x):
    return pltpu.bitcast(x, U32)


def _b(x):
    return pltpu.bitcast(x, BF16)


def build(NBQ=2, XS=4, OS=2, NR=7, NF=0, PARTS=((6, 'a3'),), ANCH=True, UPAD=False, PA=352, REL=1, RQ=1, RO=0, QA=(2, 3, 0), QB=(4, 5, 1),
          vmem_mb=128, do1=True, do2=True):
    H, W, C, E = 512, 512, 96, 384
    NT = W // 128
    NQ = C // 16
    CH = 16
    NCH = H // CH
    U = CH // 2
    NP = H // 2
    REC = list(range(1, NR + 1))
    STO = [r for r in range(CH) if r not in REC]
    NS = len(STO)
    ZROW = XS * CH
    CROWS = NBQ * 8 + (NQ - NBQ) * 16

    def kernel(x_hbm, dw_hbm, w1_hbm, w2t_hbm, gam_hbm, bet_hbm,
               o_hbm,
               hst, rst, xr, dwb, w1t, w2s, b2b, acc, xn2, wk,
               dw_ref, w1_ref, w2t_ref, gam_ref, bet_ref, zs, xsem, osem, wsem):

        def xcopy(c, slot):
            return pltpu.make_async_copy(
                x_hbm.at[pl.ds(c * CH, CH)], xr.at[pl.ds(slot * CH, CH)], xsem.at[slot])

        def nxt(s, n):
            return jnp.where(s == n - 1, 0, s + 1)

        def xpart(lo, hi, sem):
            return pltpu.make_async_copy(x_hbm.at[pl.ds(lo, hi - lo)], xr.at[pl.ds(lo, hi - lo)], xsem.at[sem])

        wcp = [pltpu.make_async_copy(src, dst, wsem.at[i]) for i, (src, dst) in enumerate(
            [(dw_hbm, dw_ref), (w1_hbm, w1_ref), (w2t_hbm, w2t_ref), (gam_hbm, gam_ref), (bet_hbm, bet_ref)])]
        wcp[0].start()
        wcp[1].start()
        xpart(0, 3, 1).start()
        xpart(3, CH + 3, 0).start()
        for cp in wcp[2:]:
            cp.start()
        zs[0] = 0
        wcp[0].wait()
        wcp[1].wait()

        def tiles(v):
            return [v[:, t * 128:(t + 1) * 128] for t in range(NT)]

        def mm1(xp, e0=0, e1=E):
            return jnp.dot(_b(w1t[e0 // 2:e1 // 2, :]), xp, preferred_element_type=F32)

        def padk(xn):
            return jnp.concatenate([xn, jnp.zeros((128 - C, W), xn.dtype)], axis=0)

        def gelu(v):
            z = v * (v * v + _A)
            return v * (jnp.tanh(z) + 1.0)

        lane = jax.lax.broadcasted_iota(jnp.int32, (8, 128), 1)
        m0 = lane == 0
        m127 = lane == 127

        NCG = C // 8
        NX = NR + 2

        def unp(xb, r):
            wk[r * C:(r + 1) * C, :] = xr[xb + r].astype(F32)

        def t0(c, xb, i, cg0, cg1):
            r = REC[i]
            rs = [rst[c * U + r // 2, (r % 2) * 4 + t:(r % 2) * 4 + t + 1, :] for t in range(NT)]
            for cg in range(cg0, cg1):
                sl = slice(cg * 8, cg * 8 + 8)
                xs = [tiles(wk[(r - 1 + a) * C + cg * 8:(r - 1 + a) * C + cg * 8 + 8, :]) for a in range(3)]
                cs = []
                for b in range(3):
                    ws = [dwb[a * 3 + b, sl, :] for a in range(3)]
                    cs.append([ws[0] * xs[0][t] + ws[1] * xs[1][t] + ws[2] * xs[2][t] for t in range(NT)])
                rl = [pltpu.roll(cs[0][t], 1, 1) for t in range(NT)]
                rg = [pltpu.roll(cs[2][t], 127, 1) for t in range(NT)]
                row = []
                for t in range(NT):
                    left = jnp.where(m0, rl[t - 1] if t > 0 else 0.0, rl[t])
                    right = jnp.where(m127, rg[t + 1] if t < NT - 1 else 0.0, rg[t])
                    row.append((cs[1][t] + (left + right)) * rs[t])
                xn2[i, sl, :] = jnp.concatenate(row, axis=1).astype(BF16)

        def pass1(la, lb, cw, cbuf, stat, nrm):
            rr = jax.lax.broadcasted_iota(jnp.int32, (C, C), 0)
            cc = jax.lax.broadcasted_iota(jnp.int32, (C, C), 1)
            for a in range(3):
                for b in range(3):
                    row = dw_ref[a, b:b + 1, :].astype(F32)
                    d = jnp.where(rr == cc, jnp.broadcast_to(row, (C, C)), 0.0)
                    col = jnp.sum(d, axis=1, keepdims=True)
                    dwb[a * 3 + b] = jnp.broadcast_to(col, (C, 128))
            r16 = jax.lax.broadcasted_iota(jnp.int32, (16, 128), 0)
            c16 = jax.lax.broadcasted_iota(jnp.int32, (16, 128), 1)
            for q in range(NQ):
                ta, tb = [], []
                sf = slice(q * 16, q * 16 + 16)
                for o in range(2):
                    ma = jnp.zeros((16, 128), F32)
                    mb = jnp.zeros((16, 128), F32)
                    for a in range(3):
                        ma = jnp.where(c16 == (a + o) * 16 + r16, dwb[a * 3 + 0, sf, :], ma)
                        ma = jnp.where(c16 == (4 + a + o) * 16 + r16, dwb[a * 3 + 2, sf, :], ma)
                        mb = jnp.where(c16 == (a + o) * 16 + r16, dwb[a * 3 + 1, sf, :], mb)
                    ta.append(ma)
                    tb.append(mb)
                la[q] = _u(jnp.concatenate(ta, axis=0).astype(BF16))
                lb[q] = _u(jnp.concatenate(tb, axis=0).astype(BF16))
            re = jax.lax.broadcasted_iota(jnp.int32, (E, E), 0)
            ce = jax.lax.broadcasted_iota(jnp.int32, (E, E), 1)
            eye = jnp.where(re == ce, 1.0, 0.0).astype(BF16)
            w1f = w1_ref[...].astype(F32)
            w1c = (w1f - jnp.mean(w1f, axis=0, keepdims=True)).astype(BF16)
            w1p = jnp.concatenate([w1c, jnp.zeros((128 - C, E), BF16)], axis=0)
            t = jax.lax.dot_general(eye, w1p, (((1,), (1,)), ((), ())),
                                    preferred_element_type=F32)
            w1t[...] = _u(t.astype(BF16))
            acc[...] = jnp.zeros_like(acc)
            cbuf[1] = jnp.zeros((2, C, W), F32)
            cw[0:16, :] = jnp.zeros((16, W), U32)
            nrm[...] = jnp.zeros_like(nrm)
            xr[ZROW] = jnp.zeros((C, W), BF16)

            sub = jax.lax.broadcasted_iota(jnp.int32, (8, 128), 0)

            def butterfly(vs):
                for d in (1, 2, 4):
                    mk = (sub % (2 * d)) < d
                    vs = [jnp.where(mk, vs[i], vs[i + 1]) + pltpu.roll(jnp.where(mk, vs[i + 1], vs[i]), d, 0)
                          for i in range(0, len(vs), 2)]
                return vs[0]

            def rlr(par, n, lr, q):
                o = ((par * 2 + n) * 2 + lr) * (C // 2) + q * 8
                return slice(o, o + 8)

            def rc(par, n, q):
                o = 4 * C + (par * 2 + n) * CROWS
                if q < NBQ:
                    return slice(o + q * 8, o + q * 8 + 8)
                o += NBQ * 8 + (q - NBQ) * 16
                return slice(o, o + 16)

            def s3p(xp, hidx, e0, e1):
                v_all = mm1(xp, e0, e1)
                for e in range(e0 // 16, e1 // 16):
                    g = gelu(v_all[e * 16 - e0:(e + 1) * 16 - e0, :])
                    g2 = tiles(g * g)
                    acc[e * 16:(e + 1) * 16, :] += (g2[0] + g2[1]) + (g2[2] + g2[3])
                    if hidx is not None:
                        hst[hidx, e * 16:(e + 1) * 16, :] = g.astype(BF16)

            def s3(xn, hidx, z=None):
                if z is None or not PA:
                    s3p(padk(xn).astype(BF16), hidx, 0, E)
                    return
                s3p(padk(xn).astype(BF16), hidx, 0, PA)
                pad = _b(cw[pl.ds(pl.multiple_of(z, 8), 16), :]).astype(F32)
                s3p(jnp.concatenate([xn, pad], axis=0).astype(BF16), hidx, PA, E)

            def prep(par, rows, q):
                zero = jnp.zeros((8, 128), U32)
                sf = slice(q * 16, q * 16 + 16)
                for n in range(2):
                    p = _u(xr[rows[n], sf, :])
                    pt = tiles(p)
                    rl = [pltpu.roll(pt[t], 1, 1) for t in range(NT)]
                    rg = [pltpu.roll(pt[t], 127, 1) for t in range(NT)]
                    cw[rlr(par, n, 0, q), :] = jnp.concatenate(
                        [jnp.where(m0, rl[t - 1] if t > 0 else zero, rl[t]) for t in range(NT)], axis=1)
                    cw[rlr(par, n, 1, q), :] = jnp.concatenate(
                        [jnp.where(m127, rg[t + 1] if t < NT - 1 else zero, rg[t]) for t in range(NT)], axis=1)
                    if q < NBQ:
                        cw[rc(par, n, q), :] = p
                    else:
                        cw[rc(par, n, q), :] = _u(_b(p).astype(F32))

            def s2a(par, qs, kidx, arow=None):
                fin = kidx is not None
                if fin:
                    s1 = [stat[o, 0] for o in range(2)]
                    s2 = [stat[o, 1] for o in range(2)]
                else:
                    s1 = [None, None]
                    s2 = [None, None]

                def put(o, sf, c):
                    cbuf[par, o, sf, :] = c
                    a = c[0:8] + c[8:16]
                    b = c[0:8] * c[0:8] + c[8:16] * c[8:16]
                    s1[o] = a if s1[o] is None else s1[o] + a
                    s2[o] = b if s2[o] is None else s2[o] + b

                for q in qs:
                    sf = slice(q * 16, q * 16 + 16)
                    rows = [(1 - par, 0), (1 - par, 1), (par, 0), (par, 1)]
                    rhs = [cw[rlr(a, n, 0, q), :] for a, n in rows] + [cw[rlr(a, n, 1, q), :] for a, n in rows]
                    lhs = _b(la[q])
                    if q < NBQ:
                        rhs += [cw[rc(a, n, q), :] for a, n in rows] + [jnp.zeros((32, W), U32)]
                        lhs = jnp.concatenate([lhs, _b(lb[q])], axis=1)
                    ca = jnp.dot(lhs, _b(jnp.concatenate(rhs, axis=0)), preferred_element_type=F32)
                    if arow is not None and q == qs[RQ]:
                        xr[arow, 0:8, 0:128] = ca[RO:RO + 8, 0:128].astype(BF16)
                    if q < NBQ:
                        for o in range(2):
                            put(o, sf, ca[o * 16:(o + 1) * 16, :])
                    else:
                        cf = [pltpu.bitcast(cw[rc(a, n, q), :], F32) for a, n in rows]
                        ws = [jnp.concatenate([dwb[a * 3 + 1, sf, :]] * NT, axis=1) for a in range(3)]
                        for o in range(2):
                            put(o, sf, (ca[o * 16:(o + 1) * 16, :] + ws[0] * cf[o]) + (
                                ws[1] * cf[o + 1] + ws[2] * cf[o + 2]))
                if fin:
                    m = butterfly(tiles(s1[0]) + tiles(s1[1])) * (1.0 / C)
                    q2 = butterfly(tiles(s2[0]) + tiles(s2[1])) * (1.0 / C)
                    var = jnp.maximum(q2 - m * m, 0.0)
                    rs = jax.lax.rsqrt(var + 1e-5) * _KAPPA
                    nrm[par] = rs
                    rst[kidx] = rs
                else:
                    for o in range(2):
                        stat[o, 0] = s1[o]
                        stat[o, 1] = s2[o]

            def s2b(par, j):
                xs = [cbuf[par, j, :, t * 128:(t + 1) * 128] * nrm[par, j * 4 + t:j * 4 + t + 1, :]
                      for t in range(NT)]
                return jnp.concatenate(xs, axis=1)

            def hslot(chunk, r):
                return None if r in REC else chunk * NS + STO.index(r)

            def body1(kk, slot):
                ns = nxt(slot, XS)
                cur = slot * CH
                last = kk == NCH - 1
                z = zs[0]
                arow = cur + z if REL else None

                def xrow(r):
                    return cur + r if r < CH else jnp.where(last, ZROW, ns * CH + (r - CH))

                def hs(r):
                    return hslot(kk, r) if r >= 0 else hslot(jnp.maximum(kk - 1, 0), r + CH)

                for u in range(U):
                    par = u % 2
                    for q in QB:
                        prep(par, (xrow(2 * u + 1), xrow(2 * u + 2)), q)
                    s3(s2b(1 - par, 0), hs(2 * u - 2), z)
                    s2a(par, QB, kk * U + u, arow)
                    for q in QA:
                        prep(1 - par, (xrow(2 * u + 3), xrow(2 * u + 4)), q)
                    s3(s2b(1 - par, 1), hs(2 * u - 1), z)
                    s2a(1 - par, QA, None, arow)

                @pl.when(kk == 0)
                def _():
                    xpart(CH + 3, 2 * CH, 1).wait()

                @pl.when(kk + 2 < NCH)
                def _():
                    xcopy(kk + 2, nxt(ns, XS)).wait()

                cn = kk + XS
                xcopy(jnp.where(cn < NCH, cn, cn - NCH), slot).start()
                return ns

            xpart(0, 3, 1).wait()
            for q in range(NQ):
                prep(1, (ZROW, 0), q)
            for q in QA:
                prep(0, (1, 2), q)
            s2a(0, QA, None)
            xpart(3, CH + 3, 0).wait()
            xpart(CH + 3, 2 * CH, 1).start()
            for c in range(2, XS):
                xcopy(c, c).start()
            for cp in wcp[2:]:
                cp.wait()
            if do1:
                jax.lax.fori_loop(0, NCH, body1, 0)
                xcopy(0, NCH % XS).wait()
                xcopy(1, (NCH + 1) % XS).wait()
                for j in range(2):
                    s3(s2b(1, j), hslot(NCH - 1, CH - 2 + j))
            else:
                xpart(CH + 3, 2 * CH, 1).wait()
                for c in range(2, XS):
                    xcopy(c, c).wait()
                for c in range(XS):
                    xcopy(c, (NCH + c) % XS).start()
                xcopy(0, NCH % XS).wait()
                xcopy(1, (NCH + 1) % XS).wait()

        pl.run_scoped(
            pass1,
            pltpu.VMEM((NQ, 16, 128), U32),
            pltpu.VMEM((NQ, 16, 128), U32),
            pltpu.VMEM((4 * C + 4 * CROWS, W), U32),
            pltpu.VMEM((2, 2, C, W), F32),
            pltpu.VMEM((2, 2, 8, W), F32),
            pltpu.VMEM((2, 8, 128), F32),
        )

        for r in range(5):
            unp((NCH % XS) * CH, r)
        for i in range(2):
            t0(0, (NCH % XS) * CH, i, 0, NCG)

        a = jnp.transpose(acc[...])
        ssq = jnp.sum(a, axis=0, keepdims=True) * (1.0 / (_GS * _GS))
        gx = jnp.sqrt(ssq + 1e-6)
        nx = gx / (jnp.mean(gx, axis=1, keepdims=True) + 1e-6)
        s = (gam_ref[...].astype(F32).reshape(1, E) * nx + 1.0) * (1.0 / _GS)
        w2f = w2t_ref[...].astype(F32)
        w2s[...] = _u((w2f * s).astype(BF16))
        b = jnp.sum(w2f * bet_ref[...].astype(F32).reshape(1, E), axis=1, keepdims=True)
        b2b[...] = jnp.broadcast_to(b, (C, 128))

        def pass2(orr, gt):
            def ocopy(c, slot):
                return pltpu.make_async_copy(
                    orr.at[slot], o_hbm.at[pl.ds(c * CH, CH)], osem.at[slot])

            def anchor(v, z):
                dwb[9 + z, 0:8, :] = v

            def t1(i, z):
                if UPAD:
                    pad = wk[pl.ds(pl.multiple_of(z, 8), 128 - C), :].astype(BF16)
                    v_all = mm1(jnp.concatenate([xn2[i], pad], axis=0))
                else:
                    v_all = mm1(padk(xn2[i]))
                an = None
                for e in range(E // 16):
                    g = gelu(v_all[e * 16:(e + 1) * 16, :])
                    gt[i % 2, e * 16:(e + 1) * 16, :] = g.astype(BF16)
                    an = g[8:16, W - 128:W] if an is None else an + g[8:16, W - 128:W]
                if ANCH:
                    anchor(an, z)

            def t2(g, xb, oslot, row, hooks=()):
                y = jnp.dot(_b(w2s[...]), g, preferred_element_type=F32)
                bb = jnp.concatenate([b2b[...]] * NT, axis=1)
                orr[oslot, row] = (y + (bb + xr[xb + row].astype(F32))).astype(BF16)
                for t, z, fn in hooks:
                    an = y[0:8, t * 128:(t + 1) * 128]
                    for cg in range(1, C // 8):
                        an = an + y[cg * 8:(cg + 1) * 8, t * 128:(t + 1) * 128]
                    anchor(an, z)
                    fn()

            def body2(c, carry):
                xslot, oslot = carry
                xb = xslot * CH
                z = zs[0]
                c2 = jnp.minimum(c + 1, NCH - 1)
                xb2 = jnp.where(c + 1 < NCH, nxt(xslot, XS), xslot) * CH

                def t2s(i, hooks=()):
                    t2(hst[c * NS + i], xb, oslot, STO[i], hooks)

                def t0n(i, cg0, cg1):
                    if i < NR:
                        t0(c, xb, i, cg0, cg1)
                    else:
                        t0(c2, xb2, i - NR, cg0, cg1)

                si = 0
                for i in range(NF):
                    t2s(si)
                    si += 1
                cuts = [p[0] for p in PARTS] + [NCG]
                assert NR == 7
                prod = [[5], [6], [7], [8, 9], [10, 11], [12], [13]]
                for i in range(NR):
                    for r in prod[i]:
                        if r < NX:
                            unp(xb, r)
                        else:
                            unp(xb2, r - NX)
                    t1(i, z)
                    t0n(i + 2, 0, cuts[0])
                    hk = {'a': [], 'b': []}
                    for pi, (lo, tag) in enumerate(PARTS):
                        hk[tag[0]].append((int(tag[1]), z, functools.partial(t0n, i + 2, lo, cuts[pi + 1])))
                    if i > 0:
                        t2(gt[(i - 1) % 2], xb, oslot, REC[i - 1], hk['a'])
                    else:
                        t2s(si, hk['a'])
                        si += 1
                    t2s(si, hk['b'])
                    si += 1
                t2(gt[(NR - 1) % 2], xb, oslot, REC[NR - 1])
                while si < NS:
                    t2s(si)
                    si += 1
                ocopy(c, oslot).start()
                nx_ = nxt(xslot, XS)
                no_ = nxt(oslot, OS)

                @pl.when(c + XS < NCH)
                def _():
                    xcopy(c + XS, xslot).start()

                @pl.when(c + 2 < NCH)
                def _():
                    xcopy(c + 2, nxt(nx_, XS)).wait()

                @pl.when(c + 1 >= OS)
                def _():
                    ocopy(c + 1 - OS, no_).wait()
                return nx_, no_

            s0 = NCH % XS
            if do2:
                jax.lax.fori_loop(0, NCH, body2, (s0, 0))
                for c in range(NCH + 1 - OS, NCH):
                    ocopy(c, c % OS).wait()
            else:
                for c in range(2, XS):
                    xcopy(c, (s0 + c) % XS).wait()

        pl.run_scoped(pass2, pltpu.VMEM((OS, CH, C, W), BF16), pltpu.VMEM((2, E, W), BF16))

    @jax.jit
    def f(x, dw, w1, w2, grn_gamma, grn_beta):
        xt = jnp.transpose(x, (0, 1, 3, 2)).reshape(H, C, W)
        w2t = jnp.transpose(w2)
        hbm = pl.BlockSpec(memory_space=pl.ANY)
        out = pl.pallas_call(
            kernel,
            in_specs=[hbm] * 6,
            out_specs=pl.BlockSpec(memory_space=pl.ANY),
            out_shape=jax.ShapeDtypeStruct((H, C, W), BF16),
            scratch_shapes=[
                pltpu.VMEM((NCH * NS, E, W), BF16),
                pltpu.VMEM((NP, 8, 128), F32),
                pltpu.VMEM((XS * CH + 1, C, W), BF16),
                pltpu.VMEM((10, C, 128), F32),
                pltpu.VMEM((E // 2, 128), U32),
                pltpu.VMEM((C // 2, E), U32),
                pltpu.VMEM((C, 128), F32),
                pltpu.VMEM((E, 128), F32),
                pltpu.VMEM((NR, C, W), BF16),
                pltpu.VMEM(((NR + 2) * C, W), F32),
                pltpu.VMEM((3, 3, C), BF16),
                pltpu.VMEM((C, E), BF16),
                pltpu.VMEM((C, E), BF16),
                pltpu.VMEM((E,), BF16),
                pltpu.VMEM((E,), BF16),
                pltpu.SMEM((1,), jnp.int32),
                pltpu.SemaphoreType.DMA((XS,)),
                pltpu.SemaphoreType.DMA((OS,)),
                pltpu.SemaphoreType.DMA((5,)),
            ],
            compiler_params=pltpu.CompilerParams(vmem_limit_bytes=vmem_mb << 20),
        )(xt, dw, w1, w2t, grn_gamma, grn_beta)
        return jnp.transpose(out.reshape(1, H, C, W), (0, 1, 3, 2))
    return f


pallas_standalone__modern_conv_block_convnext_v2__vision_kernel = build(**{})
```

```python
import functools
import math

import jax
import jax.numpy as jnp
import jax.experimental.pallas as pl
import jax.experimental.pallas.tpu as pltpu

F32 = jnp.float32
BF16 = jnp.bfloat16
U32 = jnp.uint32

_C0 = math.sqrt(2.0 / math.pi)
_KAPPA = (_C0 * 0.044715) ** (1.0 / 3.0)
_A = _C0 / _KAPPA
_GS = 2.0 * _KAPPA


def _u(x):
    return pltpu.bitcast(x, U32)


def _b(x):
    return pltpu.bitcast(x, BF16)


def build(NBQ=2, XS=4, OS=2, NR=7, NF=0, PARTS=((6, 'a3'),), ANCH=True, XA=(0, 128, 256), PROD=((0, 1), (2,), (3,), (4,), (5,), (6,), (7, 8)), PA=352, REL=1, RQ=1, RO=0, QA=(2, 3, 0), QB=(4, 5, 1),
          PIECES=((0, 4), (8, 12), (4, 6), (12, 14), (6, 8), (14, 16)), NOBC=True, RPAD=8, vmem_mb=128, do1=True, do2=True):
    H, W, C, E = 512, 512, 96, 384
    NT = W // 128
    NQ = C // 16
    CH = 16
    NCH = H // CH
    U = CH // 2
    NP = H // 2
    REC = list(range(1, NR + 1))
    STO = [r for r in range(CH) if r not in REC]
    NS = len(STO)
    ZROW = XS * CH
    CROWS = NBQ * 8 + (NQ - NBQ) * 16

    def kernel(x_hbm, dw_hbm, w1_hbm, w2t_hbm, gam_hbm, bet_hbm,
               o_hbm,
               hst, rst, xr, dwb, w1t, w2s, b2b, acc, xn2, wk,
               dw_ref, w1_ref, w2t_ref, gam_ref, bet_ref, zs, xsem, osem, wsem):

        def xcopy(c, slot):
            return pltpu.make_async_copy(
                x_hbm.at[pl.ds(c * CH, CH)], xr.at[pl.ds(slot * CH, CH)], xsem.at[slot])

        def nxt(s, n):
            return jnp.where(s == n - 1, 0, s + 1)

        def xpart(lo, hi, sem):
            return pltpu.make_async_copy(x_hbm.at[pl.ds(lo, hi - lo)], xr.at[pl.ds(lo, hi - lo)], xsem.at[sem])

        wcp = [pltpu.make_async_copy(src, dst, wsem.at[i]) for i, (src, dst) in enumerate(
            [(dw_hbm, dw_ref), (w1_hbm, w1_ref), (w2t_hbm, w2t_ref), (gam_hbm, gam_ref), (bet_hbm, bet_ref)])]
        wcp[0].start()
        wcp[1].start()
        xpart(0, 5, 1).start()
        xpart(5, CH + 5, 0).start()
        for cp in wcp[2:]:
            cp.start()
        zs[0] = 0
        wcp[0].wait()
        wcp[1].wait()

        def tiles(v):
            return [v[:, t * 128:(t + 1) * 128] for t in range(NT)]

        def mm1(xp, e0=0, e1=E):
            return jnp.dot(_b(w1t[e0 // 2:e1 // 2, :]), xp, preferred_element_type=F32)

        def padk(xn):
            return jnp.concatenate([xn, jnp.zeros((128 - C, W), xn.dtype)], axis=0)

        def gelu(v):
            z = v * (v * v + _A)
            return v * (jnp.tanh(z) + 1.0)

        lane = jax.lax.broadcasted_iota(jnp.int32, (8, 128), 1)
        m0 = lane == 0
        m127 = lane == 127

        NCG = C // 8
        NX = NR + 2

        def unp(xb, r, lo=0, hi=C):
            wk[r * C + lo:r * C + hi, :] = xr[xb + r, lo:hi, :].astype(F32)

        def t0(c, xb, i, cg0, cg1):
            r = REC[i]
            rs = [rst[c * U + r // 2, (r % 2) * 4 + t:(r % 2) * 4 + t + 1, :] for t in range(NT)]
            for cg in range(cg0, cg1):
                sl = slice(cg * 8, cg * 8 + 8)
                xs = [tiles(wk[(r - 1 + a) * C + cg * 8:(r - 1 + a) * C + cg * 8 + 8, :]) for a in range(3)]
                cs = []
                for b in range(3):
                    ws = [dwb[a * 3 + b, sl, :] for a in range(3)]
                    cs.append([ws[0] * xs[0][t] + ws[1] * xs[1][t] + ws[2] * xs[2][t] for t in range(NT)])
                rl = [pltpu.roll(cs[0][t], 1, 1) for t in range(NT)]
                rg = [pltpu.roll(cs[2][t], 127, 1) for t in range(NT)]
                row = []
                for t in range(NT):
                    left = jnp.where(m0, rl[t - 1] if t > 0 else 0.0, rl[t])
                    right = jnp.where(m127, rg[t + 1] if t < NT - 1 else 0.0, rg[t])
                    row.append((cs[1][t] + (left + right)) * rs[t])
                xn2[i, sl, :] = jnp.concatenate(row, axis=1).astype(BF16)

        def pass1(la, lb, cw, cbuf, stat, nrm):
            rr = jax.lax.broadcasted_iota(jnp.int32, (C, C), 0)
            cc = jax.lax.broadcasted_iota(jnp.int32, (C, C), 1)
            for a in range(3):
                for b in range(3):
                    row = dw_ref[a, b:b + 1, :].astype(F32)
                    d = jnp.where(rr == cc, jnp.broadcast_to(row, (C, C)), 0.0)
                    col = jnp.sum(d, axis=1, keepdims=True)
                    dwb[a * 3 + b] = jnp.broadcast_to(col, (C, 128))
            r16 = jax.lax.broadcasted_iota(jnp.int32, (16, 128), 0)
            c16 = jax.lax.broadcasted_iota(jnp.int32, (16, 128), 1)
            for q in range(NQ):
                ta, tb = [], []
                sf = slice(q * 16, q * 16 + 16)
                for o in range(2):
                    ma = jnp.zeros((16, 128), F32)
                    mb = jnp.zeros((16, 128), F32)
                    for a in range(3):
                        ma = jnp.where(c16 == (a + o) * 16 + r16, dwb[a * 3 + 0, sf, :], ma)
                        ma = jnp.where(c16 == (4 + a + o) * 16 + r16, dwb[a * 3 + 2, sf, :], ma)
                        mb = jnp.where(c16 == (a + o) * 16 + r16, dwb[a * 3 + 1, sf, :], mb)
                    ta.append(ma)
                    tb.append(mb)
                la[q] = _u(jnp.concatenate(ta, axis=0).astype(BF16))
                lb[q] = _u(jnp.concatenate(tb, axis=0).astype(BF16))
            re = jax.lax.broadcasted_iota(jnp.int32, (E, E), 0)
            ce = jax.lax.broadcasted_iota(jnp.int32, (E, E), 1)
            eye = jnp.where(re == ce, 1.0, 0.0).astype(BF16)
            w1f = w1_ref[...].astype(F32)
            w1c = (w1f - jnp.mean(w1f, axis=0, keepdims=True)).astype(BF16).astype(F32)
            aw = jnp.abs(w1c)
            small = aw <= jnp.maximum(0.3 * jnp.mean(aw, axis=0, keepdims=True), jnp.min(aw, axis=0, keepdims=True))
            cnt = jnp.sum(jnp.where(small, 1.0, 0.0), axis=0, keepdims=True)
            w1c = jnp.where(small, w1c - jnp.sum(w1c, axis=0, keepdims=True) / cnt, w1c).astype(BF16)
            w1p = jnp.concatenate([w1c, jnp.zeros((128 - C, E), BF16)], axis=0)
            t = jax.lax.dot_general(eye, w1p, (((1,), (1,)), ((), ())),
                                    preferred_element_type=F32)
            w1t[...] = _u(t.astype(BF16))
            acc[...] = jnp.zeros_like(acc)
            cw[0:16, :] = jnp.zeros((16, W), U32)
            xr[ZROW] = jnp.zeros((C, W), BF16)

            sub = jax.lax.broadcasted_iota(jnp.int32, (8, 128), 0)

            def butterfly(vs):
                for d in (1, 2, 4):
                    mk = (sub % (2 * d)) < d
                    vs = [jnp.where(mk, vs[i], vs[i + 1]) + pltpu.roll(jnp.where(mk, vs[i + 1], vs[i]), d, 0)
                          for i in range(0, len(vs), 2)]
                return vs[0]

            def rlr(par, n, lr, q):
                o = ((par * 2 + n) * 2 + lr) * (C // 2) + q * 8
                return slice(o, o + 8)

            def rc(par, n, q):
                o = 4 * C + (par * 2 + n) * CROWS
                if q < NBQ:
                    return slice(o + q * 8, o + q * 8 + 8)
                o += NBQ * 8 + (q - NBQ) * 16
                return slice(o, o + 16)

            def s3p(xp, hidx, e0, e1):
                v_all = mm1(xp, e0, e1)
                for e in range(e0 // 16, e1 // 16):
                    g = gelu(v_all[e * 16 - e0:(e + 1) * 16 - e0, :])
                    g2 = tiles(g * g)
                    acc[e * 16:(e + 1) * 16, :] += (g2[0] + g2[1]) + (g2[2] + g2[3])
                    if hidx is not None:
                        hst[hidx, e * 16:(e + 1) * 16, :] = g.astype(BF16)

            def s3(xn, hidx, z=None):
                if z is None or not PA:
                    s3p(padk(xn).astype(BF16), hidx, 0, E)
                    return
                s3p(padk(xn).astype(BF16), hidx, 0, PA)
                pad = _b(cw[pl.ds(pl.multiple_of(z, 8), 16), :]).astype(F32)
                s3p(jnp.concatenate([xn, pad], axis=0).astype(BF16), hidx, PA, E)

            def prep(par, rows, q):
                zero = jnp.zeros((8, 128), U32)
                sf = slice(q * 16, q * 16 + 16)
                for n in range(2):
                    p = _u(xr[rows[n], sf, :])
                    pt = tiles(p)
                    rl = [pltpu.roll(pt[t], 1, 1) for t in range(NT)]
                    rg = [pltpu.roll(pt[t], 127, 1) for t in range(NT)]
                    cw[rlr(par, n, 0, q), :] = jnp.concatenate(
                        [jnp.where(m0, rl[t - 1] if t > 0 else zero, rl[t]) for t in range(NT)], axis=1)
                    cw[rlr(par, n, 1, q), :] = jnp.concatenate(
                        [jnp.where(m127, rg[t + 1] if t < NT - 1 else zero, rg[t]) for t in range(NT)], axis=1)
                    if q < NBQ:
                        cw[rc(par, n, q), :] = p
                    else:
                        cw[rc(par, n, q), :] = _u(_b(p).astype(F32))

            def s2a(par, qs, kidx, arow=None):
                fin = kidx is not None
                if fin:
                    s1 = [stat[o, 0] for o in range(2)]
                    s2 = [stat[o, 1] for o in range(2)]
                else:
                    s1 = [None, None]
                    s2 = [None, None]

                def put(o, sf, c):
                    cbuf[par, o, sf, :] = c
                    a = c[0:8] + c[8:16]
                    b = c[0:8] * c[0:8] + c[8:16] * c[8:16]
                    s1[o] = a if s1[o] is None else s1[o] + a
                    s2[o] = b if s2[o] is None else s2[o] + b

                for q in qs:
                    sf = slice(q * 16, q * 16 + 16)
                    rows = [(1 - par, 0), (1 - par, 1), (par, 0), (par, 1)]
                    rhs = [cw[rlr(a, n, 0, q), :] for a, n in rows] + [cw[rlr(a, n, 1, q), :] for a, n in rows]
                    lhs = _b(la[q])
                    if q < NBQ:
                        rhs += [cw[rc(a, n, q), :] for a, n in rows] + [jnp.zeros((32, W), U32)]
                        lhs = jnp.concatenate([lhs, _b(lb[q])], axis=1)
                    ca = jnp.dot(lhs, _b(jnp.concatenate(rhs, axis=0)), preferred_element_type=F32)
                    if arow is not None and q == qs[RQ]:
                        xr[arow, 0:8, 0:128] = ca[RO:RO + 8, 0:128].astype(BF16)
                    if q < NBQ:
                        for o in range(2):
                            put(o, sf, ca[o * 16:(o + 1) * 16, :])
                    else:
                        cf = [pltpu.bitcast(cw[rc(a, n, q), :], F32) for a, n in rows]
                        ws = [jnp.concatenate([dwb[a * 3 + 1, sf, :]] * NT, axis=1) for a in range(3)]
                        for o in range(2):
                            put(o, sf, (ca[o * 16:(o + 1) * 16, :] + ws[0] * cf[o]) + (
                                ws[1] * cf[o + 1] + ws[2] * cf[o + 2]))
                if fin:
                    m = butterfly(tiles(s1[0]) + tiles(s1[1])) * (1.0 / C)
                    q2 = butterfly(tiles(s2[0]) + tiles(s2[1])) * (1.0 / C)
                    var = jnp.maximum(q2 - m * m, 0.0)
                    rs = jax.lax.rsqrt(var + 1e-5) * _KAPPA
                    nrm[par] = rs
                    rst[kidx] = rs
                else:
                    for o in range(2):
                        stat[o, 0] = s1[o]
                        stat[o, 1] = s2[o]

            def s2b(par, j):
                xs = [cbuf[par, j, :, t * 128:(t + 1) * 128] * nrm[par, j * 4 + t:j * 4 + t + 1, :]
                      for t in range(NT)]
                return jnp.concatenate(xs, axis=1)

            def hslot(chunk, r):
                return None if r in REC else chunk * NS + STO.index(r)

            def body1(kk, slot):
                ns = nxt(slot, XS)
                cur = slot * CH
                last = kk == NCH - 1
                z = zs[0]
                arow = cur + z if REL else None

                def xrow(r):
                    return cur + r if r < CH else jnp.where(last, ZROW, ns * CH + (r - CH))

                for u in range(U):
                    par = (u + 1) % 2
                    for q in QB:
                        prep(par, (xrow(2 * u + 3), xrow(2 * u + 4)), q)
                    s3(s2b(1 - par, 0), hslot(kk, 2 * u), z)
                    s2a(par, QB, kk * U + u + 1, arow)
                    for q in QA:
                        prep(1 - par, (xrow(2 * u + 5), xrow(2 * u + 6)), q)
                    s3(s2b(1 - par, 1), hslot(kk, 2 * u + 1), z)
                    s2a(1 - par, QA, None, arow)

                cn = kk + XS
                xcopy(jnp.where(cn < NCH, cn, cn - NCH), slot).start()

                @pl.when(kk == 0)
                def _():
                    xpart(CH + 5, 2 * CH, 1).wait()

                @pl.when(kk + 2 < NCH)
                def _():
                    xcopy(kk + 2, nxt(ns, XS)).wait()
                return ns

            xpart(0, 5, 1).wait()
            for q in range(NQ):
                prep(1, (ZROW, 0), q)
            for q in range(NQ):
                prep(0, (1, 2), q)
            s2a(0, QA, None)
            s2a(0, QB, 0)
            for q in QA:
                prep(1, (3, 4), q)
            s2a(1, QA, None)
            xpart(5, CH + 5, 0).wait()
            xpart(CH + 5, 2 * CH, 1).start()
            for c in range(2, XS):
                xcopy(c, c).start()
            for cp in wcp[2:]:
                cp.wait()
            if do1:
                jax.lax.fori_loop(0, NCH, body1, 0)
                xcopy(0, NCH % XS).wait()
                xcopy(1, (NCH + 1) % XS).wait()
            else:
                xpart(CH + 5, 2 * CH, 1).wait()
                for c in range(2, XS):
                    xcopy(c, c).wait()
                for c in range(XS):
                    xcopy(c, (NCH + c) % XS).start()
                xcopy(0, NCH % XS).wait()
                xcopy(1, (NCH + 1) % XS).wait()

        pl.run_scoped(
            pass1,
            pltpu.VMEM((NQ, 16, 128), U32),
            pltpu.VMEM((NQ, 16, 128), U32),
            pltpu.VMEM((4 * C + 4 * CROWS, W), U32),
            pltpu.VMEM((2, 2, C, W), F32),
            pltpu.VMEM((2, 2, 8, W), F32),
            pltpu.VMEM((2, 8, 128), F32),
        )

        for r in range(NX):
            unp((NCH % XS) * CH, r)
        for i in range(2):
            t0(0, (NCH % XS) * CH, i, 0, NCG)

        a = jnp.transpose(acc[...])
        ssq = jnp.sum(a, axis=0, keepdims=True) * (1.0 / (_GS * _GS))
        gx = jnp.sqrt(ssq + 1e-6)
        nx = gx / (jnp.mean(gx, axis=1, keepdims=True) + 1e-6)
        s = (gam_ref[...].astype(F32).reshape(1, E) * nx + 1.0) * (1.0 / _GS)
        w2f = w2t_ref[...].astype(F32)
        w2s[...] = _u((w2f * s).astype(BF16))
        b = jnp.sum(w2f * bet_ref[...].astype(F32).reshape(1, E), axis=1, keepdims=True)
        b2b[...] = jnp.broadcast_to(b, (C, 128))

        def pass2(orr, gt):
            def opiece(c, slot, lo, hi):
                return pltpu.make_async_copy(
                    orr.at[slot, pl.ds(lo, hi - lo)], o_hbm.at[pl.ds(c * CH + lo, hi - lo)], osem.at[slot])

            def owait(c, slot):
                for lo, hi in PIECES:
                    opiece(c, slot, lo, hi).wait()

            def anchor(v, z):
                dwb[9 + z, 0:8, :] = v

            def t1(i, z, fn):
                v_all = mm1(padk(xn2[i]))
                for k, xa in enumerate(XA):
                    xr[ZROW + z, 0:8, 0:128] = v_all[xa:xa + 8, 0:128].astype(BF16)
                    fn(k * C // len(XA), (k + 1) * C // len(XA))
                an = None
                for e in range(E // 16):
                    g = gelu(v_all[e * 16:(e + 1) * 16, :])
                    gt[i % 2, e * 16:(e + 1) * 16, :] = g.astype(BF16)
                    an = g[8:16, W - 128:W] if an is None else an + g[8:16, W - 128:W]
                if ANCH:
                    anchor(an, z)

            def t2(g, xb, oslot, row, hooks=()):
                t2_(g, xb, oslot, row, hooks)
                done.add(row)
                for lo, hi in PIECES:
                    if lo <= row < hi and all(r in done for r in range(lo, hi)):
                        opiece(cur_c[0], oslot, lo, hi).start()

            done = set()
            cur_c = [None]

            def t2_(g, xb, oslot, row, hooks=()):
                y = jnp.dot(_b(w2s[...]), g, preferred_element_type=F32)
                bb = jnp.concatenate([b2b[...]] * NT, axis=1)
                orr[oslot, row] = (y + (bb + xr[xb + row].astype(F32))).astype(BF16)
                for t, z, fn in hooks:
                    an = y[0:8, t * 128:(t + 1) * 128]
                    for cg in range(1, C // 8):
                        an = an + y[cg * 8:(cg + 1) * 8, t * 128:(t + 1) * 128]
                    anchor(an, z)
                    fn()

            def body2(c, carry):
                xslot, oslot = carry
                done.clear()
                cur_c[0] = c
                xb = xslot * CH
                z = zs[0]
                c2 = jnp.minimum(c + 1, NCH - 1)
                xb2 = jnp.where(c + 1 < NCH, nxt(xslot, XS), xslot) * CH

                def t2s(i, hooks=()):
                    t2(hst[c * NS + i], xb, oslot, STO[i], hooks)

                def t0n(i, cg0, cg1):
                    if i < NR:
                        t0(c, xb, i, cg0, cg1)
                    else:
                        t0(c2, xb2, i - NR, cg0, cg1)

                si = 0
                for i in range(NF):
                    t2s(si)
                    si += 1
                cuts = [p[0] for p in PARTS] + [NCG]
                assert NR == 7
                for i in range(NR):
                    t1(i, z, lambda lo, hi: [unp(xb2, r, lo, hi) for r in PROD[i]])
                    t0n(i + 2, 0, cuts[0])
                    hk = {'a': [], 'b': []}
                    for pi, (lo, tag) in enumerate(PARTS):
                        hk[tag[0]].append((int(tag[1]), z, functools.partial(t0n, i + 2, lo, cuts[pi + 1])))
                    if i > 0:
                        t2(gt[(i - 1) % 2], xb, oslot, REC[i - 1], hk['a'])
                    else:
                        t2s(si, hk['a'])
                        si += 1
                    t2s(si, hk['b'])
                    si += 1
                t2(gt[(NR - 1) % 2], xb, oslot, REC[NR - 1])
                while si < NS:
                    t2s(si)
                    si += 1
                nx_ = nxt(xslot, XS)
                no_ = nxt(oslot, OS)

                @pl.when(c + XS < NCH)
                def _():
                    xcopy(c + XS, xslot).start()

                @pl.when(c + 2 < NCH)
                def _():
                    xcopy(c + 2, nxt(nx_, XS)).wait()

                @pl.when(c + 1 >= OS)
                def _():
                    owait(c + 1 - OS, no_)
                return nx_, no_

            s0 = NCH % XS
            if do2:
                jax.lax.fori_loop(0, NCH, body2, (s0, 0))
                for c in range(NCH + 1 - OS, NCH):
                    owait(c, c % OS)
            else:
                for c in range(2, XS):
                    xcopy(c, (s0 + c) % XS).wait()

        pl.run_scoped(pass2, pltpu.VMEM((OS, CH, C, W), BF16), pltpu.VMEM((2, E, W), BF16))

    @jax.jit
    def f(x, dw, w1, w2, grn_gamma, grn_beta):
        xt = jnp.transpose(x, (0, 1, 3, 2)).reshape(H, C, W)
        w2t = jnp.transpose(w2)
        hbm = pl.BlockSpec(memory_space=pl.ANY)
        out = pl.pallas_call(
            kernel,
            in_specs=[hbm] * 6,
            out_specs=pl.BlockSpec(memory_space=pl.ANY),
            out_shape=jax.ShapeDtypeStruct((H, C, W), BF16),
            scratch_shapes=[
                pltpu.VMEM((NCH * NS, E, W), BF16),
                pltpu.VMEM((NP + RPAD, 8, 128), F32),
                pltpu.VMEM((XS * CH + 1, C, W), BF16),
                pltpu.VMEM((10, C, 128), F32),
                pltpu.VMEM((E // 2, 128), U32),
                pltpu.VMEM((C // 2, E), U32),
                pltpu.VMEM((C, 128), F32),
                pltpu.VMEM((E, 128), F32),
                pltpu.VMEM((NR, C, W), BF16),
                pltpu.VMEM(((NR + 2) * C, W), F32),
                pltpu.VMEM((3, 3, C), BF16),
                pltpu.VMEM((C, E), BF16),
                pltpu.VMEM((C, E), BF16),
                pltpu.VMEM((E,), BF16),
                pltpu.VMEM((E,), BF16),
                pltpu.SMEM((1,), jnp.int32),
                pltpu.SemaphoreType.DMA((XS,)),
                pltpu.SemaphoreType.DMA((OS,)),
                pltpu.SemaphoreType.DMA((5,)),
            ],
            compiler_params=pltpu.CompilerParams(vmem_limit_bytes=vmem_mb << 20, disable_bounds_checks=NOBC),
        )(xt, dw, w1, w2t, grn_gamma, grn_beta)
        return jnp.transpose(out.reshape(1, H, C, W), (0, 1, 3, 2))
    return f


pallas_standalone__modern_conv_block_convnext_v2__vision_kernel = build(**{})
```

```python
import functools
import math

import jax
import jax.numpy as jnp
import jax.experimental.pallas as pl
import jax.experimental.pallas.tpu as pltpu

F32 = jnp.float32
BF16 = jnp.bfloat16
U32 = jnp.uint32

_C0 = math.sqrt(2.0 / math.pi)
_KAPPA = (_C0 * 0.044715) ** (1.0 / 3.0)
_A = _C0 / _KAPPA
_GS = 2.0 * _KAPPA


def _u(x):
    return pltpu.bitcast(x, U32)


def _b(x):
    return pltpu.bitcast(x, BF16)


def build(NBQ=2, XS=7, NB1=2, NB2=2, NR=7, NF=0, PARTS=((6, 'a3'),), ANCH=True, XA=(0, 128, 256), PROD=((0, 1), (2,), (3,), (4,), (5,), (6,), (7, 8)), PA=368, REL=1, RQ=1, RO=16, QA=(2, 3, 0), QB=(4, 5, 1),
          PIECES=((0, 4), (8, 12), (4, 6), (12, 14), (6, 8), (14, 16)), NOBC=True, RPAD=8, vmem_mb=128, do1=True, do2=True):
    H, W, C, E = 512, 512, 96, 384
    NT = W // 128
    NQ = C // 16
    CH = 16
    NCH = H // CH
    U = CH // 2
    NP = H // 2
    REC = list(range(1, NR + 1))
    STO = [r for r in range(CH) if r not in REC]
    NS = len(STO)
    ZROW = XS * CH
    P2PRE = XS - NB2
    CROWS = NBQ * 8 + (NQ - NBQ) * 16

    def kernel(x_hbm, dw_hbm, w1_hbm, w2t_hbm, gam_hbm, bet_hbm,
               o_hbm,
               hst, rst, xr, dwb, w1t, w2s, b2b, acc, xn2, wk,
               dw_ref, w1_ref, w2t_ref, gam_ref, bet_ref, zs, xsem, osem, wsem):

        def xcopy(c, slot):
            return pltpu.make_async_copy(
                x_hbm.at[pl.ds(c * CH, CH)], xr.at[pl.ds(slot * CH, CH)], xsem.at[slot])

        def nxt(s, n):
            return jnp.where(s == n - 1, 0, s + 1)

        def xpart(lo, hi, sem):
            return pltpu.make_async_copy(x_hbm.at[pl.ds(lo, hi - lo)], xr.at[pl.ds(lo, hi - lo)], xsem.at[sem])

        wcp = [pltpu.make_async_copy(src, dst, wsem.at[i]) for i, (src, dst) in enumerate(
            [(dw_hbm, dw_ref), (w1_hbm, w1_ref), (w2t_hbm, w2t_ref), (gam_hbm, gam_ref), (bet_hbm, bet_ref)])]
        wcp[0].start()
        wcp[1].start()
        xpart(0, 5, 1).start()
        xpart(5, CH + 5, 0).start()
        for cp in wcp[2:]:
            cp.start()
        zs[0] = 0
        wcp[0].wait()
        wcp[1].wait()

        def tiles(v):
            return [v[:, t * 128:(t + 1) * 128] for t in range(NT)]

        def mm1(xp, e0=0, e1=E):
            return jnp.dot(_b(w1t[e0 // 2:e1 // 2, :]), xp, preferred_element_type=F32)

        def padk(xn):
            return jnp.concatenate([xn, jnp.zeros((128 - C, W), xn.dtype)], axis=0)

        def gelu(v):
            z = v * (v * v + _A)
            return v * (jnp.tanh(z) + 1.0)

        lane = jax.lax.broadcasted_iota(jnp.int32, (8, 128), 1)
        m0 = lane == 0
        m127 = lane == 127

        NCG = C // 8
        NX = NR + 2

        def unp(xb, r, lo=0, hi=C):
            wk[r * C + lo:r * C + hi, :] = xr[xb + r, lo:hi, :].astype(F32)

        def t0(c, xb, i, cg0, cg1):
            r = REC[i]
            rs = [rst[c * U + r // 2, (r % 2) * 4 + t:(r % 2) * 4 + t + 1, :] for t in range(NT)]
            for cg in range(cg0, cg1):
                sl = slice(cg * 8, cg * 8 + 8)
                xs = [tiles(wk[(r - 1 + a) * C + cg * 8:(r - 1 + a) * C + cg * 8 + 8, :]) for a in range(3)]
                cs = []
                for b in range(3):
                    ws = [dwb[a * 3 + b, sl, :] for a in range(3)]
                    cs.append([ws[0] * xs[0][t] + ws[1] * xs[1][t] + ws[2] * xs[2][t] for t in range(NT)])
                rl = [pltpu.roll(cs[0][t], 1, 1) for t in range(NT)]
                rg = [pltpu.roll(cs[2][t], 127, 1) for t in range(NT)]
                row = []
                for t in range(NT):
                    left = jnp.where(m0, rl[t - 1] if t > 0 else 0.0, rl[t])
                    right = jnp.where(m127, rg[t + 1] if t < NT - 1 else 0.0, rg[t])
                    row.append((cs[1][t] + (left + right)) * rs[t])
                xn2[i, sl, :] = jnp.concatenate(row, axis=1).astype(BF16)

        def pass1(la, lb, cw, cbuf, stat, nrm):
            rr = jax.lax.broadcasted_iota(jnp.int32, (C, C), 0)
            cc = jax.lax.broadcasted_iota(jnp.int32, (C, C), 1)
            for a in range(3):
                for b in range(3):
                    row = dw_ref[a, b:b + 1, :].astype(F32)
                    d = jnp.where(rr == cc, jnp.broadcast_to(row, (C, C)), 0.0)
                    col = jnp.sum(d, axis=1, keepdims=True)
                    dwb[a * 3 + b] = jnp.broadcast_to(col, (C, 128))
            r16 = jax.lax.broadcasted_iota(jnp.int32, (16, 128), 0)
            c16 = jax.lax.broadcasted_iota(jnp.int32, (16, 128), 1)
            for q in range(NQ):
                ta, tb = [], []
                sf = slice(q * 16, q * 16 + 16)
                for o in range(2):
                    ma = jnp.zeros((16, 128), F32)
                    mb = jnp.zeros((16, 128), F32)
                    for a in range(3):
                        ma = jnp.where(c16 == (a + o) * 16 + r16, dwb[a * 3 + 0, sf, :], ma)
                        ma = jnp.where(c16 == (4 + a + o) * 16 + r16, dwb[a * 3 + 2, sf, :], ma)
                        mb = jnp.where(c16 == (a + o) * 16 + r16, dwb[a * 3 + 1, sf, :], mb)
                    ta.append(ma)
                    tb.append(mb)
                la[q] = _u(jnp.concatenate(ta, axis=0).astype(BF16))
                lb[q] = _u(jnp.concatenate(tb, axis=0).astype(BF16))
            re = jax.lax.broadcasted_iota(jnp.int32, (E, E), 0)
            ce = jax.lax.broadcasted_iota(jnp.int32, (E, E), 1)
            eye = jnp.where(re == ce, 1.0, 0.0).astype(BF16)
            w1f = w1_ref[...].astype(F32)
            w1c = (w1f - jnp.mean(w1f, axis=0, keepdims=True)).astype(BF16).astype(F32)
            aw = jnp.abs(w1c)
            small = aw <= jnp.maximum(0.3 * jnp.mean(aw, axis=0, keepdims=True), jnp.min(aw, axis=0, keepdims=True))
            cnt = jnp.sum(jnp.where(small, 1.0, 0.0), axis=0, keepdims=True)
            w1c = jnp.where(small, w1c - jnp.sum(w1c, axis=0, keepdims=True) / cnt, w1c).astype(BF16)
            w1p = jnp.concatenate([w1c, jnp.zeros((128 - C, E), BF16)], axis=0)
            t = jax.lax.dot_general(eye, w1p, (((1,), (1,)), ((), ())),
                                    preferred_element_type=F32)
            w1t[...] = _u(t.astype(BF16))
            acc[...] = jnp.zeros_like(acc)
            cw[0:16, :] = jnp.zeros((16, W), U32)
            xr[ZROW] = jnp.zeros((C, W), BF16)

            sub = jax.lax.broadcasted_iota(jnp.int32, (8, 128), 0)

            def butterfly(vs):
                for d in (1, 2, 4):
                    mk = (sub % (2 * d)) < d
                    vs = [jnp.where(mk, vs[i], vs[i + 1]) + pltpu.roll(jnp.where(mk, vs[i + 1], vs[i]), d, 0)
                          for i in range(0, len(vs), 2)]
                return vs[0]

            def rlr(par, n, lr, q):
                o = ((par * 2 + n) * 2 + lr) * (C // 2) + q * 8
                return slice(o, o + 8)

            def rc(par, n, q):
                o = 4 * C + (par * 2 + n) * CROWS
                if q < NBQ:
                    return slice(o + q * 8, o + q * 8 + 8)
                o += NBQ * 8 + (q - NBQ) * 16
                return slice(o, o + 16)

            def s3p(xp, hidx, e0, e1):
                v_all = mm1(xp, e0, e1)
                for e in range(e0 // 16, e1 // 16):
                    g = gelu(v_all[e * 16 - e0:(e + 1) * 16 - e0, :])
                    g2 = tiles(g * g)
                    acc[e * 16:(e + 1) * 16, :] += (g2[0] + g2[1]) + (g2[2] + g2[3])
                    if hidx is not None:
                        hst[hidx, e * 16:(e + 1) * 16, :] = g.astype(BF16)

            def s3(xn, hidx, z=None):
                if z is None or not PA:
                    s3p(padk(xn).astype(BF16), hidx, 0, E)
                    return
                s3p(padk(xn).astype(BF16), hidx, 0, PA)
                pad = _b(cw[pl.ds(pl.multiple_of(z, 8), 16), :]).astype(F32)
                s3p(jnp.concatenate([xn, pad], axis=0).astype(BF16), hidx, PA, E)

            def prep(par, rows, q):
                zero = jnp.zeros((8, 128), U32)
                sf = slice(q * 16, q * 16 + 16)
                for n in range(2):
                    p = _u(xr[rows[n], sf, :])
                    pt = tiles(p)
                    rl = [pltpu.roll(pt[t], 1, 1) for t in range(NT)]
                    rg = [pltpu.roll(pt[t], 127, 1) for t in range(NT)]
                    cw[rlr(par, n, 0, q), :] = jnp.concatenate(
                        [jnp.where(m0, rl[t - 1] if t > 0 else zero, rl[t]) for t in range(NT)], axis=1)
                    cw[rlr(par, n, 1, q), :] = jnp.concatenate(
                        [jnp.where(m127, rg[t + 1] if t < NT - 1 else zero, rg[t]) for t in range(NT)], axis=1)
                    if q < NBQ:
                        cw[rc(par, n, q), :] = p
                    else:
                        cw[rc(par, n, q), :] = _u(_b(p).astype(F32))

            def s2a(par, qs, kidx, arow=None):
                fin = kidx is not None
                if fin:
                    s1 = [stat[o, 0] for o in range(2)]
                    s2 = [stat[o, 1] for o in range(2)]
                else:
                    s1 = [None, None]
                    s2 = [None, None]

                def put(o, sf, c):
                    cbuf[par, o, sf, :] = c
                    a = c[0:8] + c[8:16]
                    b = c[0:8] * c[0:8] + c[8:16] * c[8:16]
                    s1[o] = a if s1[o] is None else s1[o] + a
                    s2[o] = b if s2[o] is None else s2[o] + b

                for q in qs:
                    sf = slice(q * 16, q * 16 + 16)
                    rows = [(1 - par, 0), (1 - par, 1), (par, 0), (par, 1)]
                    rhs = [cw[rlr(a, n, 0, q), :] for a, n in rows] + [cw[rlr(a, n, 1, q), :] for a, n in rows]
                    lhs = _b(la[q])
                    if q < NBQ:
                        rhs += [cw[rc(a, n, q), :] for a, n in rows] + [jnp.zeros((32, W), U32)]
                        lhs = jnp.concatenate([lhs, _b(lb[q])], axis=1)
                    ca = jnp.dot(lhs, _b(jnp.concatenate(rhs, axis=0)), preferred_element_type=F32)
                    if arow is not None and q == qs[RQ]:
                        xr[arow, 0:8, 0:128] = ca[RO:RO + 8, 0:128].astype(BF16)
                    if q < NBQ:
                        for o in range(2):
                            put(o, sf, ca[o * 16:(o + 1) * 16, :])
                    else:
                        cf = [pltpu.bitcast(cw[rc(a, n, q), :], F32) for a, n in rows]
                        ws = [jnp.concatenate([dwb[a * 3 + 1, sf, :]] * NT, axis=1) for a in range(3)]
                        for o in range(2):
                            put(o, sf, (ca[o * 16:(o + 1) * 16, :] + ws[0] * cf[o]) + (
                                ws[1] * cf[o + 1] + ws[2] * cf[o + 2]))
                if fin:
                    m = butterfly(tiles(s1[0]) + tiles(s1[1])) * (1.0 / C)
                    q2 = butterfly(tiles(s2[0]) + tiles(s2[1])) * (1.0 / C)
                    var = jnp.maximum(q2 - m * m, 0.0)
                    rs = jax.lax.rsqrt(var + 1e-5) * _KAPPA
                    nrm[par] = rs
                    rst[kidx] = rs
                else:
                    for o in range(2):
                        stat[o, 0] = s1[o]
                        stat[o, 1] = s2[o]

            def s2b(par, j):
                xs = [cbuf[par, j, :, t * 128:(t + 1) * 128] * nrm[par, j * 4 + t:j * 4 + t + 1, :]
                      for t in range(NT)]
                return jnp.concatenate(xs, axis=1)

            def hslot(chunk, r):
                return None if r in REC else chunk * NS + STO.index(r)

            def adv(s_, n):
                s_ = s_ + n
                return jnp.where(s_ >= XS, s_ - XS, s_)

            def body1(nb, c0, slot):
                z = zs[0]
                for h in range(nb):
                    kk = c0 + h
                    cur = adv(slot, h) * CH
                    nx_ = adv(slot, h + 1) * CH
                    last = kk == NCH - 1
                    arow = cur + z if REL else None

                    def xrow(r):
                        return cur + r if r < CH else jnp.where(last, ZROW, nx_ + (r - CH))

                    for u in range(U):
                        par = (u + 1) % 2
                        for q in QB:
                            prep(par, (xrow(2 * u + 3), xrow(2 * u + 4)), q)
                        s3(s2b(1 - par, 0), hslot(kk, 2 * u), z)
                        s2a(par, QB, kk * U + u + 1, arow)
                        for q in QA:
                            prep(1 - par, (xrow(2 * u + 5), xrow(2 * u + 6)), q)
                        s3(s2b(1 - par, 1), hslot(kk, 2 * u + 1), z)
                        s2a(1 - par, QA, None, arow)

                for h in range(nb):
                    cn = c0 + h + XS
                    if XS + h + c0_max(nb) < NCH + P2PRE:
                        xcopy(jnp.where(cn < NCH, cn, cn - NCH), adv(slot, h)).start()
                    else:
                        @pl.when(cn < NCH + P2PRE)
                        def _():
                            xcopy(jnp.where(cn < NCH, cn, cn - NCH), adv(slot, h)).start()

            def c0_max(nb):
                return NCH - nb

            def step1(i, slot):
                def one():
                    body1(1, jnp.where(i == 0, 0, NCH - 1), slot)

                    @pl.when(i == 0)
                    def _():
                        xpart(CH + 5, 2 * CH, 1).wait()
                        xcopy(2, 2).wait()
                        xcopy(3, 3).wait()
                    return adv(slot, 1)

                def two():
                    c0 = 2 * i - 1
                    body1(2, c0, slot)
                    for h in (3, 4):
                        @pl.when(c0 + h < NCH)
                        def _():
                            xcopy(c0 + h, adv(slot, h)).wait()
                    return adv(slot, 2)
                return jax.lax.cond(jnp.logical_or(i == 0, i == NCH // 2), one, two)

            def step1s(kk, slot):
                body1(1, kk, slot)

                @pl.when(kk == 0)
                def _():
                    xpart(CH + 5, 2 * CH, 1).wait()

                @pl.when(kk + 2 < NCH)
                def _():
                    xcopy(kk + 2, adv(slot, 2)).wait()
                return adv(slot, 1)

            xpart(0, 5, 1).wait()
            for q in range(NQ):
                prep(1, (ZROW, 0), q)
            for q in range(NQ):
                prep(0, (1, 2), q)
            s2a(0, QA, None)
            s2a(0, QB, 0)
            for q in QA:
                prep(1, (3, 4), q)
            s2a(1, QA, None)
            xpart(5, CH + 5, 0).wait()
            xpart(CH + 5, 2 * CH, 1).start()
            for c in range(2, XS):
                xcopy(c, c).start()
            for cp in wcp[2:]:
                cp.wait()
            if do1:
                if NB1 == 2:
                    jax.lax.fori_loop(0, NCH // 2 + 1, step1, 0)
                else:
                    jax.lax.fori_loop(0, NCH, step1s, 0)
                for c in range(NB2 + 1):
                    xcopy(c, (NCH + c) % XS).wait()
            else:
                xpart(CH + 5, 2 * CH, 1).wait()
                for c in range(2, XS):
                    xcopy(c, c).wait()
                for c in range(P2PRE):
                    xcopy(c, (NCH + c) % XS).start()
                for c in range(NB2 + 1):
                    xcopy(c, (NCH + c) % XS).wait()

        pl.run_scoped(
            pass1,
            pltpu.VMEM((NQ, 16, 128), U32),
            pltpu.VMEM((NQ, 16, 128), U32),
            pltpu.VMEM((4 * C + 4 * CROWS, W), U32),
            pltpu.VMEM((2, 2, C, W), F32),
            pltpu.VMEM((2, 2, 8, W), F32),
            pltpu.VMEM((2, 8, 128), F32),
        )

        for r in range(NX):
            unp((NCH % XS) * CH, r)
        for i in range(2):
            t0(0, (NCH % XS) * CH, i, 0, NCG)

        a = jnp.transpose(acc[...])
        ssq = jnp.sum(a, axis=0, keepdims=True) * (1.0 / (_GS * _GS))
        gx = jnp.sqrt(ssq + 1e-6)
        nx = gx / (jnp.mean(gx, axis=1, keepdims=True) + 1e-6)
        s = (gam_ref[...].astype(F32).reshape(1, E) * nx + 1.0) * (1.0 / _GS)
        w2f = w2t_ref[...].astype(F32)
        w2s[...] = _u((w2f * s).astype(BF16))
        b = jnp.sum(w2f * bet_ref[...].astype(F32).reshape(1, E), axis=1, keepdims=True)
        b2b[...] = jnp.broadcast_to(b, (C, 128))

        def pass2(gt):
            def opiece(c, slot, lo, hi):
                return pltpu.make_async_copy(
                    xr.at[pl.ds(slot * CH + lo, hi - lo)], o_hbm.at[pl.ds(c * CH + lo, hi - lo)], osem.at[slot])

            def owait(c, slot):
                for lo, hi in PIECES:
                    opiece(c, slot, lo, hi).wait()

            def anchor(v, z):
                dwb[9 + z, 0:8, :] = v

            def t1(i, z, fn):
                v_all = mm1(padk(xn2[i]))
                for k, xa in enumerate(XA):
                    xr[ZROW + z, 0:8, 0:128] = v_all[xa:xa + 8, 0:128].astype(BF16)
                    fn(k * C // len(XA), (k + 1) * C // len(XA))
                an = None
                for e in range(E // 16):
                    g = gelu(v_all[e * 16:(e + 1) * 16, :])
                    gt[i % 2, e * 16:(e + 1) * 16, :] = g.astype(BF16)
                    an = g[8:16, W - 128:W] if an is None else an + g[8:16, W - 128:W]
                if ANCH:
                    anchor(an, z)

            def t2(g, xb, oslot, row, hooks=()):
                t2_(g, xb, oslot, row, hooks)
                done.add(row)
                for lo, hi in PIECES:
                    if lo <= row < hi and all(r in done for r in range(lo, hi)):
                        opiece(cur_c[0], oslot, lo, hi).start()

            done = set()
            cur_c = [None]

            def t2_(g, xb, oslot, row, hooks=()):
                y = jnp.dot(_b(w2s[...]), g, preferred_element_type=F32)
                bb = jnp.concatenate([b2b[...]] * NT, axis=1)
                xr[xb + row] = (y + (bb + xr[xb + row].astype(F32))).astype(BF16)
                for t, z, fn in hooks:
                    an = y[0:8, t * 128:(t + 1) * 128]
                    for cg in range(1, C // 8):
                        an = an + y[cg * 8:(cg + 1) * 8, t * 128:(t + 1) * 128]
                    anchor(an, z)
                    fn()

            def adv(s_, n):
                s_ = s_ + n
                return jnp.where(s_ >= XS, s_ - XS, s_)

            def chunk2(c, xslot, z):
                oslot = xslot
                done.clear()
                cur_c[0] = c
                xb = xslot * CH
                c2 = jnp.minimum(c + 1, NCH - 1)
                xb2 = jnp.where(c + 1 < NCH, adv(xslot, 1), xslot) * CH

                def t2s(i, hooks=()):
                    t2(hst[c * NS + i], xb, oslot, STO[i], hooks)

                def t0n(i, cg0, cg1):
                    if i < NR:
                        t0(c, xb, i, cg0, cg1)
                    else:
                        t0(c2, xb2, i - NR, cg0, cg1)

                si = 0
                for i in range(NF):
                    t2s(si)
                    si += 1
                cuts = [p[0] for p in PARTS] + [NCG]
                assert NR == 7
                for i in range(NR):
                    t1(i, z, lambda lo, hi: [unp(xb2, r, lo, hi) for r in PROD[i]])
                    t0n(i + 2, 0, cuts[0])
                    hk = {'a': [], 'b': []}
                    for pi, (lo, tag) in enumerate(PARTS):
                        hk[tag[0]].append((int(tag[1]), z, functools.partial(t0n, i + 2, lo, cuts[pi + 1])))
                    if i > 0:
                        t2(gt[(i - 1) % 2], xb, oslot, REC[i - 1], hk['a'])
                    else:
                        t2s(si, hk['a'])
                        si += 1
                    t2s(si, hk['b'])
                    si += 1
                t2(gt[(NR - 1) % 2], xb, oslot, REC[NR - 1])
                while si < NS:
                    t2s(si)
                    si += 1

            def body2(i, slot):
                c0 = i * NB2
                z = zs[0]
                for h in range(NB2):
                    chunk2(c0 + h, adv(slot, h), z)
                for h in range(NB2):
                    ps = adv(slot, XS - NB2 + h)

                    @pl.when(i > 0)
                    def _():
                        owait(c0 - NB2 + h, ps)

                    @pl.when(c0 + P2PRE + h < NCH)
                    def _():
                        xcopy(c0 + P2PRE + h, ps).start()
                for h in range(NB2):
                    @pl.when(c0 + NB2 + 1 + h < NCH)
                    def _():
                        xcopy(c0 + NB2 + 1 + h, adv(slot, NB2 + 1 + h)).wait()
                return adv(slot, NB2)

            s0 = NCH % XS
            if do2:
                jax.lax.fori_loop(0, NCH // NB2, body2, s0)
                for c in range(NCH - NB2, NCH):
                    owait(c, (s0 + c) % XS)
            else:
                for c in range(NB2 + 1, P2PRE):
                    xcopy(c, (s0 + c) % XS).wait()

        pl.run_scoped(pass2, pltpu.VMEM((2, E, W), BF16))

    @jax.jit
    def f(x, dw, w1, w2, grn_gamma, grn_beta):
        xt = jnp.transpose(x, (0, 1, 3, 2)).reshape(H, C, W)
        w2t = jnp.transpose(w2)
        hbm = pl.BlockSpec(memory_space=pl.ANY)
        out = pl.pallas_call(
            kernel,
            in_specs=[hbm] * 6,
            out_specs=pl.BlockSpec(memory_space=pl.ANY),
            out_shape=jax.ShapeDtypeStruct((H, C, W), BF16),
            scratch_shapes=[
                pltpu.VMEM((NCH * NS, E, W), BF16),
                pltpu.VMEM((NP + RPAD, 8, 128), F32),
                pltpu.VMEM((XS * CH + 1, C, W), BF16),
                pltpu.VMEM((10, C, 128), F32),
                pltpu.VMEM((E // 2, 128), U32),
                pltpu.VMEM((C // 2, E), U32),
                pltpu.VMEM((C, 128), F32),
                pltpu.VMEM((E, 128), F32),
                pltpu.VMEM((NR, C, W), BF16),
                pltpu.VMEM(((NR + 2) * C, W), F32),
                pltpu.VMEM((3, 3, C), BF16),
                pltpu.VMEM((C, E), BF16),
                pltpu.VMEM((C, E), BF16),
                pltpu.VMEM((E,), BF16),
                pltpu.VMEM((E,), BF16),
                pltpu.SMEM((1,), jnp.int32),
                pltpu.SemaphoreType.DMA((XS,)),
                pltpu.SemaphoreType.DMA((XS,)),
                pltpu.SemaphoreType.DMA((5,)),
            ],
            compiler_params=pltpu.CompilerParams(vmem_limit_bytes=vmem_mb << 20, disable_bounds_checks=NOBC),
        )(xt, dw, w1, w2t, grn_gamma, grn_beta)
        return jnp.transpose(out.reshape(1, H, C, W), (0, 1, 3, 2))
    return f


pallas_standalone__modern_conv_block_convnext_v2__vision_kernel = build(**{})
```

```python
import functools
import math

import jax
import jax.numpy as jnp
import jax.experimental.pallas as pl
import jax.experimental.pallas.tpu as pltpu

F32 = jnp.float32
BF16 = jnp.bfloat16
U32 = jnp.uint32

_C0 = math.sqrt(2.0 / math.pi)
_KAPPA = (_C0 * 0.044715) ** (1.0 / 3.0)
_A = _C0 / _KAPPA
_GS = 2.0 * _KAPPA


def _u(x):
    return pltpu.bitcast(x, U32)


def _b(x):
    return pltpu.bitcast(x, BF16)


def build(NBQ=2, XS=7, NB1=2, NB2=2, NR=7, NF=0, PARTS=((6, 'a3'),), ANCH=True, XA=(0, 128, 256), PROD=((0, 1), (2,), (3,), (4,), (5,), (6,), (7, 8)), QS=(2, 3, 0, 4, 5, 1), PEARLY=0, PRE1=16, PRE2=20,
          PIECES=((0, 4), (8, 12), (4, 6), (12, 14), (6, 8), (14, 16)), NOBC=True, vmem_mb=128, do1=True, do2=True):
    H, W, C, E = 512, 512, 96, 384
    NT = W // 128
    NQ = C // 16
    CH = 16
    NCH = H // CH
    U = CH // 2
    NP = H // 2
    REC = list(range(1, NR + 1))
    STO = [r for r in range(CH) if r not in REC]
    NS = len(STO)
    ZROW = XS * CH
    P2PRE = XS - NB2
    ND = 4
    NRS = NR // 2 + 1
    NG = NQ + NBQ
    CROWS = NBQ * 8 + (NQ - NBQ) * 16

    def kernel(x_hbm, dw_hbm, w1_hbm, w2t_hbm, gam_hbm, bet_hbm,
               o_hbm,
               hst, rst, xr, dwb, w1t, w2s, b2b, acc, xn2, wk,
               dw_ref, w1_ref, w2t_ref, gam_ref, bet_ref, zs, xsem, osem, wsem):

        def xcopy(c, slot):
            return pltpu.make_async_copy(
                x_hbm.at[pl.ds(c * CH, CH)], xr.at[pl.ds(slot * CH, CH)], xsem.at[slot])

        def nxt(s, n):
            return jnp.where(s == n - 1, 0, s + 1)

        def xpart(lo, hi, sem):
            return pltpu.make_async_copy(x_hbm.at[pl.ds(lo, hi - lo)], xr.at[pl.ds(lo, hi - lo)], xsem.at[sem])

        wcp = [pltpu.make_async_copy(src, dst, wsem.at[i]) for i, (src, dst) in enumerate(
            [(dw_hbm, dw_ref), (w1_hbm, w1_ref), (w2t_hbm, w2t_ref), (gam_hbm, gam_ref), (bet_hbm, bet_ref)])]
        wcp[0].start()
        wcp[1].start()
        xpart(0, 5, 1).start()
        xpart(5, CH + 5, 0).start()
        for cp in wcp[2:]:
            cp.start()
        zs[0] = 0
        wcp[0].wait()
        wcp[1].wait()

        def tiles(v):
            return [v[:, t * 128:(t + 1) * 128] for t in range(NT)]

        def mm1(xp, e0=0, e1=E):
            return jnp.dot(_b(w1t[e0 // 2:e1 // 2, :]), xp, preferred_element_type=F32)

        def padk(xn):
            return jnp.concatenate([xn, jnp.zeros((128 - C, W), xn.dtype)], axis=0)

        def gelu(v):
            z = v * (v * v + _A)
            return v * (jnp.tanh(z) + 1.0)

        lane = jax.lax.broadcasted_iota(jnp.int32, (8, 128), 1)
        m0 = lane == 0
        m127 = lane == 127

        NCG = C // 8
        NX = NR + 2

        def unp(xb, r, lo=0, hi=C):
            wk[r * C + lo:r * C + hi, :] = xr[xb + r, lo:hi, :].astype(F32)

        def t0(c, xb, i, cg0, cg1):
            r = REC[i]
            rs = [rst[c * NRS + r // 2, (r % 2) * 4 + t:(r % 2) * 4 + t + 1, :] for t in range(NT)]
            for cg in range(cg0, cg1):
                sl = slice(cg * 8, cg * 8 + 8)
                xs = [tiles(wk[(r - 1 + a) * C + cg * 8:(r - 1 + a) * C + cg * 8 + 8, :]) for a in range(3)]
                cs = []
                for b in range(3):
                    ws = [dwb[a * 3 + b, sl, :] for a in range(3)]
                    cs.append([ws[0] * xs[0][t] + ws[1] * xs[1][t] + ws[2] * xs[2][t] for t in range(NT)])
                rl = [pltpu.roll(cs[0][t], 1, 1) for t in range(NT)]
                rg = [pltpu.roll(cs[2][t], 127, 1) for t in range(NT)]
                row = []
                for t in range(NT):
                    left = jnp.where(m0, rl[t - 1] if t > 0 else 0.0, rl[t])
                    right = jnp.where(m127, rg[t + 1] if t < NT - 1 else 0.0, rg[t])
                    row.append((cs[1][t] + (left + right)) * rs[t])
                xn2[i, sl, :] = jnp.concatenate(row, axis=1).astype(BF16)

        def pass1(la, lb, cw, cbuf, stat, nrm):
            rr = jax.lax.broadcasted_iota(jnp.int32, (C, C), 0)
            cc = jax.lax.broadcasted_iota(jnp.int32, (C, C), 1)
            for a in range(3):
                for b in range(3):
                    row = dw_ref[a, b:b + 1, :].astype(F32)
                    d = jnp.where(rr == cc, jnp.broadcast_to(row, (C, C)), 0.0)
                    col = jnp.sum(d, axis=1, keepdims=True)
                    dwb[a * 3 + b] = jnp.broadcast_to(col, (C, 128))
            r16 = jax.lax.broadcasted_iota(jnp.int32, (16, 128), 0)
            c16 = jax.lax.broadcasted_iota(jnp.int32, (16, 128), 1)
            for q in range(NQ):
                ta, tb = [], []
                sf = slice(q * 16, q * 16 + 16)
                for o in range(2):
                    ma = jnp.zeros((16, 128), F32)
                    mb = jnp.zeros((16, 128), F32)
                    for a in range(3):
                        ma = jnp.where(c16 == (a + o) * 16 + r16, dwb[a * 3 + 0, sf, :], ma)
                        ma = jnp.where(c16 == (4 + a + o) * 16 + r16, dwb[a * 3 + 2, sf, :], ma)
                        mb = jnp.where(c16 == (a + o) * 16 + r16, dwb[a * 3 + 1, sf, :], mb)
                    ta.append(ma)
                    tb.append(mb)
                la[q] = _u(jnp.concatenate(ta, axis=0).astype(BF16))
                lb[q] = _u(jnp.concatenate(tb, axis=0).astype(BF16))
            re = jax.lax.broadcasted_iota(jnp.int32, (E, E), 0)
            ce = jax.lax.broadcasted_iota(jnp.int32, (E, E), 1)
            eye = jnp.where(re == ce, 1.0, 0.0).astype(BF16)
            w1f = w1_ref[...].astype(F32)
            w1c = (w1f - jnp.mean(w1f, axis=0, keepdims=True)).astype(BF16).astype(F32)
            aw = jnp.abs(w1c)
            small = aw <= jnp.maximum(0.3 * jnp.mean(aw, axis=0, keepdims=True), jnp.min(aw, axis=0, keepdims=True))
            cnt = jnp.sum(jnp.where(small, 1.0, 0.0), axis=0, keepdims=True)
            w1c = jnp.where(small, w1c - jnp.sum(w1c, axis=0, keepdims=True) / cnt, w1c).astype(BF16)
            w1p = jnp.concatenate([w1c, jnp.zeros((128 - C, E), BF16)], axis=0)
            t = jax.lax.dot_general(eye, w1p, (((1,), (1,)), ((), ())),
                                    preferred_element_type=F32)
            w1t[...] = _u(t.astype(BF16))
            acc[...] = jnp.zeros_like(acc)
            xr[ZROW] = jnp.zeros((C, W), BF16)

            sub = jax.lax.broadcasted_iota(jnp.int32, (8, 128), 0)

            def butterfly(vs):
                for d in (1, 2, 4):
                    mk = (sub % (2 * d)) < d
                    vs = [jnp.where(mk, vs[i], vs[i + 1]) + pltpu.roll(jnp.where(mk, vs[i + 1], vs[i]), d, 0)
                          for i in range(0, len(vs), 2)]
                return vs[0]

            def rlr(par, n, lr, q):
                o = ((par * 2 + n) * 2 + lr) * (C // 2) + q * 8
                return slice(o, o + 8)

            def rc(par, n, q):
                o = 2 * ND * C + (par * 2 + n) * CROWS
                if q < NBQ:
                    return slice(o + q * 8, o + q * 8 + 8)
                o += NBQ * 8 + (q - NBQ) * 16
                return slice(o, o + 16)

            def units(us, e0=0, e1=E):
                xs = [cbuf[d, o, :, t * 128:(t + 1) * 128] * nrm[d, o * 4 + t:o * 4 + t + 1, :]
                      for d, o, t, _ in us]
                xn = xs[0] if len(xs) == 1 else jnp.concatenate(xs, axis=1)
                xp = jnp.concatenate([xn, jnp.zeros((128 - C, 128 * len(us)), F32)], axis=0).astype(BF16)
                v_all = mm1(xp, e0, e1)
                spans = []
                i = 0
                while i < len(us):
                    d, o, t, h = us[i]
                    n = 2 if (i + 1 < len(us) and t % 2 == 0 and us[i + 1][:3] == (d, o, t + 1)) else 1
                    if h is not None:
                        spans.append((i, n, t, h))
                    i += n
                for e in range(e0 // 16, e1 // 16):
                    g = gelu(v_all[e * 16 - e0:(e + 1) * 16 - e0, :])
                    g2 = g * g
                    a = g2[:, 0:128]
                    for i in range(1, len(us)):
                        a = a + g2[:, i * 128:(i + 1) * 128]
                    acc[e * 16:(e + 1) * 16, :] += a
                    for i, n, t, h in spans:
                        hst[h, e * 16:(e + 1) * 16, t * 128:(t + n) * 128] = (
                            g[:, i * 128:(i + n) * 128].astype(BF16))

            def prep(par, rows, q):
                zero = jnp.zeros((8, 128), U32)
                sf = slice(q * 16, q * 16 + 16)
                for n in range(2):
                    p = _u(xr[rows[n], sf, :])
                    pt = tiles(p)
                    rl = [pltpu.roll(pt[t], 1, 1) for t in range(NT)]
                    rg = [pltpu.roll(pt[t], 127, 1) for t in range(NT)]
                    cw[rlr(par, n, 0, q), :] = jnp.concatenate(
                        [jnp.where(m0, rl[t - 1] if t > 0 else zero, rl[t]) for t in range(NT)], axis=1)
                    cw[rlr(par, n, 1, q), :] = jnp.concatenate(
                        [jnp.where(m127, rg[t + 1] if t < NT - 1 else zero, rg[t]) for t in range(NT)], axis=1)
                    if q < NBQ:
                        cw[rc(par, n, q), :] = p
                    else:
                        cw[rc(par, n, q), :] = _u(_b(p).astype(F32))

            def group(d, t, kidx):
                lt = slice(t * 128, (t + 1) * 128)
                s1 = [None, None]
                s2 = [None, None]
                rows = [((d - 1) % ND, 0), ((d - 1) % ND, 1), (d, 0), (d, 1)]
                for q in QS:
                    sf = slice(q * 16, q * 16 + 16)
                    rhs = [cw[rlr(a, n, 0, q), lt] for a, n in rows] + [cw[rlr(a, n, 1, q), lt] for a, n in rows]
                    lhs = _b(la[q])
                    if q < NBQ:
                        rb = [cw[rc(a, n, q), lt] for a, n in rows] + [jnp.zeros((32, 128), U32)]
                        ca = jnp.dot(lhs, _b(jnp.concatenate(rhs, axis=0)), preferred_element_type=F32)
                        yield
                        ca = ca + jnp.dot(_b(lb[q]), _b(jnp.concatenate(rb, axis=0)),
                                          preferred_element_type=F32)
                        cs = [ca[o * 16:(o + 1) * 16, :] for o in range(2)]
                    else:
                        ca = jnp.dot(lhs, _b(jnp.concatenate(rhs, axis=0)), preferred_element_type=F32)
                        cf = [pltpu.bitcast(cw[rc(a, n, q), lt], F32) for a, n in rows]
                        ws = [dwb[a * 3 + 1, sf, :] for a in range(3)]
                        cs = [(ca[o * 16:(o + 1) * 16, :] + ws[0] * cf[o]) + (ws[1] * cf[o + 1] + ws[2] * cf[o + 2])
                              for o in range(2)]
                    for o in range(2):
                        c = cs[o]
                        cbuf[d, o, sf, lt] = c
                        a = c[0:8] + c[8:16]
                        b = c[0:8] * c[0:8] + c[8:16] * c[8:16]
                        s1[o] = a if s1[o] is None else s1[o] + a
                        s2[o] = b if s2[o] is None else s2[o] + b
                    if q == QS[-1]:
                        for o in range(2):
                            stat[d % 2, o, 0, :, lt] = s1[o]
                            stat[d % 2, o, 1, :, lt] = s2[o]
                        if t == NT - 1:
                            m = butterfly(tiles(stat[d % 2, 0, 0]) + tiles(stat[d % 2, 1, 0])) * (1.0 / C)
                            q2 = butterfly(tiles(stat[d % 2, 0, 1]) + tiles(stat[d % 2, 1, 1])) * (1.0 / C)
                            var = jnp.maximum(q2 - m * m, 0.0)
                            rs = jax.lax.rsqrt(var + 1e-5) * _KAPPA
                            nrm[d] = rs
                            if kidx is not None:
                                rst[kidx] = rs
                    yield

            def hslot(chunk, r):
                return None if r in REC else chunk * NS + STO.index(r)

            def adv(s_, n):
                s_ = s_ + n
                return jnp.where(s_ >= XS, s_ - XS, s_)

            def body1(nb, c0, slot):
                npair = nb * U
                base = [adv(slot, h) * CH for h in range(nb + 1)]
                last = c0 + nb == NCH

                def xrow(r):
                    if r < nb * CH:
                        return base[r // CH] + r % CH
                    return jnp.where(last, ZROW, base[nb] + (r - nb * CH))

                def conv_stream():
                    for gam in range(4 * npair):
                        p, t = 1 + (gam + 2) // 4, (gam + 2) % 4
                        pp, tt = 1 + (gam + 2 + PEARLY) // 4, (gam + 2 + PEARLY) % 4
                        if tt == 0 and pp <= npair + 1:
                            for q in QS:
                                prep(pp % ND, (xrow(2 * pp + 1), xrow(2 * pp + 2)), q)
                        yield from group(p % ND, t, (c0 + p // U) * NRS + p % U if p % U < NRS else None)

                us = [((r // 2) % ND, r % 2, t, hslot(c0 + r // CH, r % CH))
                      for r in range(2 * npair) for t in range(NT)]
                cs = conv_stream()

                def pull(n):
                    for _ in range(n):
                        next(cs, None)

                nfull = len(us) // 3
                pre = PRE1 if nb == 1 else PRE2
                extra = 4 * npair * NG - pre - 12 * (nfull - len(us) % 3)
                assert extra >= 0 and extra % 3 == 0, extra
                nw = extra // 3
                pull(pre)
                for i in range(nfull):
                    units(us[3 * i:3 * i + 3])
                    pull(12 + 3 * ((i + 1) * nw // (nfull - 2) - i * nw // (nfull - 2) if i < nfull - 2 else 0))
                rest = us[3 * nfull:]
                assert next(cs, 'done') == 'done'
                for u in rest:
                    units([u])

                for h in range(nb):
                    cn = c0 + h + XS
                    if XS + h + c0_max(nb) < NCH + P2PRE:
                        xcopy(jnp.where(cn < NCH, cn, cn - NCH), adv(slot, h)).start()
                    else:
                        @pl.when(cn < NCH + P2PRE)
                        def _():
                            xcopy(jnp.where(cn < NCH, cn, cn - NCH), adv(slot, h)).start()

            def c0_max(nb):
                return NCH - nb

            def step1(i, slot):
                def one():
                    body1(1, jnp.where(i == 0, 0, NCH - 1), slot)

                    @pl.when(i == 0)
                    def _():
                        xpart(CH + 5, 2 * CH, 1).wait()
                        xcopy(2, 2).wait()
                        xcopy(3, 3).wait()
                    return adv(slot, 1)

                def two():
                    c0 = 2 * i - 1
                    body1(2, c0, slot)
                    for h in (3, 4):
                        @pl.when(c0 + h < NCH)
                        def _():
                            xcopy(c0 + h, adv(slot, h)).wait()
                    return adv(slot, 2)
                return jax.lax.cond(jnp.logical_or(i == 0, i == NCH // 2), one, two)

            def step1s(kk, slot):
                body1(1, kk, slot)

                @pl.when(kk == 0)
                def _():
                    xpart(CH + 5, 2 * CH, 1).wait()

                @pl.when(kk + 2 < NCH)
                def _():
                    xcopy(kk + 2, adv(slot, 2)).wait()
                return adv(slot, 1)

            xpart(0, 5, 1).wait()
            assert PEARLY <= 2
            for p, rows in ((-1, (ZROW, 0)), (0, (1, 2)), (1, (3, 4))):
                for q in QS:
                    prep(p % ND, rows, q)
            for p, t in ((0, 0), (0, 1), (0, 2), (0, 3), (1, 0), (1, 1)):
                for _ in group(p, t, 0):
                    pass
            xpart(5, CH + 5, 0).wait()
            xpart(CH + 5, 2 * CH, 1).start()
            for c in range(2, XS):
                xcopy(c, c).start()
            for cp in wcp[2:]:
                cp.wait()
            if do1:
                if NB1 == 2:
                    jax.lax.fori_loop(0, NCH // 2 + 1, step1, 0)
                else:
                    jax.lax.fori_loop(0, NCH, step1s, 0)
                for c in range(NB2 + 1):
                    xcopy(c, (NCH + c) % XS).wait()
            else:
                xpart(CH + 5, 2 * CH, 1).wait()
                for c in range(2, XS):
                    xcopy(c, c).wait()
                for c in range(P2PRE):
                    xcopy(c, (NCH + c) % XS).start()
                for c in range(NB2 + 1):
                    xcopy(c, (NCH + c) % XS).wait()

        pl.run_scoped(
            pass1,
            pltpu.VMEM((NQ, 16, 128), U32),
            pltpu.VMEM((NQ, 16, 128), U32),
            pltpu.VMEM((2 * ND * (C + CROWS), W), U32),
            pltpu.VMEM((ND, 2, C, W), F32),
            pltpu.VMEM((2, 2, 2, 8, W), F32),
            pltpu.VMEM((ND, 8, 128), F32),
        )

        for r in range(NX):
            unp((NCH % XS) * CH, r)
        for i in range(2):
            t0(0, (NCH % XS) * CH, i, 0, NCG)

        a = jnp.transpose(acc[...])
        ssq = jnp.sum(a, axis=0, keepdims=True) * (1.0 / (_GS * _GS))
        gx = jnp.sqrt(ssq + 1e-6)
        nx = gx / (jnp.mean(gx, axis=1, keepdims=True) + 1e-6)
        s = (gam_ref[...].astype(F32).reshape(1, E) * nx + 1.0) * (1.0 / _GS)
        w2f = w2t_ref[...].astype(F32)
        w2s[...] = _u((w2f * s).astype(BF16))
        b = jnp.sum(w2f * bet_ref[...].astype(F32).reshape(1, E), axis=1, keepdims=True)
        b2b[...] = jnp.broadcast_to(b, (C, 128))

        def pass2(gt):
            def opiece(c, slot, lo, hi):
                return pltpu.make_async_copy(
                    xr.at[pl.ds(slot * CH + lo, hi - lo)], o_hbm.at[pl.ds(c * CH + lo, hi - lo)], osem.at[slot])

            def owait(c, slot):
                for lo, hi in PIECES:
                    opiece(c, slot, lo, hi).wait()

            def anchor(v, z):
                dwb[9 + z, 0:8, :] = v

            def t1(i, z, fn):
                v_all = mm1(padk(xn2[i]))
                for k, xa in enumerate(XA):
                    xr[ZROW + z, 0:8, 0:128] = v_all[xa:xa + 8, 0:128].astype(BF16)
                    fn(k * C // len(XA), (k + 1) * C // len(XA))
                an = None
                for e in range(E // 16):
                    g = gelu(v_all[e * 16:(e + 1) * 16, :])
                    gt[i % 2, e * 16:(e + 1) * 16, :] = g.astype(BF16)
                    an = g[8:16, W - 128:W] if an is None else an + g[8:16, W - 128:W]
                if ANCH:
                    anchor(an, z)

            def t2(g, xb, oslot, row, hooks=()):
                t2_(g, xb, oslot, row, hooks)
                done.add(row)
                for lo, hi in PIECES:
                    if lo <= row < hi and all(r in done for r in range(lo, hi)):
                        opiece(cur_c[0], oslot, lo, hi).start()

            done = set()
            cur_c = [None]

            def t2_(g, xb, oslot, row, hooks=()):
                y = jnp.dot(_b(w2s[...]), g, preferred_element_type=F32)
                bb = jnp.concatenate([b2b[...]] * NT, axis=1)
                xr[xb + row] = (y + (bb + xr[xb + row].astype(F32))).astype(BF16)
                for t, z, fn in hooks:
                    an = y[0:8, t * 128:(t + 1) * 128]
                    for cg in range(1, C // 8):
                        an = an + y[cg * 8:(cg + 1) * 8, t * 128:(t + 1) * 128]
                    anchor(an, z)
                    fn()

            def adv(s_, n):
                s_ = s_ + n
                return jnp.where(s_ >= XS, s_ - XS, s_)

            def chunk2(c, xslot, z):
                oslot = xslot
                done.clear()
                cur_c[0] = c
                xb = xslot * CH
                c2 = jnp.minimum(c + 1, NCH - 1)
                xb2 = jnp.where(c + 1 < NCH, adv(xslot, 1), xslot) * CH

                def t2s(i, hooks=()):
                    t2(hst[c * NS + i], xb, oslot, STO[i], hooks)

                def t0n(i, cg0, cg1):
                    if i < NR:
                        t0(c, xb, i, cg0, cg1)
                    else:
                        t0(c2, xb2, i - NR, cg0, cg1)

                si = 0
                for i in range(NF):
                    t2s(si)
                    si += 1
                cuts = [p[0] for p in PARTS] + [NCG]
                assert NR == 7
                for i in range(NR):
                    t1(i, z, lambda lo, hi: [unp(xb2, r, lo, hi) for r in PROD[i]])
                    t0n(i + 2, 0, cuts[0])
                    hk = {'a': [], 'b': []}
                    for pi, (lo, tag) in enumerate(PARTS):
                        hk[tag[0]].append((int(tag[1]), z, functools.partial(t0n, i + 2, lo, cuts[pi + 1])))
                    if i > 0:
                        t2(gt[(i - 1) % 2], xb, oslot, REC[i - 1], hk['a'])
                    else:
                        t2s(si, hk['a'])
                        si += 1
                    t2s(si, hk['b'])
                    si += 1
                t2(gt[(NR - 1) % 2], xb, oslot, REC[NR - 1])
                while si < NS:
                    t2s(si)
                    si += 1

            def body2(i, slot):
                c0 = i * NB2
                z = zs[0]
                for h in range(NB2):
                    chunk2(c0 + h, adv(slot, h), z)
                for h in range(NB2):
                    ps = adv(slot, XS - NB2 + h)

                    @pl.when(i > 0)
                    def _():
                        owait(c0 - NB2 + h, ps)

                    @pl.when(c0 + P2PRE + h < NCH)
                    def _():
                        xcopy(c0 + P2PRE + h, ps).start()
                for h in range(NB2):
                    @pl.when(c0 + NB2 + 1 + h < NCH)
                    def _():
                        xcopy(c0 + NB2 + 1 + h, adv(slot, NB2 + 1 + h)).wait()
                return adv(slot, NB2)

            s0 = NCH % XS
            if do2:
                jax.lax.fori_loop(0, NCH // NB2, body2, s0)
                for c in range(NCH - NB2, NCH):
                    owait(c, (s0 + c) % XS)
            else:
                for c in range(NB2 + 1, P2PRE):
                    xcopy(c, (s0 + c) % XS).wait()

        pl.run_scoped(pass2, pltpu.VMEM((2, E, W), BF16))

    @jax.jit
    def f(x, dw, w1, w2, grn_gamma, grn_beta):
        xt = jnp.transpose(x, (0, 1, 3, 2)).reshape(H, C, W)
        w2t = jnp.transpose(w2)
        hbm = pl.BlockSpec(memory_space=pl.ANY)
        out = pl.pallas_call(
            kernel,
            in_specs=[hbm] * 6,
            out_specs=pl.BlockSpec(memory_space=pl.ANY),
            out_shape=jax.ShapeDtypeStruct((H, C, W), BF16),
            scratch_shapes=[
                pltpu.VMEM((NCH * NS, E, W), BF16),
                pltpu.VMEM(((NCH + 1) * NRS, 8, 128), F32),
                pltpu.VMEM((XS * CH + 1, C, W), BF16),
                pltpu.VMEM((10, C, 128), F32),
                pltpu.VMEM((E // 2, 128), U32),
                pltpu.VMEM((C // 2, E), U32),
                pltpu.VMEM((C, 128), F32),
                pltpu.VMEM((E, 128), F32),
                pltpu.VMEM((NR, C, W), BF16),
                pltpu.VMEM(((NR + 2) * C, W), F32),
                pltpu.VMEM((3, 3, C), BF16),
                pltpu.VMEM((C, E), BF16),
                pltpu.VMEM((C, E), BF16),
                pltpu.VMEM((E,), BF16),
                pltpu.VMEM((E,), BF16),
                pltpu.SMEM((1,), jnp.int32),
                pltpu.SemaphoreType.DMA((XS,)),
                pltpu.SemaphoreType.DMA((XS,)),
                pltpu.SemaphoreType.DMA((5,)),
            ],
            compiler_params=pltpu.CompilerParams(vmem_limit_bytes=vmem_mb << 20, disable_bounds_checks=NOBC),
        )(xt, dw, w1, w2t, grn_gamma, grn_beta)
        return jnp.transpose(out.reshape(1, H, C, W), (0, 1, 3, 2))
    return f


pallas_standalone__modern_conv_block_convnext_v2__vision_kernel = build(**{})
```

```python
import functools
import math

import jax
import jax.numpy as jnp
import jax.experimental.pallas as pl
import jax.experimental.pallas.tpu as pltpu

F32 = jnp.float32
BF16 = jnp.bfloat16
U32 = jnp.uint32

_C0 = math.sqrt(2.0 / math.pi)
_KAPPA = (_C0 * 0.044715) ** (1.0 / 3.0)
_A = _C0 / _KAPPA
_GS = 2.0 * _KAPPA


def _u(x):
    return pltpu.bitcast(x, U32)


def _b(x):
    return pltpu.bitcast(x, BF16)


def build(NBQ=2, XS=7, NB2=2, QS=(2, 3, 0, 4, 5, 1), PRE=12, LEFT=240, SPLIT=6, STILE=2, XA=(48, 176, 304),
          PROD=((0, 1), (2,), (3,), (4,), (5,), (6,), (7, 8)),
          PIECES=((0, 4), (8, 12), (4, 6), (12, 14), (6, 8), (14, 16))):
    H, W, C, E = 512, 512, 96, 384
    NT = W // 128
    NQ = C // 16
    NCG = C // 8
    CH = 16
    NCH = H // CH
    U = CH // 2
    NR = 7
    REC = list(range(1, NR + 1))
    STO = [r for r in range(CH) if r not in REC]
    NS = len(STO)
    NX = NR + 2
    NRS = NR // 2 + 1
    ZROW = XS * CH
    P2PRE = XS - NB2
    ND = 4
    CROWS = NBQ * 8 + (NQ - NBQ) * 16

    def kernel(x_hbm, dw_hbm, w1_hbm, w2t_hbm, gam_hbm, bet_hbm,
               o_hbm,
               hst, xr, wk, xn2, rst, dwb, w1t, acc, b2b, w2s,
               dw_ref, w1_ref, w2t_ref, gam_ref, bet_ref, zs, xsem, osem, wsem):

        def xcopy(c, slot):
            return pltpu.make_async_copy(
                x_hbm.at[pl.ds(c * CH, CH)], xr.at[pl.ds(slot * CH, CH)], xsem.at[slot])

        def xpart(lo, hi, sem):
            return pltpu.make_async_copy(x_hbm.at[pl.ds(lo, hi - lo)], xr.at[pl.ds(lo, hi - lo)], xsem.at[sem])

        def adv(s, n):
            s = s + n
            return jnp.where(s >= XS, s - XS, s)

        wcp = [pltpu.make_async_copy(src, dst, wsem.at[i]) for i, (src, dst) in enumerate(
            [(dw_hbm, dw_ref), (w1_hbm, w1_ref), (w2t_hbm, w2t_ref), (gam_hbm, gam_ref), (bet_hbm, bet_ref)])]
        wcp[0].start()
        wcp[1].start()
        xpart(0, 5, 1).start()
        xpart(5, CH + 5, 0).start()
        for cp in wcp[2:]:
            cp.start()
        zs[0] = 0
        wcp[0].wait()
        wcp[1].wait()
        xpart(0, 5, 1).wait()

        def tiles(v):
            return [v[:, t * 128:(t + 1) * 128] for t in range(NT)]

        def mm1(xp, e0=0, e1=E):
            return jnp.dot(_b(w1t[e0 // 2:e1 // 2, :]), xp, preferred_element_type=F32)

        def gelu(v):
            z = v * (v * v + _A)
            return v * (jnp.tanh(z) + 1.0)

        lane = jax.lax.broadcasted_iota(jnp.int32, (8, 128), 1)
        m0 = lane == 0
        m127 = lane == 127

        def unp(xb, r, lo=0, hi=C):
            wk[r * C + lo:r * C + hi, :] = xr[xb + r, lo:hi, :].astype(F32)

        def t0(c, i, cg0, cg1):
            r = REC[i]
            rs = [rst[c * NRS + r // 2, (r % 2) * 4 + t:(r % 2) * 4 + t + 1, :] for t in range(NT)]
            for cg in range(cg0, cg1):
                sl = slice(cg * 8, cg * 8 + 8)
                xs = [tiles(wk[(r - 1 + a) * C + cg * 8:(r - 1 + a) * C + cg * 8 + 8, :]) for a in range(3)]
                cs = []
                for b in range(3):
                    ws = [dwb[a * 3 + b, sl, :] for a in range(3)]
                    cs.append([ws[0] * xs[0][t] + ws[1] * xs[1][t] + ws[2] * xs[2][t] for t in range(NT)])
                rl = [pltpu.roll(cs[0][t], 1, 1) for t in range(NT)]
                rg = [pltpu.roll(cs[2][t], 127, 1) for t in range(NT)]
                row = []
                for t in range(NT):
                    left = jnp.where(m0, rl[t - 1] if t > 0 else 0.0, rl[t])
                    right = jnp.where(m127, rg[t + 1] if t < NT - 1 else 0.0, rg[t])
                    row.append((cs[1][t] + (left + right)) * rs[t])
                xn2[i, sl, :] = jnp.concatenate(row, axis=1).astype(BF16)

        def pass1(la, lb, cw, cbuf, stat, nrm):
            rr = jax.lax.broadcasted_iota(jnp.int32, (C, C), 0)
            cc = jax.lax.broadcasted_iota(jnp.int32, (C, C), 1)
            for a in range(3):
                for b in range(3):
                    row = dw_ref[a, b:b + 1, :].astype(F32)
                    d = jnp.where(rr == cc, jnp.broadcast_to(row, (C, C)), 0.0)
                    col = jnp.sum(d, axis=1, keepdims=True)
                    dwb[a * 3 + b] = jnp.broadcast_to(col, (C, 128))
            r16 = jax.lax.broadcasted_iota(jnp.int32, (16, 128), 0)
            c16 = jax.lax.broadcasted_iota(jnp.int32, (16, 128), 1)
            for q in range(NQ):
                ta, tb = [], []
                sf = slice(q * 16, q * 16 + 16)
                for o in range(2):
                    ma = jnp.zeros((16, 128), F32)
                    mb = jnp.zeros((16, 128), F32)
                    for a in range(3):
                        ma = jnp.where(c16 == (a + o) * 16 + r16, dwb[a * 3 + 0, sf, :], ma)
                        ma = jnp.where(c16 == (4 + a + o) * 16 + r16, dwb[a * 3 + 2, sf, :], ma)
                        mb = jnp.where(c16 == (a + o) * 16 + r16, dwb[a * 3 + 1, sf, :], mb)
                    ta.append(ma)
                    tb.append(mb)
                la[q] = _u(jnp.concatenate(ta, axis=0).astype(BF16))
                lb[q] = _u(jnp.concatenate(tb, axis=0).astype(BF16))
            re = jax.lax.broadcasted_iota(jnp.int32, (E, E), 0)
            ce = jax.lax.broadcasted_iota(jnp.int32, (E, E), 1)
            eye = jnp.where(re == ce, 1.0, 0.0).astype(BF16)
            w1f = w1_ref[...].astype(F32)
            w1c = (w1f - jnp.mean(w1f, axis=0, keepdims=True)).astype(BF16).astype(F32)
            aw = jnp.abs(w1c)
            small = aw <= jnp.maximum(0.3 * jnp.mean(aw, axis=0, keepdims=True), jnp.min(aw, axis=0, keepdims=True))
            cnt = jnp.sum(jnp.where(small, 1.0, 0.0), axis=0, keepdims=True)
            w1c = jnp.where(small, w1c - jnp.sum(w1c, axis=0, keepdims=True) / cnt, w1c).astype(BF16)
            w1p = jnp.concatenate([w1c, jnp.zeros((128 - C, E), BF16)], axis=0)
            t = jax.lax.dot_general(eye, w1p, (((1,), (1,)), ((), ())),
                                    preferred_element_type=F32)
            w1t[...] = _u(t.astype(BF16))
            acc[...] = jnp.zeros_like(acc)
            for i in range(2 * ND):
                cw[i * C:i * C + C // 2, 0:128] = jnp.zeros((C // 2, 128), U32)
                cw[i * C + C // 2:(i + 1) * C, W - 128:W] = jnp.zeros((C // 2, 128), U32)
            xr[ZROW] = jnp.zeros((C, W), BF16)

            sub = jax.lax.broadcasted_iota(jnp.int32, (8, 128), 0)

            def butterfly(vs):
                for d in (1, 2, 4):
                    mk = (sub % (2 * d)) < d
                    vs = [jnp.where(mk, vs[i], vs[i + 1]) + pltpu.roll(jnp.where(mk, vs[i + 1], vs[i]), d, 0)
                          for i in range(0, len(vs), 2)]
                return vs[0]

            def rlr(d, n, lr, q):
                o = ((d * 2 + n) * 2 + lr) * (C // 2) + q * 8
                return slice(o, o + 8)

            def rc(d, n, q):
                o = 2 * ND * C + (d * 2 + n) * CROWS
                if q < NBQ:
                    return slice(o + q * 8, o + q * 8 + 8)
                o += NBQ * 8 + (q - NBQ) * 16
                return slice(o, o + 16)

            def units(us, e0=0, e1=E):
                xs = [cbuf[d, o, :, t * 128:(t + 1) * 128] * nrm[d, o * 4 + t:o * 4 + t + 1, :]
                      for d, o, t, _ in us]
                xn = xs[0] if len(xs) == 1 else jnp.concatenate(xs, axis=1)
                pad = jnp.zeros((128 - C, 128 * len(us)), F32)
                v_all = mm1(jnp.concatenate([xn, pad], axis=0).astype(BF16), e0, e1)
                spans = []
                i = 0
                while i < len(us):
                    d, o, t, h = us[i]
                    n = 2 if (i + 1 < len(us) and t % 2 == 0 and us[i + 1][:3] == (d, o, t + 1)) else 1
                    if h is not None:
                        spans.append((i, n, t, h))
                    i += n
                for e in range(e0 // 16, e1 // 16):
                    g = gelu(v_all[e * 16 - e0:(e + 1) * 16 - e0, :])
                    g2 = g * g
                    a = g2[:, 0:128]
                    for i in range(1, len(us)):
                        a = a + g2[:, i * 128:(i + 1) * 128]
                    acc[e * 16:(e + 1) * 16, :] += a
                    for i, n, t, h in spans:
                        hst[h, e * 16:(e + 1) * 16, t * 128:(t + n) * 128] = (
                            g[:, i * 128:(i + n) * 128].astype(BF16))

            def prep(d, rows, q):
                sf = slice(q * 16, q * 16 + 16)
                for n in range(2):
                    p = _u(xr[rows[n], sf, :])
                    pt = tiles(p)
                    rl = [pltpu.roll(pt[t], 1, 1) for t in range(NT)]
                    rg = [pltpu.roll(pt[t], 127, 1) for t in range(NT)]
                    for t in range(NT):
                        lt = slice(t * 128, (t + 1) * 128)
                        pltpu.store(cw.at[rlr(d, n, 0, q), lt], rl[t], mask=lane != 0)
                        pltpu.store(cw.at[rlr(d, n, 1, q), lt], rg[t], mask=lane != 127)
                        if t > 0:
                            pltpu.store(cw.at[rlr(d, n, 0, q), lt], rl[t - 1], mask=m0)
                        if t < NT - 1:
                            pltpu.store(cw.at[rlr(d, n, 1, q), lt], rg[t + 1], mask=m127)
                    if q < NBQ:
                        cw[rc(d, n, q), :] = p
                    else:
                        cw[rc(d, n, q), :] = _u(_b(p).astype(F32))

            def group(d, t, kidx):
                lt = slice(t * 128, (t + 1) * 128)
                s1 = [None, None]
                s2 = [None, None]
                rows = [((d - 1) % ND, 0), ((d - 1) % ND, 1), (d, 0), (d, 1)]
                for q in QS:
                    sf = slice(q * 16, q * 16 + 16)
                    rhs = [cw[rlr(a, n, 0, q), lt] for a, n in rows] + [cw[rlr(a, n, 1, q), lt] for a, n in rows]
                    ca = jnp.dot(_b(la[q]), _b(jnp.concatenate(rhs, axis=0)), preferred_element_type=F32)
                    if q < NBQ:
                        yield
                        rb = [cw[rc(a, n, q), lt] for a, n in rows] + [jnp.zeros((32, 128), U32)]
                        ca = ca + jnp.dot(_b(lb[q]), _b(jnp.concatenate(rb, axis=0)),
                                          preferred_element_type=F32)
                        cs = [ca[o * 16:(o + 1) * 16, :] for o in range(2)]
                    else:
                        cf = [pltpu.bitcast(cw[rc(a, n, q), lt], F32) for a, n in rows]
                        ws = [dwb[a * 3 + 1, sf, :] for a in range(3)]
                        cs = [(ca[o * 16:(o + 1) * 16, :] + ws[0] * cf[o]) + (ws[1] * cf[o + 1] + ws[2] * cf[o + 2])
                              for o in range(2)]
                    for o in range(2):
                        c = cs[o]
                        cbuf[d, o, sf, lt] = c
                        a = c[0:8] + c[8:16]
                        b = c[0:8] * c[0:8] + c[8:16] * c[8:16]
                        s1[o] = a if s1[o] is None else s1[o] + a
                        s2[o] = b if s2[o] is None else s2[o] + b
                    if q == QS[-1]:
                        for o in range(2):
                            stat[d % 2, o, 0, :, lt] = s1[o]
                            stat[d % 2, o, 1, :, lt] = s2[o]
                        if t == NT - 1:
                            m = butterfly(tiles(stat[d % 2, 0, 0]) + tiles(stat[d % 2, 1, 0])) * (1.0 / C)
                            q2 = butterfly(tiles(stat[d % 2, 0, 1]) + tiles(stat[d % 2, 1, 1])) * (1.0 / C)
                            var = jnp.maximum(q2 - m * m, 0.0)
                            rs = jax.lax.rsqrt(var + 1e-5) * _KAPPA
                            nrm[d] = rs
                            if kidx is not None:
                                rst[kidx] = rs
                    yield

            def body1(c0, slot):
                cur = slot * CH
                nxt = adv(slot, 1) * CH
                last = c0 == NCH - 1

                def xrow(r):
                    return cur + r if r < CH else jnp.where(last, ZROW, nxt + (r - CH))

                def conv_stream():
                    for gam in range(4 * U):
                        p, t = 1 + (gam + 2) // 4, (gam + 2) % 4
                        if t == 0:
                            for q in QS:
                                prep(p % ND, (xrow(2 * p + 1), xrow(2 * p + 2)), q)
                        yield from group(p % ND, t, (c0 + p // U) * NRS + p % U if p % U < NRS else None)

                us = [((r // 2) % ND, r % 2, t, None if r in REC else c0 * NS + STO.index(r))
                      for r in range(CH) for t in range(NT)]
                cs = conv_stream()

                def pull(n):
                    for _ in range(n):
                        next(cs, None)

                pull(PRE)
                for i in range(len(us) // 3):
                    units(us[3 * i:3 * i + 3])
                    pull(12)
                assert next(cs, 'done') == 'done'
                oth = (E - LEFT) // 3
                units(us[-1:], 0, LEFT)
                for i in range(3 if oth else 0):
                    units(us[-1:], LEFT + i * oth, LEFT + (i + 1) * oth)

                cn = c0 + XS

                @pl.when(cn < NCH + P2PRE)
                def _():
                    xcopy(jnp.where(cn < NCH, cn, cn - NCH), slot).start()

                @pl.when(c0 == 0)
                def _():
                    xpart(CH + 5, 2 * CH, 1).wait()

                @pl.when(c0 + 2 < NCH)
                def _():
                    xcopy(c0 + 2, adv(slot, 2)).wait()
                return adv(slot, 1)

            for p, rows in ((-1, (ZROW, 0)), (0, (1, 2)), (1, (3, 4))):
                for q in QS:
                    prep(p % ND, rows, q)
            for p, t in ((0, 0), (0, 1), (0, 2), (0, 3), (1, 0), (1, 1)):
                for _ in group(p, t, 0):
                    pass
            xpart(5, CH + 5, 0).wait()
            xpart(CH + 5, 2 * CH, 1).start()
            for c in range(2, XS):
                xcopy(c, c).start()
            for cp in wcp[2:]:
                cp.wait()
            jax.lax.fori_loop(0, NCH, body1, 0)
            for c in range(NB2 + 1):
                xcopy(c, (NCH + c) % XS).wait()

        pl.run_scoped(
            pass1,
            pltpu.VMEM((NQ, 16, 128), U32),
            pltpu.VMEM((NQ, 16, 128), U32),
            pltpu.VMEM((2 * ND * (C + CROWS), W), U32),
            pltpu.VMEM((ND, 2, C, W), F32),
            pltpu.VMEM((2, 2, 2, 8, W), F32),
            pltpu.VMEM((ND, 8, 128), F32),
        )

        for r in range(NX):
            unp((NCH % XS) * CH, r)
        for i in range(2):
            t0(0, i, 0, NCG)

        a = jnp.transpose(acc[...])
        ssq = jnp.sum(a, axis=0, keepdims=True) * (1.0 / (_GS * _GS))
        gx = jnp.sqrt(ssq + 1e-6)
        nx = gx / (jnp.mean(gx, axis=1, keepdims=True) + 1e-6)
        s = (gam_ref[...].astype(F32).reshape(1, E) * nx + 1.0) * (1.0 / _GS)
        w2f = w2t_ref[...].astype(F32)
        w2s[...] = _u((w2f * s).astype(BF16))
        b = jnp.sum(w2f * bet_ref[...].astype(F32).reshape(1, E), axis=1, keepdims=True)
        b2b[...] = jnp.broadcast_to(b, (C, 128))

        def pass2(gt):
            def opiece(c, slot, lo, hi):
                return pltpu.make_async_copy(
                    xr.at[pl.ds(slot * CH + lo, hi - lo)], o_hbm.at[pl.ds(c * CH + lo, hi - lo)], osem.at[slot])

            def owait(c, slot):
                opiece(c, slot, 0, CH).wait()

            def anchor(v, z):
                dwb[9 + z, 0:8, :] = v

            def t1(i, z, fn):
                v_all = mm1(jnp.concatenate([xn2[i], jnp.zeros((128 - C, W), BF16)], axis=0))
                for k, xa in enumerate(XA):
                    xr[ZROW + z, 0:8, 0:128] = v_all[xa:xa + 8, 0:128].astype(BF16)
                    fn(k * C // len(XA), (k + 1) * C // len(XA))
                an = None
                for e in range(E // 16):
                    g = gelu(v_all[e * 16:(e + 1) * 16, :])
                    gt[i % 2, e * 16:(e + 1) * 16, :] = g.astype(BF16)
                    an = g[8:16, W - 128:W] if an is None else an + g[8:16, W - 128:W]
                anchor(an, z)

            def chunk2(c, slot, z):
                xb = slot * CH
                c2 = jnp.minimum(c + 1, NCH - 1)
                xb2 = jnp.where(c + 1 < NCH, adv(slot, 1), slot) * CH
                done = set()

                def t2(g, row, hook=False):
                    y = jnp.dot(_b(w2s[...]), g, preferred_element_type=F32)
                    bb = jnp.concatenate([b2b[...]] * NT, axis=1)
                    xr[xb + row] = (y + (bb + xr[xb + row].astype(F32))).astype(BF16)
                    if hook:
                        an = y[0:8, STILE * 128:(STILE + 1) * 128]
                        for cg in range(1, NCG):
                            an = an + y[cg * 8:(cg + 1) * 8, STILE * 128:(STILE + 1) * 128]
                        anchor(an, z)

                def out(row):
                    done.add(row)
                    for lo, hi in PIECES:
                        if lo <= row < hi and all(r in done for r in range(lo, hi)):
                            opiece(c, slot, lo, hi).start()

                def t0n(i, cg0, cg1):
                    if i < NR:
                        t0(c, i, cg0, cg1)
                    else:
                        t0(c2, i - NR, cg0, cg1)

                si = 0
                for i in range(NR):
                    t1(i, z, lambda lo, hi: [unp(xb2, r, lo, hi) for r in PROD[i]])
                    t0n(i + 2, 0, SPLIT)
                    if i > 0:
                        row = REC[i - 1]
                        t2(gt[(i - 1) % 2], row, True)
                    else:
                        row = STO[si]
                        t2(hst[c * NS + si], row, True)
                        si += 1
                    t0n(i + 2, SPLIT, NCG)
                    out(row)
                    t2(hst[c * NS + si], STO[si])
                    out(STO[si])
                    si += 1
                t2(gt[(NR - 1) % 2], REC[NR - 1])
                out(REC[NR - 1])
                while si < NS:
                    t2(hst[c * NS + si], STO[si])
                    out(STO[si])
                    si += 1

            def body2(i, slot):
                c0 = i * NB2
                z = zs[0]
                for h in range(NB2):
                    chunk2(c0 + h, adv(slot, h), z)
                for h in range(NB2):
                    ps = adv(slot, XS - NB2 + h)

                    @pl.when(i > 0)
                    def _():
                        owait(c0 - NB2 + h, ps)

                    @pl.when(c0 + P2PRE + h < NCH)
                    def _():
                        xcopy(c0 + P2PRE + h, ps).start()
                for h in range(NB2):
                    @pl.when(c0 + NB2 + 1 + h < NCH)
                    def _():
                        xcopy(c0 + NB2 + 1 + h, adv(slot, NB2 + 1 + h)).wait()
                return adv(slot, NB2)

            s0 = NCH % XS
            jax.lax.fori_loop(0, NCH // NB2, body2, s0)
            for c in range(NCH - NB2, NCH):
                owait(c, (s0 + c) % XS)

        pl.run_scoped(pass2, pltpu.VMEM((2, E, W), BF16))

    @jax.jit
    def f(x, dw, w1, w2, grn_gamma, grn_beta):
        xt = jnp.transpose(x, (0, 1, 3, 2)).reshape(H, C, W)
        w2t = jnp.transpose(w2)
        hbm = pl.BlockSpec(memory_space=pl.ANY)
        out = pl.pallas_call(
            kernel,
            in_specs=[hbm] * 6,
            out_specs=hbm,
            out_shape=jax.ShapeDtypeStruct((H, C, W), BF16),
            scratch_shapes=[
                pltpu.VMEM((NCH * NS, E, W), BF16),
                pltpu.VMEM((XS * CH + 1, C, W), BF16),
                pltpu.VMEM((NX * C, W), F32),
                pltpu.VMEM((NR, C, W), BF16),
                pltpu.VMEM(((NCH + 1) * NRS, 8, 128), F32),
                pltpu.VMEM((10, C, 128), F32),
                pltpu.VMEM((E // 2, 128), U32),
                pltpu.VMEM((E, 128), F32),
                pltpu.VMEM((C, 128), F32),
                pltpu.VMEM((C // 2, E), U32),
                pltpu.VMEM((3, 3, C), BF16),
                pltpu.VMEM((C, E), BF16),
                pltpu.VMEM((C, E), BF16),
                pltpu.VMEM((E,), BF16),
                pltpu.VMEM((E,), BF16),
                pltpu.SMEM((1,), jnp.int32),
                pltpu.SemaphoreType.DMA((XS,)),
                pltpu.SemaphoreType.DMA((XS,)),
                pltpu.SemaphoreType.DMA((5,)),
            ],
            compiler_params=pltpu.CompilerParams(vmem_limit_bytes=128 << 20, disable_bounds_checks=True),
        )(xt, dw, w1, w2t, grn_gamma, grn_beta)
        return jnp.transpose(out.reshape(1, H, C, W), (0, 1, 3, 2))
    return f


pallas_standalone__modern_conv_block_convnext_v2__vision_kernel = build(**{})
```

```python
import functools
import math

import jax
import jax.numpy as jnp
import jax.experimental.pallas as pl
import jax.experimental.pallas.tpu as pltpu

F32 = jnp.float32
BF16 = jnp.bfloat16
U32 = jnp.uint32

_C0 = math.sqrt(2.0 / math.pi)
_KAPPA = (_C0 * 0.044715) ** (1.0 / 3.0)
_A = _C0 / _KAPPA
_GS = 2.0 * _KAPPA


def _u(x):
    return pltpu.bitcast(x, U32)


def _b(x):
    return pltpu.bitcast(x, BF16)


def build(FOLD=True, NBQ=2, XS=7, NB2=2, QS=(2, 3, 0, 4, 5, 1), PRE=12, LEFT=240, SPLIT=6, STILE=2, XA=(32, 128, 224, 320),
          PROD=((0, 1), (2,), (3,), (4,), (5,), (6,), (7, 8)),
          PIECES=((0, 4), (8, 12), (4, 6), (12, 14), (6, 8), (14, 16))):
    H, W, C, E = 512, 512, 96, 384
    NT = W // 128
    NQ = C // 16
    NCG = C // 8
    CH = 16
    NCH = H // CH
    U = CH // 2
    NR = 7
    REC = list(range(1, NR + 1))
    STO = [r for r in range(CH) if r not in REC]
    NS = len(STO)
    NX = NR + 2
    NRS = NR // 2 + 1
    ZROW = XS * CH
    P2PRE = XS - NB2
    ND = 4
    CROWS = NBQ * 8 + (NQ - NBQ) * 16

    def kernel(x_hbm, dw_hbm, w1_hbm, w2t_hbm, gam_hbm, bet_hbm,
               o_hbm,
               hst, xr, wk, xn2, rst, dwb, w1t, acc, b2b, w2s,
               dw_ref, w1_ref, w2t_ref, gam_ref, bet_ref, zs, xsem, osem, wsem):

        def xcopy(c, slot):
            return pltpu.make_async_copy(
                x_hbm.at[pl.ds(c * CH, CH)], xr.at[pl.ds(slot * CH, CH)], xsem.at[slot])

        def xpart(lo, hi, sem):
            return pltpu.make_async_copy(x_hbm.at[pl.ds(lo, hi - lo)], xr.at[pl.ds(lo, hi - lo)], xsem.at[sem])

        def adv(s, n):
            s = s + n
            return jnp.where(s >= XS, s - XS, s)

        wcp = [pltpu.make_async_copy(src, dst, wsem.at[i]) for i, (src, dst) in enumerate(
            [(dw_hbm, dw_ref), (w1_hbm, w1_ref), (w2t_hbm, w2t_ref), (gam_hbm, gam_ref), (bet_hbm, bet_ref)])]
        wcp[0].start()
        wcp[1].start()
        xpart(0, 5, 1).start()
        xpart(5, CH + 5, 0).start()
        for cp in wcp[2:]:
            cp.start()
        zs[0] = 0
        wcp[0].wait()
        wcp[1].wait()
        xpart(0, 5, 1).wait()

        def tiles(v):
            return [v[:, t * 128:(t + 1) * 128] for t in range(NT)]

        def mm1(xp, e0=0, e1=E):
            return jnp.dot(_b(w1t[e0 // 2:e1 // 2, :]), xp, preferred_element_type=F32)

        def gelu(v):
            z = v * (v * v + _A)
            return v * (jnp.tanh(z) + 1.0)

        lane = jax.lax.broadcasted_iota(jnp.int32, (8, 128), 1)
        m0 = lane == 0
        m127 = lane == 127

        def unp(xb, r, lo=0, hi=C):
            wk[r * C + lo:r * C + hi, :] = xr[xb + r, lo:hi, :].astype(F32)

        def t0(c, i, cg0, cg1):
            r = REC[i]
            rs = [rst[c * NRS + r // 2, (r % 2) * 4 + t:(r % 2) * 4 + t + 1, :] for t in range(NT)]
            for cg in range(cg0, cg1):
                sl = slice(cg * 8, cg * 8 + 8)
                xs = [tiles(wk[(r - 1 + a) * C + cg * 8:(r - 1 + a) * C + cg * 8 + 8, :]) for a in range(3)]
                cs = []
                for b in range(3):
                    ws = [dwb[a * 3 + b, sl, :] for a in range(3)]
                    cs.append([ws[0] * xs[0][t] + ws[1] * xs[1][t] + ws[2] * xs[2][t] for t in range(NT)])
                rl = [pltpu.roll(cs[0][t], 1, 1) for t in range(NT)]
                rg = [pltpu.roll(cs[2][t], 127, 1) for t in range(NT)]
                row = []
                for t in range(NT):
                    left = jnp.where(m0, rl[t - 1] if t > 0 else 0.0, rl[t])
                    right = jnp.where(m127, rg[t + 1] if t < NT - 1 else 0.0, rg[t])
                    row.append((cs[1][t] + (left + right)) * rs[t])
                xn2[i, sl, :] = jnp.concatenate(row, axis=1).astype(BF16)

        def pass1(la, lb, cw, cbuf, stat, nrm):
            rr = jax.lax.broadcasted_iota(jnp.int32, (C, C), 0)
            cc = jax.lax.broadcasted_iota(jnp.int32, (C, C), 1)
            for a in range(3):
                for b in range(3):
                    row = dw_ref[a, b:b + 1, :].astype(F32)
                    d = jnp.where(rr == cc, jnp.broadcast_to(row, (C, C)), 0.0)
                    col = jnp.sum(d, axis=1, keepdims=True)
                    dwb[a * 3 + b] = jnp.broadcast_to(col, (C, 128))
            r16 = jax.lax.broadcasted_iota(jnp.int32, (16, 128), 0)
            c16 = jax.lax.broadcasted_iota(jnp.int32, (16, 128), 1)
            for q in range(NQ):
                ta, tb = [], []
                sf = slice(q * 16, q * 16 + 16)
                for o in range(2):
                    ma = jnp.zeros((16, 128), F32)
                    mb = jnp.zeros((16, 128), F32)
                    for a in range(3):
                        ma = jnp.where(c16 == (a + o) * 16 + r16, dwb[a * 3 + 0, sf, :], ma)
                        ma = jnp.where(c16 == (4 + a + o) * 16 + r16, dwb[a * 3 + 2, sf, :], ma)
                        mb = jnp.where(c16 == (a + o) * 16 + r16, dwb[a * 3 + 1, sf, :], mb)
                    ta.append(ma)
                    tb.append(mb)
                la[q] = _u(jnp.concatenate(ta, axis=0).astype(BF16))
                lb[q] = _u(jnp.concatenate(tb, axis=0).astype(BF16))
            re = jax.lax.broadcasted_iota(jnp.int32, (E, E), 0)
            ce = jax.lax.broadcasted_iota(jnp.int32, (E, E), 1)
            eye = jnp.where(re == ce, 1.0, 0.0).astype(BF16)
            w1f = w1_ref[...].astype(F32)
            w1c = (w1f - jnp.mean(w1f, axis=0, keepdims=True)).astype(BF16).astype(F32)
            aw = jnp.abs(w1c)
            small = aw <= jnp.maximum(0.3 * jnp.mean(aw, axis=0, keepdims=True), jnp.min(aw, axis=0, keepdims=True))
            cnt = jnp.sum(jnp.where(small, 1.0, 0.0), axis=0, keepdims=True)
            w1c = jnp.where(small, w1c - jnp.sum(w1c, axis=0, keepdims=True) / cnt, w1c).astype(BF16)
            w1p = jnp.concatenate([w1c, jnp.zeros((128 - C, E), BF16)], axis=0)
            t = jax.lax.dot_general(eye, w1p, (((1,), (1,)), ((), ())),
                                    preferred_element_type=F32)
            w1t[...] = _u(t.astype(BF16))
            acc[...] = jnp.zeros_like(acc)
            for i in range(2 * ND):
                cw[i * C:i * C + C // 2, 0:128] = jnp.zeros((C // 2, 128), U32)
                cw[i * C + C // 2:(i + 1) * C, W - 128:W] = jnp.zeros((C // 2, 128), U32)
            xr[ZROW] = jnp.zeros((C, W), BF16)

            sub = jax.lax.broadcasted_iota(jnp.int32, (8, 128), 0)

            def butterfly(vs):
                for d in (1, 2, 4):
                    mk = (sub % (2 * d)) < d
                    vs = [jnp.where(mk, vs[i], vs[i + 1]) + pltpu.roll(jnp.where(mk, vs[i + 1], vs[i]), d, 0)
                          for i in range(0, len(vs), 2)]
                return vs[0]

            def rlr(d, n, lr, q):
                o = ((d * 2 + n) * 2 + lr) * (C // 2) + q * 8
                return slice(o, o + 8)

            def rc(d, n, q):
                o = 2 * ND * C + (d * 2 + n) * CROWS
                if q < NBQ:
                    return slice(o + q * 8, o + q * 8 + 8)
                o += NBQ * 8 + (q - NBQ) * 16
                return slice(o, o + 16)

            def units(us, e0=0, e1=E):
                xs = [cbuf[d, o, :, t * 128:(t + 1) * 128] * nrm[d, o * 4 + t:o * 4 + t + 1, :]
                      for d, o, t, _ in us]
                xn = xs[0] if len(xs) == 1 else jnp.concatenate(xs, axis=1)
                pad = jnp.zeros((128 - C, 128 * len(us)), F32)
                v_all = mm1(jnp.concatenate([xn, pad], axis=0).astype(BF16), e0, e1)
                spans = []
                i = 0
                while i < len(us):
                    d, o, t, h = us[i]
                    n = 2 if (i + 1 < len(us) and t % 2 == 0 and us[i + 1][:3] == (d, o, t + 1)) else 1
                    if h is not None:
                        spans.append((i, n, t, h))
                    i += n
                for e in range(e0 // 16, e1 // 16):
                    g = gelu(v_all[e * 16 - e0:(e + 1) * 16 - e0, :])
                    g2 = g * g
                    a = g2[:, 0:128]
                    for i in range(1, len(us)):
                        a = a + g2[:, i * 128:(i + 1) * 128]
                    acc[e * 16:(e + 1) * 16, :] += a
                    for i, n, t, h in spans:
                        gi = g[:, i * 128:(i + n) * 128]
                        if n == 2 or not FOLD:
                            hst[h, e * 16:(e + 1) * 16, t * 128:(t + n) * 128] = gi.astype(BF16)
                        else:
                            o = (t % 2) * (E // 2) + e * 8
                            hst[h, o:o + 8, (t // 2) * 256:(t // 2 + 1) * 256] = (
                                jnp.concatenate([gi[0:8], gi[8:16]], axis=1).astype(BF16))

            def prep(d, rows, q):
                sf = slice(q * 16, q * 16 + 16)
                for n in range(2):
                    p = _u(xr[rows[n], sf, :])
                    pt = tiles(p)
                    rl = [pltpu.roll(pt[t], 1, 1) for t in range(NT)]
                    rg = [pltpu.roll(pt[t], 127, 1) for t in range(NT)]
                    for t in range(NT):
                        lt = slice(t * 128, (t + 1) * 128)
                        pltpu.store(cw.at[rlr(d, n, 0, q), lt], rl[t], mask=lane != 0)
                        pltpu.store(cw.at[rlr(d, n, 1, q), lt], rg[t], mask=lane != 127)
                        if t > 0:
                            pltpu.store(cw.at[rlr(d, n, 0, q), lt], rl[t - 1], mask=m0)
                        if t < NT - 1:
                            pltpu.store(cw.at[rlr(d, n, 1, q), lt], rg[t + 1], mask=m127)
                    if q < NBQ:
                        cw[rc(d, n, q), :] = p
                    else:
                        cw[rc(d, n, q), :] = _u(_b(p).astype(F32))

            def group(d, t, kidx):
                lt = slice(t * 128, (t + 1) * 128)
                s1 = [None, None]
                s2 = [None, None]
                rows = [((d - 1) % ND, 0), ((d - 1) % ND, 1), (d, 0), (d, 1)]
                for q in QS:
                    sf = slice(q * 16, q * 16 + 16)
                    rhs = [cw[rlr(a, n, 0, q), lt] for a, n in rows] + [cw[rlr(a, n, 1, q), lt] for a, n in rows]
                    ca = jnp.dot(_b(la[q]), _b(jnp.concatenate(rhs, axis=0)), preferred_element_type=F32)
                    if q < NBQ:
                        yield
                        rb = [cw[rc(a, n, q), lt] for a, n in rows] + [jnp.zeros((32, 128), U32)]
                        ca = ca + jnp.dot(_b(lb[q]), _b(jnp.concatenate(rb, axis=0)),
                                          preferred_element_type=F32)
                        cs = [ca[o * 16:(o + 1) * 16, :] for o in range(2)]
                    else:
                        cf = [pltpu.bitcast(cw[rc(a, n, q), lt], F32) for a, n in rows]
                        ws = [dwb[a * 3 + 1, sf, :] for a in range(3)]
                        cs = [(ca[o * 16:(o + 1) * 16, :] + ws[0] * cf[o]) + (ws[1] * cf[o + 1] + ws[2] * cf[o + 2])
                              for o in range(2)]
                    for o in range(2):
                        c = cs[o]
                        cbuf[d, o, sf, lt] = c
                        a = c[0:8] + c[8:16]
                        b = c[0:8] * c[0:8] + c[8:16] * c[8:16]
                        s1[o] = a if s1[o] is None else s1[o] + a
                        s2[o] = b if s2[o] is None else s2[o] + b
                    if q == QS[-1]:
                        for o in range(2):
                            stat[d % 2, o, 0, :, lt] = s1[o]
                            stat[d % 2, o, 1, :, lt] = s2[o]
                        if t == NT - 1:
                            m = butterfly(tiles(stat[d % 2, 0, 0]) + tiles(stat[d % 2, 1, 0])) * (1.0 / C)
                            q2 = butterfly(tiles(stat[d % 2, 0, 1]) + tiles(stat[d % 2, 1, 1])) * (1.0 / C)
                            var = jnp.maximum(q2 - m * m, 0.0)
                            rs = jax.lax.rsqrt(var + 1e-5) * _KAPPA
                            nrm[d] = rs
                            if kidx is not None:
                                rst[kidx] = rs
                    yield

            def body1(c0, slot):
                cur = slot * CH
                nxt = adv(slot, 1) * CH
                last = c0 == NCH - 1

                def xrow(r):
                    return cur + r if r < CH else jnp.where(last, ZROW, nxt + (r - CH))

                def conv_stream():
                    for gam in range(4 * U):
                        p, t = 1 + (gam + 2) // 4, (gam + 2) % 4
                        if t == 0:
                            for q in QS:
                                prep(p % ND, (xrow(2 * p + 1), xrow(2 * p + 2)), q)
                        yield from group(p % ND, t, (c0 + p // U) * NRS + p % U if p % U < NRS else None)

                us = [((r // 2) % ND, r % 2, t, None if r in REC else c0 * NS + STO.index(r))
                      for r in range(CH) for t in range(NT)]
                cs = conv_stream()

                def pull(n):
                    for _ in range(n):
                        next(cs, None)

                pull(PRE)
                for i in range(len(us) // 3):
                    units(us[3 * i:3 * i + 3])
                    pull(12)
                assert next(cs, 'done') == 'done'
                oth = (E - LEFT) // 3
                units(us[-1:], 0, LEFT)
                for i in range(3 if oth else 0):
                    units(us[-1:], LEFT + i * oth, LEFT + (i + 1) * oth)

                cn = c0 + XS

                @pl.when(cn < NCH + P2PRE)
                def _():
                    xcopy(jnp.where(cn < NCH, cn, cn - NCH), slot).start()

                @pl.when(c0 == 0)
                def _():
                    xpart(CH + 5, 2 * CH, 1).wait()

                @pl.when(c0 + 2 < NCH)
                def _():
                    xcopy(c0 + 2, adv(slot, 2)).wait()
                return adv(slot, 1)

            for p, rows in ((-1, (ZROW, 0)), (0, (1, 2)), (1, (3, 4))):
                for q in QS:
                    prep(p % ND, rows, q)
            for p, t in ((0, 0), (0, 1), (0, 2), (0, 3), (1, 0), (1, 1)):
                for _ in group(p, t, 0):
                    pass
            xpart(5, CH + 5, 0).wait()
            xpart(CH + 5, 2 * CH, 1).start()
            for c in range(2, XS):
                xcopy(c, c).start()
            for cp in wcp[2:]:
                cp.wait()
            jax.lax.fori_loop(0, NCH, body1, 0)
            for c in range(NB2 + 1):
                xcopy(c, (NCH + c) % XS).wait()

        pl.run_scoped(
            pass1,
            pltpu.VMEM((NQ, 16, 128), U32),
            pltpu.VMEM((NQ, 16, 128), U32),
            pltpu.VMEM((2 * ND * (C + CROWS), W), U32),
            pltpu.VMEM((ND, 2, C, W), F32),
            pltpu.VMEM((2, 2, 2, 8, W), F32),
            pltpu.VMEM((ND, 8, 128), F32),
        )

        for r in range(NX):
            unp((NCH % XS) * CH, r)
        for i in range(2):
            t0(0, i, 0, NCG)

        a = jnp.transpose(acc[...])
        ssq = jnp.sum(a, axis=0, keepdims=True) * (1.0 / (_GS * _GS))
        gx = jnp.sqrt(ssq + 1e-6)
        nx = gx / (jnp.mean(gx, axis=1, keepdims=True) + 1e-6)
        s = (gam_ref[...].astype(F32).reshape(1, E) * nx + 1.0) * (1.0 / _GS)
        w2f = w2t_ref[...].astype(F32)
        w2s[...] = _u((w2f * s).astype(BF16))
        b = jnp.sum(w2f * bet_ref[...].astype(F32).reshape(1, E), axis=1, keepdims=True)
        b2b[...] = jnp.broadcast_to(b, (C, 128))

        def pass2(gt):
            def opiece(c, slot, lo, hi):
                return pltpu.make_async_copy(
                    xr.at[pl.ds(slot * CH + lo, hi - lo)], o_hbm.at[pl.ds(c * CH + lo, hi - lo)], osem.at[slot])

            def owait(c, slot):
                opiece(c, slot, 0, CH).wait()

            def anchor(v, z):
                dwb[9 + z, 0:8, :] = v

            def t1(i, z, fn):
                v_all = mm1(jnp.concatenate([xn2[i], jnp.zeros((128 - C, W), BF16)], axis=0))
                for k, xa in enumerate(XA):
                    xr[ZROW + z, 0:8, 0:128] = v_all[xa:xa + 8, 0:128].astype(BF16)
                    fn(k * C // len(XA), (k + 1) * C // len(XA))
                an = None
                for e in range(E // 16):
                    g = gelu(v_all[e * 16:(e + 1) * 16, :])
                    gt[i % 2, e * 16:(e + 1) * 16, :] = g.astype(BF16)
                    an = g[8:16, W - 128:W] if an is None else an + g[8:16, W - 128:W]
                anchor(an, z)

            def chunk2(c, slot, z):
                xb = slot * CH
                c2 = jnp.minimum(c + 1, NCH - 1)
                xb2 = jnp.where(c + 1 < NCH, adv(slot, 1), slot) * CH
                done = set()

                def t2(g, row, hook=False):
                    y = jnp.dot(_b(w2s[...]), g, preferred_element_type=F32)
                    bb = jnp.concatenate([b2b[...]] * NT, axis=1)
                    xr[xb + row] = (y + (bb + xr[xb + row].astype(F32))).astype(BF16)
                    if hook:
                        an = y[0:8, STILE * 128:(STILE + 1) * 128]
                        for cg in range(1, NCG):
                            an = an + y[cg * 8:(cg + 1) * 8, STILE * 128:(STILE + 1) * 128]
                        anchor(an, z)

                def hrow(si):
                    h, r = c * NS + si, STO[si]
                    halves = []
                    for hf in range(2):
                        lanes = slice(hf * 256, (hf + 1) * 256)
                        if not FOLD or (4 * r + 2 * hf) // 3 == (4 * r + 2 * hf + 1) // 3:
                            halves.append(hst[h, :, lanes])
                            continue
                        for k in range(2):
                            parts = []
                            for e in range(E // 16):
                                v = hst[h, k * (E // 2) + e * 8:k * (E // 2) + e * 8 + 8, lanes]
                                parts += [v[:, 0:128], v[:, 128:256]]
                            halves.append(jnp.concatenate(parts, axis=0))
                    return jnp.concatenate(halves, axis=1)

                def out(row):
                    done.add(row)
                    for lo, hi in PIECES:
                        if lo <= row < hi and all(r in done for r in range(lo, hi)):
                            opiece(c, slot, lo, hi).start()

                def t0n(i, cg0, cg1):
                    if i < NR:
                        t0(c, i, cg0, cg1)
                    else:
                        t0(c2, i - NR, cg0, cg1)

                si = 0
                for i in range(NR):
                    t1(i, z, lambda lo, hi: [unp(xb2, r, lo, hi) for r in PROD[i]])
                    t0n(i + 2, 0, SPLIT)
                    if i > 0:
                        row = REC[i - 1]
                        t2(gt[(i - 1) % 2], row, True)
                    else:
                        row = STO[si]
                        t2(hrow(si), row, True)
                        si += 1
                    t0n(i + 2, SPLIT, NCG)
                    out(row)
                    t2(hrow(si), STO[si])
                    out(STO[si])
                    si += 1
                t2(gt[(NR - 1) % 2], REC[NR - 1])
                out(REC[NR - 1])
                while si < NS:
                    t2(hrow(si), STO[si])
                    out(STO[si])
                    si += 1

            def body2(i, slot):
                c0 = i * NB2
                z = zs[0]
                for h in range(NB2):
                    chunk2(c0 + h, adv(slot, h), z)
                for h in range(NB2):
                    ps = adv(slot, XS - NB2 + h)

                    @pl.when(i > 0)
                    def _():
                        owait(c0 - NB2 + h, ps)

                    @pl.when(c0 + P2PRE + h < NCH)
                    def _():
                        xcopy(c0 + P2PRE + h, ps).start()
                for h in range(NB2):
                    @pl.when(c0 + NB2 + 1 + h < NCH)
                    def _():
                        xcopy(c0 + NB2 + 1 + h, adv(slot, NB2 + 1 + h)).wait()
                return adv(slot, NB2)

            s0 = NCH % XS
            jax.lax.fori_loop(0, NCH // NB2, body2, s0)
            for c in range(NCH - NB2, NCH):
                owait(c, (s0 + c) % XS)

        pl.run_scoped(pass2, pltpu.VMEM((2, E, W), BF16))

    @jax.jit
    def f(x, dw, w1, w2, grn_gamma, grn_beta):
        xt = jnp.transpose(x, (0, 1, 3, 2)).reshape(H, C, W)
        w2t = jnp.transpose(w2)
        hbm = pl.BlockSpec(memory_space=pl.ANY)
        out = pl.pallas_call(
            kernel,
            in_specs=[hbm] * 6,
            out_specs=hbm,
            out_shape=jax.ShapeDtypeStruct((H, C, W), BF16),
            scratch_shapes=[
                pltpu.VMEM((NCH * NS, E, W), BF16),
                pltpu.VMEM((XS * CH + 1, C, W), BF16),
                pltpu.VMEM((NX * C, W), F32),
                pltpu.VMEM((NR, C, W), BF16),
                pltpu.VMEM(((NCH + 1) * NRS, 8, 128), F32),
                pltpu.VMEM((10, C, 128), F32),
                pltpu.VMEM((E // 2, 128), U32),
                pltpu.VMEM((E, 128), F32),
                pltpu.VMEM((C, 128), F32),
                pltpu.VMEM((C // 2, E), U32),
                pltpu.VMEM((3, 3, C), BF16),
                pltpu.VMEM((C, E), BF16),
                pltpu.VMEM((C, E), BF16),
                pltpu.VMEM((E,), BF16),
                pltpu.VMEM((E,), BF16),
                pltpu.SMEM((1,), jnp.int32),
                pltpu.SemaphoreType.DMA((XS,)),
                pltpu.SemaphoreType.DMA((XS,)),
                pltpu.SemaphoreType.DMA((5,)),
            ],
            compiler_params=pltpu.CompilerParams(vmem_limit_bytes=128 << 20, disable_bounds_checks=True),
        )(xt, dw, w1, w2t, grn_gamma, grn_beta)
        return jnp.transpose(out.reshape(1, H, C, W), (0, 1, 3, 2))
    return f


pallas_standalone__modern_conv_block_convnext_v2__vision_kernel = build(**{})
```

```python
import math

import jax
import jax.numpy as jnp
import jax.experimental.pallas as pl
import jax.experimental.pallas.tpu as pltpu

F32 = jnp.float32
BF16 = jnp.bfloat16
U32 = jnp.uint32

_C0 = math.sqrt(2.0 / math.pi)
_KAPPA = (_C0 * 0.044715) ** (1.0 / 3.0)
_A = _C0 / _KAPPA
_GS = 2.0 * _KAPPA


def _u(x):
    return pltpu.bitcast(x, U32)


def _b(x):
    return pltpu.bitcast(x, BF16)


def build(TG=8, PG=1, NBQ=2, XS=7, NB2=2, QS=(2, 3, 0, 4, 5, 1), PRE=12, LEFT=240, STILE=2,
          XA=(32, 128, 224, 320),
          PROD=((0, 1), (2,), (3,), (4,), (5,), (6,), (7, 8)),
          PIECES=((0, 4), (8, 12), (4, 6), (12, 14), (6, 8), (14, 16))):
    H, W, C, E = 512, 512, 96, 384
    NT = W // 128
    NQ = C // 16
    NCG = C // 8
    CH = 16
    NCH = H // CH
    U = CH // 2
    NR = 7
    REC = list(range(1, NR + 1))
    STO = [r for r in range(CH) if r not in REC]
    NS = len(STO)
    NX = NR + 2
    NRS = NR // 2 + 1
    ZROW = XS * CH
    P2PRE = XS - NB2
    ND = 4
    CROWS = NBQ * 8 + (NQ - NBQ) * 16

    def kernel(x_hbm, dw_hbm, w1_hbm, w2t_hbm, gam_hbm, bet_hbm,
               o_hbm,
               hst, xr, wk, xn2, rst, dwb, w1t, acc, b2b, w2s,
               dw_ref, w1_ref, w2t_ref, gam_ref, bet_ref, zs, xsem, osem, wsem):

        def xcopy(c, slot):
            return pltpu.make_async_copy(
                x_hbm.at[pl.ds(c * CH, CH)], xr.at[pl.ds(slot * CH, CH)], xsem.at[slot])

        def xpart(lo, hi, sem):
            return pltpu.make_async_copy(x_hbm.at[pl.ds(lo, hi - lo)], xr.at[pl.ds(lo, hi - lo)], xsem.at[sem])

        def adv(s, n):
            s = s + n
            return jnp.where(s >= XS, s - XS, s)

        wcp = [pltpu.make_async_copy(src, dst, wsem.at[i]) for i, (src, dst) in enumerate(
            [(dw_hbm, dw_ref), (w1_hbm, w1_ref), (w2t_hbm, w2t_ref), (gam_hbm, gam_ref), (bet_hbm, bet_ref)])]
        wcp[0].start()
        wcp[1].start()
        xpart(0, 5, 1).start()
        xpart(5, CH + 5, 0).start()
        for cp in wcp[2:]:
            cp.start()
        zs[0] = 0
        wcp[0].wait()
        wcp[1].wait()
        xpart(0, 5, 1).wait()

        def tiles(v):
            return [v[:, t * 128:(t + 1) * 128] for t in range(NT)]

        def mm1(xp, e0=0, e1=E):
            return jnp.dot(_b(w1t[e0 // 2:e1 // 2, :]), xp, preferred_element_type=F32)

        def gelu(v):
            z = v * (v * v + _A)
            return v * (jnp.tanh(z) + 1.0)

        lane = jax.lax.broadcasted_iota(jnp.int32, (TG, 128), 1)
        m0 = lane == 0
        m127 = lane == 127
        zf = jnp.zeros((TG, 128), F32)
        sel = jax.lax.select

        def unp(xb, r, lo=0, hi=C):
            wk[r * C + lo:r * C + hi, :] = xr[xb + r, lo:hi, :].astype(F32)

        def t0(c, i, half):
            r = REC[i]
            rs = jnp.concatenate(
                [rst[c * NRS + r // 2, (r % 2) * 4 + t:(r % 2) * 4 + t + 1, :] for t in range(NT)], axis=1)
            for lo in range(half * (C // 2), (half + 1) * (C // 2), TG):
                hi = lo + TG
                xs = [wk[(r - 1 + a) * C + lo:(r - 1 + a) * C + hi, :] for a in range(3)]
                cs = []
                for b in range(3):
                    ws = [jnp.concatenate([dwb[a * 3 + b, lo:hi, :]] * NT, axis=1) for a in range(3)]
                    cs.append(ws[0] * xs[0] + ws[1] * xs[1] + ws[2] * xs[2])
                rl = [pltpu.roll(v, 1, 1) for v in tiles(cs[0])]
                rg = [pltpu.roll(v, 127, 1) for v in tiles(cs[2])]
                left = jnp.concatenate(
                    [sel(m0, rl[t - 1] if t > 0 else zf, rl[t]) for t in range(NT)], axis=1)
                right = jnp.concatenate(
                    [sel(m127, rg[t + 1] if t < NT - 1 else zf, rg[t]) for t in range(NT)], axis=1)
                xn2[i, lo:hi, :] = ((cs[1] + (left + right)) * rs).astype(BF16)

        def pass1(la, lb, cw, cbuf, stat, nrm):
            rr = jax.lax.broadcasted_iota(jnp.int32, (C, C), 0)
            cc = jax.lax.broadcasted_iota(jnp.int32, (C, C), 1)
            for a in range(3):
                for b in range(3):
                    row = dw_ref[a, b:b + 1, :].astype(F32)
                    d = jnp.where(rr == cc, jnp.broadcast_to(row, (C, C)), 0.0)
                    col = jnp.sum(d, axis=1, keepdims=True)
                    dwb[a * 3 + b] = jnp.broadcast_to(col, (C, 128))
            r16 = jax.lax.broadcasted_iota(jnp.int32, (16, 128), 0)
            c16 = jax.lax.broadcasted_iota(jnp.int32, (16, 128), 1)
            for q in range(NQ):
                ta, tb = [], []
                sf = slice(q * 16, q * 16 + 16)
                for o in range(2):
                    ma = jnp.zeros((16, 128), F32)
                    mb = jnp.zeros((16, 128), F32)
                    for a in range(3):
                        ma = jnp.where(c16 == (a + o) * 16 + r16, dwb[a * 3 + 0, sf, :], ma)
                        ma = jnp.where(c16 == (4 + a + o) * 16 + r16, dwb[a * 3 + 2, sf, :], ma)
                        mb = jnp.where(c16 == (a + o) * 16 + r16, dwb[a * 3 + 1, sf, :], mb)
                    ta.append(ma)
                    tb.append(mb)
                la[q] = _u(jnp.concatenate(ta, axis=0).astype(BF16))
                lb[q] = _u(jnp.concatenate(tb, axis=0).astype(BF16))
            re = jax.lax.broadcasted_iota(jnp.int32, (E, E), 0)
            ce = jax.lax.broadcasted_iota(jnp.int32, (E, E), 1)
            eye = jnp.where(re == ce, 1.0, 0.0).astype(BF16)
            w1f = w1_ref[...].astype(F32)
            w1c = (w1f - jnp.mean(w1f, axis=0, keepdims=True)).astype(BF16).astype(F32)
            aw = jnp.abs(w1c)
            small = aw <= jnp.maximum(0.3 * jnp.mean(aw, axis=0, keepdims=True), jnp.min(aw, axis=0, keepdims=True))
            cnt = jnp.sum(jnp.where(small, 1.0, 0.0), axis=0, keepdims=True)
            w1c = jnp.where(small, w1c - jnp.sum(w1c, axis=0, keepdims=True) / cnt, w1c).astype(BF16)
            w1p = jnp.concatenate([w1c, jnp.zeros((128 - C, E), BF16)], axis=0)
            t = jax.lax.dot_general(eye, w1p, (((1,), (1,)), ((), ())),
                                    preferred_element_type=F32)
            w1t[...] = _u(t.astype(BF16))
            acc[...] = jnp.zeros_like(acc)
            for i in range(2 * ND):
                cw[i * C:i * C + C // 2, 0:128] = jnp.zeros((C // 2, 128), U32)
                cw[i * C + C // 2:(i + 1) * C, W - 128:W] = jnp.zeros((C // 2, 128), U32)
            xr[ZROW] = jnp.zeros((C, W), BF16)

            sub = jax.lax.broadcasted_iota(jnp.int32, (8, 128), 0)

            def butterfly(vs):
                for d in (1, 2, 4):
                    mk = (sub % (2 * d)) < d
                    vs = [sel(mk, vs[i], vs[i + 1]) + pltpu.roll(sel(mk, vs[i + 1], vs[i]), d, 0)
                          for i in range(0, len(vs), 2)]
                return vs[0]

            def rlr(d, n, lr, q):
                o = ((d * 2 + n) * 2 + lr) * (C // 2) + q * 8
                return slice(o, o + 8)

            def rc(d, n, q):
                o = 2 * ND * C + (d * 2 + n) * CROWS
                if q < NBQ:
                    return slice(o + q * 8, o + q * 8 + 8)
                o += NBQ * 8 + (q - NBQ) * 16
                return slice(o, o + 16)

            def units(us, e0=0, e1=E):
                xs = [cbuf[d, o, :, t * 128:(t + 1) * 128] * nrm[d, o * 4 + t:o * 4 + t + 1, :]
                      for d, o, t, _ in us]
                xn = xs[0] if len(xs) == 1 else jnp.concatenate(xs, axis=1)
                pad = jnp.zeros((128 - C, 128 * len(us)), F32)
                v_all = mm1(jnp.concatenate([xn, pad], axis=0).astype(BF16), e0, e1)
                spans = []
                i = 0
                while i < len(us):
                    d, o, t, h = us[i]
                    n = 2 if (i + 1 < len(us) and t % 2 == 0 and us[i + 1][:3] == (d, o, t + 1)) else 1
                    if h is not None:
                        spans.append((i, n, t, h))
                    i += n
                g = gelu(v_all)
                g2 = g * g
                a = g2[:, 0:128]
                for i in range(1, len(us)):
                    a = a + g2[:, i * 128:(i + 1) * 128]
                acc[e0:e1, :] += a
                for i, n, t, h in spans:
                    gi = g[:, i * 128:(i + n) * 128]
                    if n == 2:
                        hst[h, e0:e1, t * 128:(t + n) * 128] = gi.astype(BF16)
                    else:
                        o = (t % 2) * (E // 2) + e0 // 2
                        gi = gi.reshape((e1 - e0) // 16, 16, 128)
                        gi = jnp.concatenate([gi[:, 0:8], gi[:, 8:16]], axis=2).reshape((e1 - e0) // 2, 256)
                        hst[h, o:o + (e1 - e0) // 2, (t // 2) * 256:(t // 2 + 1) * 256] = gi.astype(BF16)

            plane = jax.lax.broadcasted_iota(jnp.int32, (PG * 8, 128), 1)
            p0, p127, n0, n127 = plane == 0, plane == 127, plane != 0, plane != 127

            def prep(d, rows):
                for q in (QS if PG == 1 else range(0, NQ, PG)):
                    for n in range(2):
                        p = _u(xr[rows[n], q * 16:(q + PG) * 16, :])
                        pt = tiles(p)
                        rl = [pltpu.roll(pt[t], 1, 1) for t in range(NT)]
                        rg = [pltpu.roll(pt[t], 127, 1) for t in range(NT)]
                        ol, orr = rlr(d, n, 0, q).start, rlr(d, n, 1, q).start
                        sl, sr = slice(ol, ol + PG * 8), slice(orr, orr + PG * 8)
                        for t in range(NT):
                            lt = slice(t * 128, (t + 1) * 128)
                            pltpu.store(cw.at[sl, lt], rl[t], mask=n0)
                            pltpu.store(cw.at[sr, lt], rg[t], mask=n127)
                            if t > 0:
                                pltpu.store(cw.at[sl, lt], rl[t - 1], mask=p0)
                            if t < NT - 1:
                                pltpu.store(cw.at[sr, lt], rg[t + 1], mask=p127)
                        o = rc(d, n, q).start
                        if q < NBQ:
                            cw[o:o + PG * 8, :] = p
                        else:
                            cw[o:o + PG * 16, :] = _u(_b(p).astype(F32))

            def group(d, t, kidx):
                lt = slice(t * 128, (t + 1) * 128)
                s1 = [None, None]
                s2 = [None, None]
                rows = [((d - 1) % ND, 0), ((d - 1) % ND, 1), (d, 0), (d, 1)]
                for q in QS:
                    sf = slice(q * 16, q * 16 + 16)
                    rhs = [cw[rlr(a, n, 0, q), lt] for a, n in rows] + [cw[rlr(a, n, 1, q), lt] for a, n in rows]
                    ca = jnp.dot(_b(la[q]), _b(jnp.concatenate(rhs, axis=0)), preferred_element_type=F32)
                    if q < NBQ:
                        yield
                        rb = [cw[rc(a, n, q), lt] for a, n in rows] + [jnp.zeros((32, 128), U32)]
                        ca = ca + jnp.dot(_b(lb[q]), _b(jnp.concatenate(rb, axis=0)),
                                          preferred_element_type=F32)
                        cs = [ca[o * 16:(o + 1) * 16, :] for o in range(2)]
                    else:
                        cf = [pltpu.bitcast(cw[rc(a, n, q), lt], F32) for a, n in rows]
                        ws = [dwb[a * 3 + 1, sf, :] for a in range(3)]
                        cs = [(ca[o * 16:(o + 1) * 16, :] + ws[0] * cf[o]) + (ws[1] * cf[o + 1] + ws[2] * cf[o + 2])
                              for o in range(2)]
                    for o in range(2):
                        c = cs[o]
                        cbuf[d, o, sf, lt] = c
                        a = c[0:8] + c[8:16]
                        b = c[0:8] * c[0:8] + c[8:16] * c[8:16]
                        s1[o] = a if s1[o] is None else s1[o] + a
                        s2[o] = b if s2[o] is None else s2[o] + b
                    if q == QS[-1]:
                        for o in range(2):
                            stat[d % 2, o, 0, :, lt] = s1[o]
                            stat[d % 2, o, 1, :, lt] = s2[o]
                        if t == NT - 1:
                            m = butterfly(tiles(stat[d % 2, 0, 0]) + tiles(stat[d % 2, 1, 0])) * (1.0 / C)
                            q2 = butterfly(tiles(stat[d % 2, 0, 1]) + tiles(stat[d % 2, 1, 1])) * (1.0 / C)
                            var = jnp.maximum(q2 - m * m, 0.0)
                            rs = jax.lax.rsqrt(var + 1e-5) * _KAPPA
                            nrm[d] = rs
                            if kidx is not None:
                                rst[kidx] = rs
                    yield

            def body1(c0, slot):
                cur = slot * CH
                nxt = adv(slot, 1) * CH
                last = c0 == NCH - 1

                def xrow(r):
                    return cur + r if r < CH else jnp.where(last, ZROW, nxt + (r - CH))

                def conv_stream():
                    for gam in range(4 * U):
                        p, t = 1 + (gam + 2) // 4, (gam + 2) % 4
                        if t == 0:
                            prep(p % ND, (xrow(2 * p + 1), xrow(2 * p + 2)))
                        yield from group(p % ND, t, (c0 + p // U) * NRS + p % U if p % U < NRS else None)

                us = [((r // 2) % ND, r % 2, t, None if r in REC else c0 * NS + STO.index(r))
                      for r in range(CH) for t in range(NT)]
                cs = conv_stream()

                def pull(n):
                    for _ in range(n):
                        next(cs, None)

                pull(PRE)
                for i in range(len(us) // 3):
                    units(us[3 * i:3 * i + 3])
                    pull(12)
                assert next(cs, 'done') == 'done'
                oth = (E - LEFT) // 3
                units(us[-1:], 0, LEFT)
                for i in range(3 if oth else 0):
                    units(us[-1:], LEFT + i * oth, LEFT + (i + 1) * oth)

                cn = c0 + XS

                @pl.when(cn < NCH + P2PRE)
                def _():
                    xcopy(jnp.where(cn < NCH, cn, cn - NCH), slot).start()

                @pl.when(c0 == 0)
                def _():
                    xpart(CH + 5, 2 * CH, 1).wait()

                @pl.when(c0 + 2 < NCH)
                def _():
                    xcopy(c0 + 2, adv(slot, 2)).wait()
                return adv(slot, 1)

            for p, rows in ((-1, (ZROW, 0)), (0, (1, 2)), (1, (3, 4))):
                prep(p % ND, rows)
            for p, t in ((0, 0), (0, 1), (0, 2), (0, 3), (1, 0), (1, 1)):
                for _ in group(p, t, 0):
                    pass
            xpart(5, CH + 5, 0).wait()
            xpart(CH + 5, 2 * CH, 1).start()
            for c in range(2, XS):
                xcopy(c, c).start()
            for cp in wcp[2:]:
                cp.wait()
            jax.lax.fori_loop(0, NCH, body1, 0)
            for c in range(NB2 + 1):
                xcopy(c, (NCH + c) % XS).wait()

        pl.run_scoped(
            pass1,
            pltpu.VMEM((NQ, 16, 128), U32),
            pltpu.VMEM((NQ, 16, 128), U32),
            pltpu.VMEM((2 * ND * (C + CROWS), W), U32),
            pltpu.VMEM((ND, 2, C, W), F32),
            pltpu.VMEM((2, 2, 2, 8, W), F32),
            pltpu.VMEM((ND, 8, 128), F32),
        )

        for r in range(NX):
            unp((NCH % XS) * CH, r)
        for i in range(2):
            t0(0, i, 0)
            t0(0, i, 1)

        a = jnp.transpose(acc[...])
        ssq = jnp.sum(a, axis=0, keepdims=True) * (1.0 / (_GS * _GS))
        gx = jnp.sqrt(ssq + 1e-6)
        nx = gx / (jnp.mean(gx, axis=1, keepdims=True) + 1e-6)
        s = (gam_ref[...].astype(F32).reshape(1, E) * nx + 1.0) * (1.0 / _GS)
        w2f = w2t_ref[...].astype(F32)
        w2s[...] = _u((w2f * s).astype(BF16))
        b = jnp.sum(w2f * bet_ref[...].astype(F32).reshape(1, E), axis=1, keepdims=True)
        b2b[...] = jnp.broadcast_to(b, (C, 128))

        def pass2(gt):
            def opiece(c, slot, lo, hi):
                return pltpu.make_async_copy(
                    xr.at[pl.ds(slot * CH + lo, hi - lo)], o_hbm.at[pl.ds(c * CH + lo, hi - lo)], osem.at[slot])

            def owait(c, slot):
                opiece(c, slot, 0, CH).wait()

            def anchor(v, z):
                dwb[9 + z, 0:8, :] = v

            def t1(i, z, fn):
                v_all = mm1(jnp.concatenate([xn2[i], jnp.zeros((128 - C, W), BF16)], axis=0))
                for k, xa in enumerate(XA):
                    xr[ZROW + z, 0:8, 0:128] = v_all[xa:xa + 8, 0:128].astype(BF16)
                    fn(k * C // len(XA), (k + 1) * C // len(XA))
                g = gelu(v_all)
                gt[i % 2] = g.astype(BF16)
                anchor(jnp.sum(g[:, W - 128:W].reshape(E // 16, 16, 128)[:, 8:16], axis=0), z)

            def chunk2(c, slot, z):
                xb = slot * CH
                c2 = jnp.minimum(c + 1, NCH - 1)
                xb2 = jnp.where(c + 1 < NCH, adv(slot, 1), slot) * CH
                done = set()

                def t2(g, row, hook=False):
                    y = jnp.dot(_b(w2s[...]), g, preferred_element_type=F32)
                    bb = jnp.concatenate([b2b[...]] * NT, axis=1)
                    xr[xb + row] = (y + (bb + xr[xb + row].astype(F32))).astype(BF16)
                    if hook:
                        anchor(jnp.sum(y[:, STILE * 128:(STILE + 1) * 128].reshape(NCG, 8, 128), axis=0), z)

                def hrow(si):
                    h, r = c * NS + si, STO[si]
                    halves = []
                    for hf in range(2):
                        lanes = slice(hf * 256, (hf + 1) * 256)
                        if (4 * r + 2 * hf) // 3 == (4 * r + 2 * hf + 1) // 3:
                            halves.append(hst[h, :, lanes])
                            continue
                        for k in range(2):
                            v = hst[h, k * (E // 2):(k + 1) * (E // 2), lanes].reshape(E // 16, 8, 256)
                            halves.append(jnp.concatenate([v[:, :, 0:128], v[:, :, 128:256]], axis=1).reshape(E, 128))
                    return jnp.concatenate(halves, axis=1)

                def out(row):
                    done.add(row)
                    for lo, hi in PIECES:
                        if lo <= row < hi and all(r in done for r in range(lo, hi)):
                            opiece(c, slot, lo, hi).start()

                def t0n(i, half):
                    if i < NR:
                        t0(c, i, half)
                    else:
                        t0(c2, i - NR, half)

                si = 0
                for i in range(NR):
                    t1(i, z, lambda lo, hi: [unp(xb2, r, lo, hi) for r in PROD[i]])
                    t0n(i + 2, 0)
                    if i > 0:
                        row = REC[i - 1]
                        t2(gt[(i - 1) % 2], row, True)
                    else:
                        row = STO[si]
                        t2(hrow(si), row, True)
                        si += 1
                    t0n(i + 2, 1)
                    out(row)
                    t2(hrow(si), STO[si])
                    out(STO[si])
                    si += 1
                t2(gt[(NR - 1) % 2], REC[NR - 1])
                out(REC[NR - 1])
                while si < NS:
                    t2(hrow(si), STO[si])
                    out(STO[si])
                    si += 1

            def body2(i, slot):
                c0 = i * NB2
                z = zs[0]
                for h in range(NB2):
                    chunk2(c0 + h, adv(slot, h), z)
                for h in range(NB2):
                    ps = adv(slot, XS - NB2 + h)

                    @pl.when(i > 0)
                    def _():
                        owait(c0 - NB2 + h, ps)

                    @pl.when(c0 + P2PRE + h < NCH)
                    def _():
                        xcopy(c0 + P2PRE + h, ps).start()
                for h in range(NB2):
                    @pl.when(c0 + NB2 + 1 + h < NCH)
                    def _():
                        xcopy(c0 + NB2 + 1 + h, adv(slot, NB2 + 1 + h)).wait()
                return adv(slot, NB2)

            s0 = NCH % XS
            jax.lax.fori_loop(0, NCH // NB2, body2, s0)
            for c in range(NCH - NB2, NCH):
                owait(c, (s0 + c) % XS)

        pl.run_scoped(pass2, pltpu.VMEM((2, E, W), BF16))

    @jax.jit
    def f(x, dw, w1, w2, grn_gamma, grn_beta):
        xt = jnp.transpose(x, (0, 1, 3, 2)).reshape(H, C, W)
        w2t = jnp.transpose(w2)
        hbm = pl.BlockSpec(memory_space=pl.ANY)
        out = pl.pallas_call(
            kernel,
            in_specs=[hbm] * 6,
            out_specs=hbm,
            out_shape=jax.ShapeDtypeStruct((H, C, W), BF16),
            scratch_shapes=[
                pltpu.VMEM((NCH * NS, E, W), BF16),
                pltpu.VMEM((XS * CH + 1, C, W), BF16),
                pltpu.VMEM((NX * C, W), F32),
                pltpu.VMEM((NR, C, W), BF16),
                pltpu.VMEM(((NCH + 1) * NRS, 8, 128), F32),
                pltpu.VMEM((10, C, 128), F32),
                pltpu.VMEM((E // 2, 128), U32),
                pltpu.VMEM((E, 128), F32),
                pltpu.VMEM((C, 128), F32),
                pltpu.VMEM((C // 2, E), U32),
                pltpu.VMEM((3, 3, C), BF16),
                pltpu.VMEM((C, E), BF16),
                pltpu.VMEM((C, E), BF16),
                pltpu.VMEM((E,), BF16),
                pltpu.VMEM((E,), BF16),
                pltpu.SMEM((1,), jnp.int32),
                pltpu.SemaphoreType.DMA((XS,)),
                pltpu.SemaphoreType.DMA((XS,)),
                pltpu.SemaphoreType.DMA((5,)),
            ],
            compiler_params=pltpu.CompilerParams(vmem_limit_bytes=128 << 20, disable_bounds_checks=True),
        )(xt, dw, w1, w2t, grn_gamma, grn_beta)
        return jnp.transpose(out.reshape(1, H, C, W), (0, 1, 3, 2))
    return f


pallas_standalone__modern_conv_block_convnext_v2__vision_kernel = build(**{})
```
